```python
import jax
import jax.numpy as jnp

def _softmax(x, axis=-1):
    return jax.nn.softmax(x, axis=axis)
def _gelu(x):
    return jax.nn.gelu(x, approximate=True)
def _silu(x):
    return jax.nn.silu(x)
def _sigmoid(x):
    return jax.nn.sigmoid(x)
def _layernorm(x, axis=-1, eps=1e-5):
    m = jnp.mean(x, axis=axis, keepdims=True)
    v = jnp.var(x, axis=axis, keepdims=True)
    return (x - m) / jnp.sqrt(v + eps)
def _scatter_add(tgt, idx, src, axis=0):
    return tgt.at[idx].add(src)
def _segment_sum(src, seg, n):
    return jax.ops.segment_sum(src, seg, n)
class _Rng:
    def __init__(self, key):
        self._k = key
    def _next(self):
        self._k, sub = jax.random.split(self._k)
        return sub
    def normal(self, shape):
        return jax.random.normal(self._next(), shape, dtype=jnp.bfloat16)
    def randint(self, lo, hi, shape):
        return jax.random.randint(self._next(), shape, lo, hi, dtype=jnp.int32)
    def uniform(self, shape, lo=0.0, hi=1.0):
        return jax.random.uniform(self._next(), shape, jnp.bfloat16, lo, hi)
    def permutation(self, n):
        return jax.random.permutation(self._next(), n)


kernel_name = 'concat_heads__compressed_kv_cla__sliding_local_dilated__prompt'

def setup_inputs():
    _rng = _Rng(jax.random.key(int.from_bytes(__import__("os").urandom(4), "little")))
    _w = (lambda a: (lambda t: t.astype(jnp.bfloat16) if jnp.issubdtype(t.dtype, jnp.floating) else t)(jnp.asarray(a)))
    def _A_setup():
        B, H, Sq, Sk, D, M = 1, 32, 2048, 2048, 128, 1024
        Dc = 4 * D
        return {
            "x": _w((lambda *s: _rng.normal(s) * 0.05)(B, Sq, M)),
            "c_kv": _w((lambda *s: _rng.normal(s) * 0.05)(B, Sk, Dc)),
            "w_q": _w((lambda *s: _rng.normal(s) * 0.05)(M, H, D) * (M ** -0.5)),
            "w_uk": _w((lambda *s: _rng.normal(s) * 0.05)(Dc, H, D) * (Dc ** -0.5)),
            "w_uv": _w((lambda *s: _rng.normal(s) * 0.05)(Dc, H, D) * (Dc ** -0.5)),
            "w_o": _w((lambda *s: _rng.normal(s) * 0.05)(H, D, M) * ((H * D) ** -0.5)),
        }
    _A_in = _A_setup()

    def _B_setup():
        B, S, D = 1, 2048, 1024
        return {
            "x": _w((lambda *s: _rng.normal(s) * 0.05)(B, S, D)),
            "wqkv": _w((lambda *s: _rng.normal(s) * 0.05)(D, 3 * D)),
            "wo": _w((lambda *s: _rng.normal(s) * 0.05)(D, D)),
        }
    _B_in = _B_setup()

    return {
        "A_x": _A_in["x"],
        "A_c_kv": _A_in["c_kv"],
        "A_w_q": _A_in["w_q"],
        "A_w_uk": _A_in["w_uk"],
        "A_w_uv": _A_in["w_uv"],
        "A_w_o": _A_in["w_o"],
        "B_x": _B_in["x"],
        "B_wqkv": _B_in["wqkv"],
        "B_wo": _B_in["wo"],
    }

def reference(A_x, A_c_kv, A_w_q, A_w_uk, A_w_uv, A_w_o, B_x, B_wqkv, B_wo):
    def _A_ref(x, c_kv, w_q, w_uk, w_uv, w_o):
        B, Sq, M = x.shape[0], x.shape[1], x.shape[2]
        Sk = c_kv.shape[1]
        H, D = w_q.shape[1], w_q.shape[2]
        q = jnp.einsum("bqm,mhd->bhqd", x, w_q)
        k = jnp.einsum("bkc,chd->bhkd", c_kv, w_uk)
        v = jnp.einsum("bkc,chd->bhkd", c_kv, w_uv)
        scores = jnp.einsum("bhqd,bhkd->bhqk", q, k) * (D ** -0.5)
        off = Sk - Sq
        qi = jnp.arange(Sq)[:, None]
        kj = jnp.arange(Sk)[None, :]
        cmask = kj <= (qi + off)
        scores = jnp.where(cmask[None, None], scores, -1e9)
        p = _softmax(scores, axis=-1)
        ctx = jnp.einsum("bhqk,bhkd->bhqd", p, v)
        return jnp.einsum("bhqd,hdm->bqm", ctx, w_o)

    def _B_ref(x, wqkv, wo):
        B, S, D = x.shape
        H = 32; Dh = D // H
        W, dil = 8, 2
        qkv = (lambda x, *d: x.transpose(*d))((x @ wqkv).reshape(B, S, 3, H, Dh), 2, 0, 3, 1, 4)
        q, k, v = qkv[0], qkv[1], qkv[2]
        scale = Dh ** -0.5
        pos = jnp.arange(S)
        off = jnp.arange(W) * dil
        idx = pos[:, None] - off[None, :]
        mask = idx >= 0
        idx_c = jnp.where(mask, idx, 0).reshape(-1)
        kg = k[:, :, idx_c, :].reshape(B, H, S, W, Dh)
        vg = v[:, :, idx_c, :].reshape(B, H, S, W, Dh)
        logits = jnp.einsum("bhsd,bhswd->bhsw", q, kg) * scale
        logits = jnp.where(mask[None, None, :, :], logits, -1e9)
        attn = _softmax(logits, axis=-1)
        o = jnp.einsum("bhsw,bhswd->bhsd", attn, vg)
        return (lambda x, *d: x.transpose(*d))(o, 0, 2, 1, 3).reshape(B, S, D) @ wo

    a = _A_ref(A_x, A_c_kv, A_w_q, A_w_uk, A_w_uv, A_w_o)
    b = _B_ref(B_x, B_wqkv, B_wo)
    return jnp.concatenate([a, b], axis=-1)
```

```python
import math

import jax
import jax.numpy as jnp
from jax import lax
import jax.experimental.pallas as pl
import jax.experimental.pallas.tpu as pltpu

BF16 = jnp.bfloat16
F32 = jnp.float32
U32 = jnp.uint32

T = 128
NEG = -1e9
LOG2E = math.log2(math.e)

S = 2048
M = 1024
H = 32
D = 128
DC = 512
BQ = 256
RO = 256
DB = 1024
HB = 32
DH = DB // HB
WIN = 8
DIL = 2
HALO = 16
RB = 256


def _dot(a, b):
    return lax.dot_general(a, b, (((1,), (0,)), ((), ())), preferred_element_type=F32)


def _dot_nt(a, b):
    return lax.dot_general(a, b, (((1,), (1,)), ((), ())), preferred_element_type=F32)


def _ld(ref, r0, r1):
    return pltpu.bitcast(ref[r0 // 2:r1 // 2, :], BF16)


def _st(ref, r0, r1, val):
    ref[r0 // 2:r1 // 2, :] = pltpu.bitcast(val.astype(BF16), U32)


def _kernel(x_hbm, c_hbm, wq_hbm, wuk_hbm, wuv_hbm, wo_hbm, bx_hbm, wqkv_hbm, bwo_hbm,
            out_hbm,
            x_v, c_v, wq_v, wuk_v, wuv_v, wo_v, bx_v, wqkv_v, bwo_v,
            wq_h, wkv_h, q_s, k_s, v_s, ctx_s, bq_s, bk_s, bv_s, ob_s, oa_s,
            in_sem, ob_sem, oa_sem):
    loads = [
        pltpu.make_async_copy(bx_hbm, bx_v, in_sem.at[0]),
        pltpu.make_async_copy(wqkv_hbm, wqkv_v, in_sem.at[1]),
        pltpu.make_async_copy(bwo_hbm, bwo_v, in_sem.at[2]),
        pltpu.make_async_copy(x_hbm, x_v, in_sem.at[3]),
        pltpu.make_async_copy(c_hbm, c_v, in_sem.at[4]),
        pltpu.make_async_copy(wq_hbm.bitcast(U32), wq_v, in_sem.at[5]),
        pltpu.make_async_copy(wuk_hbm.bitcast(U32), wuk_v, in_sem.at[6]),
        pltpu.make_async_copy(wuv_hbm.bitcast(U32), wuv_v, in_sem.at[7]),
        pltpu.make_async_copy(wo_hbm, wo_v, in_sem.at[8]),
    ]
    for cp in loads:
        cp.start()

    for cp in loads[:3]:
        cp.wait()
    nb = DB // T
    for j in range(nb):
        bk_s[j, 0:HALO, :] = jnp.zeros((HALO, T), F32)
        bv_s[j, 0:HALO, :] = jnp.zeros((HALO, T), F32)

    def ob_copy(i):
        r0 = pl.multiple_of(i * RB, RB)
        return pltpu.make_async_copy(
            ob_s.at[pl.ds(r0, RB), :], out_hbm.at[pl.ds(r0, RB), pl.ds(M, DB)], ob_sem.at[i])

    def b_chunk(i, carry):
        r0 = pl.multiple_of(i * RB, RB)
        xb = bx_v[pl.ds(r0, RB), :]
        qkv = _dot(xb, wqkv_v[...])
        for j in range(nb):
            bq_s[j] = qkv[:, j * T:(j + 1) * T] * (DH ** -0.5 * LOG2E)
            bk_s[j, HALO:, :] = qkv[:, DB + j * T:DB + (j + 1) * T]
            bv_s[j, HALO:, :] = qkv[:, 2 * DB + j * T:2 * DB + (j + 1) * T]
        seg = (lax.broadcasted_iota(jnp.int32, (T, T), 0) // DH
               == lax.broadcasted_iota(jnp.int32, (T, T), 1) // DH)
        ones = jnp.where(seg, 1.0, 0.0).astype(BF16)
        pos = r0 + lax.broadcasted_iota(jnp.int32, (RB, T), 0)
        outs = []
        for j in range(nb):
            q = bq_s[j]
            lg = []
            for w in range(WIN):
                kw = bk_s[j, pl.ds(HALO - DIL * w, RB), :]
                l = _dot((q * kw).astype(BF16), ones)
                if w:
                    l = jnp.where(pos >= DIL * w, l, NEG * LOG2E)
                lg.append(l)
            mx = lg[0]
            for l in lg[1:]:
                mx = jnp.maximum(mx, l)
            den = None
            acc = None
            for w in range(WIN):
                p = jnp.exp2(lg[w] - mx)
                pv = p * bv_s[j, pl.ds(HALO - DIL * w, RB), :]
                den = p if den is None else den + p
                acc = pv if acc is None else acc + pv
            outs.append((acc / den).astype(BF16))
        o = jnp.concatenate(outs, axis=1)
        ob_s[pl.ds(r0, RB), :] = _dot(o, bwo_v[...]).astype(BF16)
        for j in range(nb):
            bk_s[j, 0:HALO, :] = bk_s[j, RB:RB + HALO, :]
            bv_s[j, 0:HALO, :] = bv_s[j, RB:RB + HALO, :]
        ob_copy(i).start()
        return carry

    lax.fori_loop(0, S // RB, b_chunk, None)

    for cp in loads[3:8]:
        cp.wait()

    def head_weights(h):
        hp = h // 2
        sh = (16 * (1 - h % 2)).astype(U32)

        def pick(ref, rows):
            w = ref[pl.ds(hp, rows, stride=H // 2), :]
            return pltpu.bitcast((w << sh) & U32(0xFFFF0000), F32)

        _st(wq_h, 0, M, pick(wq_v, M))
        wkv = jnp.concatenate([pick(wuk_v, DC), pick(wuv_v, DC)], axis=1)
        _st(wkv_h, 0, DC, wkv)

    def project(r0, r1):
        q = _dot(x_v[r0:r1, :], _ld(wq_h, 0, M))
        _st(q_s, r0, r1, q * (D ** -0.5 * LOG2E))
        kv = _dot(c_v[r0:r1, :], _ld(wkv_h, 0, DC))
        _st(k_s, r0, r1, kv[:, :D])
        _st(v_s, r0, r1, kv[:, D:])

    n = BQ // T
    tri = (lax.broadcasted_iota(jnp.int32, (T, T), 1)
           <= lax.broadcasted_iota(jnp.int32, (T, T), 0))

    def scores(r0):
        tiles = [[] for _ in range(n)]
        if r0 > 0:
            sf = _dot_nt(_ld(q_s, r0, r0 + BQ), _ld(k_s, 0, r0))
            for i in range(n):
                tiles[i].append(sf[i * T:(i + 1) * T])
        for t in range(n):
            sd = _dot_nt(_ld(q_s, r0 + t * T, r0 + BQ), _ld(k_s, r0 + t * T, r0 + (t + 1) * T))
            for i in range(t, n):
                s = sd[(i - t) * T:(i - t + 1) * T]
                if i == t:
                    s = jnp.where(tri, s, NEG * LOG2E)
                tiles[i].append(s)
        return tiles

    def attend(h, r0, tiles):
        ps, ls = [], []
        for i in range(n):
            s = jnp.concatenate(tiles[i], axis=1) if len(tiles[i]) > 1 else tiles[i][0]
            p = jnp.exp2(s - jnp.max(s, axis=1, keepdims=True))
            ls.append(jnp.sum(p, axis=1, keepdims=True))
            ps.append(p.astype(BF16))
        acc = [None] * n
        if r0 > 0:
            pf = jnp.concatenate([p[:, :r0] for p in ps], axis=0) if n > 1 else ps[0][:, :r0]
            of = _dot(pf, _ld(v_s, 0, r0))
            for i in range(n):
                acc[i] = of[i * T:(i + 1) * T]
        for t in range(n):
            pd = [ps[i][:, r0 + t * T:r0 + (t + 1) * T] for i in range(t, n)]
            pd = jnp.concatenate(pd, axis=0) if len(pd) > 1 else pd[0]
            od = _dot(pd, _ld(v_s, r0 + t * T, r0 + (t + 1) * T))
            for i in range(t, n):
                o = od[(i - t) * T:(i - t + 1) * T]
                acc[i] = o if acc[i] is None else acc[i] + o
        for i in range(n):
            _st(ctx_s.at[h], r0 + i * T, r0 + (i + 1) * T, acc[i] * (1.0 / ls[i]))

    head_weights(jnp.int32(0))
    for r0 in range(0, S, BQ):
        project(r0, r0 + BQ)

    def head(h, with_next):
        if with_next:
            head_weights(h + 1)
        blocks = list(range(S - BQ, -1, -BQ))
        nxt = scores(blocks[0])
        for bi, r0 in enumerate(blocks):
            cur = nxt
            if bi + 1 < len(blocks):
                nxt = scores(blocks[bi + 1])
            attend(h, r0, cur)
            if with_next:
                project(r0, r0 + BQ)

    def head_body(h, carry):
        head(h, True)
        return carry

    lax.fori_loop(0, H - 1, head_body, None)
    head(H - 1, False)

    loads[8].wait()

    def oa_copy(i):
        r0 = pl.multiple_of(i * RO, RO)
        return pltpu.make_async_copy(
            oa_s.at[pl.ds(r0, RO), :], out_hbm.at[pl.ds(r0, RO), pl.ds(0, M)], oa_sem.at[i])

    def o_chunk(i, carry):
        r0 = pl.multiple_of(i * RO, RO)
        rw = pl.multiple_of(i * (RO // 2), RO // 2)
        ctx = jnp.concatenate(
            [pltpu.bitcast(ctx_s[h, pl.ds(rw, RO // 2), :], BF16) for h in range(H)], axis=1)
        oa_s[pl.ds(r0, RO), :] = _dot(ctx, wo_v[...]).astype(BF16)
        oa_copy(i).start()
        return carry

    lax.fori_loop(0, S // RO, o_chunk, None)
    for i in range(S // RB):
        ob_copy(i).wait()
    for i in range(S // RO):
        oa_copy(i).wait()


@jax.jit
def pallas_concat_heads__compressed_kv_cla__sliding_local_dilated__prompt_kernel(
    A_x: jax.Array,
    A_c_kv: jax.Array,
    A_w_q: jax.Array,
    A_w_uk: jax.Array,
    A_w_uv: jax.Array,
    A_w_o: jax.Array,
    B_x: jax.Array,
    B_wqkv: jax.Array,
    B_wo: jax.Array,
):
    scratch = [
        pltpu.VMEM((S, M), BF16),
        pltpu.VMEM((S, DC), BF16),
        pltpu.VMEM((M * H // 2, D), U32),
        pltpu.VMEM((DC * H // 2, D), U32),
        pltpu.VMEM((DC * H // 2, D), U32),
        pltpu.VMEM((H * D, M), BF16),
        pltpu.VMEM((S, DB), BF16),
        pltpu.VMEM((DB, 3 * DB), BF16),
        pltpu.VMEM((DB, DB), BF16),
        pltpu.VMEM((M // 2, D), U32),
        pltpu.VMEM((DC // 2, 2 * D), U32),
        pltpu.VMEM((S // 2, D), U32),
        pltpu.VMEM((S // 2, D), U32),
        pltpu.VMEM((S // 2, D), U32),
        pltpu.VMEM((H, S // 2, D), U32),
        pltpu.VMEM((DB // T, RB, T), F32),
        pltpu.VMEM((DB // T, RB + HALO, T), F32),
        pltpu.VMEM((DB // T, RB + HALO, T), F32),
        pltpu.VMEM((S, DB), BF16),
        pltpu.VMEM((S, M), BF16),
        pltpu.SemaphoreType.DMA((9,)),
        pltpu.SemaphoreType.DMA((S // RB,)),
        pltpu.SemaphoreType.DMA((S // RO,)),
    ]
    out = pl.pallas_call(
        _kernel,
        out_shape=jax.ShapeDtypeStruct((S, M + DB), BF16),
        in_specs=[pl.BlockSpec(memory_space=pl.ANY)] * 9,
        out_specs=pl.BlockSpec(memory_space=pl.ANY),
        scratch_shapes=scratch,
        compiler_params=pltpu.CompilerParams(vmem_limit_bytes=120 * 1024 * 1024),
        name="mla_local_concat",
    )(
        A_x.reshape(S, M),
        A_c_kv.reshape(S, DC),
        A_w_q.reshape(M * H, D),
        A_w_uk.reshape(DC * H, D),
        A_w_uv.reshape(DC * H, D),
        A_w_o.reshape(H * D, M),
        B_x.reshape(S, DB),
        B_wqkv,
        B_wo,
    )
    return out.reshape(1, S, M + DB)
```

```python
import functools
import math

import jax
import jax.numpy as jnp
from jax import lax
import jax.experimental.pallas as pl
import jax.experimental.pallas.tpu as pltpu

BF16 = jnp.bfloat16
F32 = jnp.float32
U32 = jnp.uint32
I32 = jnp.int32

T = 128
G = 16
LOG2E = math.log2(math.e)
NEG = -1e9 * LOG2E

S = 2048
M = 1024
H = 32
D = 128
DC = 512
EXP_TILES = 4
RO = 256
DB = 1024
DH = 32
NB = DB // T
WIN = 8
DIL = 2
HALO = 16
RB = 256


def _dot(a, b):
    return lax.dot_general(a, b, (((1,), (0,)), ((), ())), preferred_element_type=F32)


def _dot_nt(a, b):
    return lax.dot_general(a, b, (((1,), (1,)), ((), ())), preferred_element_type=F32)


def _ld(ref, r0, r1):
    return pltpu.bitcast(ref[r0 // 2:r1 // 2, :], BF16)


def _st(ref, r0, r1, val):
    ref[r0 // 2:r1 // 2, :] = pltpu.bitcast(val.astype(BF16), U32)


def _after(step, src, val):
    return jnp.where(jnp.broadcast_to(step, val.shape) < 0, src, val)


def _exchange(tiles):
    lane = lax.broadcasted_iota(I32, tiles[0].shape, 1)
    for bit in (1, 2, 4):
        pick = (lane & bit) != 0
        tiles = [jnp.where(pick, tiles[k ^ bit], tiles[k]) for k in range(NB)]
    return tiles


def _permute_lanes(tiles):
    lane = lax.broadcasted_iota(I32, (8, T), 1)
    base = ((lane >> 2) & 0x18) | ((lane << 2) & 0x60) | (lane & 7)
    return [
        jnp.concatenate(
            [jnp.take_along_axis(t[r:r + 8], base ^ k, axis=1) for r in range(0, t.shape[0], 8)],
            axis=0)
        for k, t in enumerate(tiles)
    ]


def _pack(y):
    w = pltpu.pack_elementwise([y[0:8], y[8:16]], packed_dtype=BF16)
    return [w[:, j * T:(j + 1) * T] for j in range(NB)]


def _shuffle(words):
    return [
        jnp.concatenate(
            [pltpu.unpack_elementwise(a, index=t, packed_dtype=BF16, unpacked_dtype=F32)
             for t in (0, 1)], axis=0)
        for a in _permute_lanes(_exchange(words))
    ]


def _unshuffle(tiles):
    return jnp.concatenate(_exchange(_permute_lanes(tiles)), axis=1)


def _kernel(x_hbm, c_hbm, wq_hbm, wuk_hbm, wuv_hbm, wo_hbm, bx_hbm, wqkv_hbm, bwo_hbm,
            out_hbm,
            x_v, c_v, wq_v, wuk_v, wuv_v, wo_v, bx_v, wqkv_v, bwo_v,
            wq_h, wkv_h, q_s, k_s, vc_s, bk_s, bv_s, ob_s, oa_s,
            in_sem, ob_sem, oa_sem):
    zero = pl.program_id(0)

    def cols(ref, c0, c1):
        return ref.at[:, pl.ds(c0, c1 - c0)]

    pairs = dict(
        bx0=(bx_hbm.at[pl.ds(0, RB)], bx_v.at[pl.ds(0, RB)]),
        wk=(cols(wqkv_hbm, DB, 2 * DB), cols(wqkv_v, DB, 2 * DB)),
        wq=(cols(wqkv_hbm, 0, DB), cols(wqkv_v, 0, DB)),
        wv=(cols(wqkv_hbm, 2 * DB, 3 * DB), cols(wqkv_v, 2 * DB, 3 * DB)),
        bwo=(bwo_hbm, bwo_v),
        bx1=(bx_hbm.at[pl.ds(RB, S - RB)], bx_v.at[pl.ds(RB, S - RB)]),
        x=(x_hbm, x_v),
        c=(c_hbm, c_v),
        awq=(wq_hbm.bitcast(U32), wq_v),
        awk=(wuk_hbm.bitcast(U32), wuk_v),
        awv=(wuv_hbm.bitcast(U32), wuv_v),
        awo=(wo_hbm, wo_v),
    )
    load = {name: pltpu.make_async_copy(src, dst, in_sem.at[n])
            for n, (name, (src, dst)) in enumerate(pairs.items())}

    for name in ("bx0", "wk", "wq"):
        load[name].start()

    for j in range(NB):
        bk_s[j, 0:HALO, :] = jnp.zeros((HALO, T), F32)
        bv_s[j, 0:HALO, :] = jnp.zeros((HALO, T), F32)

    def ob_copy(i):
        r0 = pl.multiple_of(i * RB, RB)
        return pltpu.make_async_copy(
            ob_s.at[pl.ds(r0, RB), :], out_hbm.at[pl.ds(r0, RB), pl.ds(M, DB)], ob_sem.at[i])

    def piece(src, col, row, rows=G):
        return src[row:row + rows, col * T:(col + 1) * T]

    def b_keys(p, k):
        for g in range(T // G):
            r = HALO + p + g * G
            for j, t in enumerate(_shuffle(_pack(k[g * G:(g + 1) * G]))):
                bk_s[j, r:r + G, :] = t

    def b_weights(step, p, q, src, first):
        attn = []
        for g in range(T // G):
            r = HALO + p + g * G
            words = _pack(q[g * G:(g + 1) * G])
            if g:
                gate = pltpu.bitcast(piece(src, g - 1, T - 8, 8), U32)
                words = [_after(step, gate, a) for a in words]
            qg = _shuffle(words)
            logits = [None] * WIN
            for j in range(NB):
                qj = _after(step, piece(src, g, j * G), qg[j])
                for w in range(WIN):
                    t = qj * bk_s[j, pl.ds(r - DIL * w, G), :]
                    logits[w] = t if logits[w] is None else logits[w] + t
            for w in range(WIN):
                t = logits[w] + pltpu.roll(logits[w], 64, 1)
                t = t + pltpu.roll(t, 32, 1)
                if first and p == 0 and g == 0 and w:
                    t = jnp.where(lax.broadcasted_iota(I32, (G, T), 0) >= DIL * w, t, NEG)
                logits[w] = t
            top = functools.reduce(jnp.maximum, logits)
            e = [jnp.exp2(t - top) for t in logits]
            inv = 1.0 / functools.reduce(jnp.add, e)
            attn.append([t * inv for t in e])
        return attn

    def b_mix(step, p, attn, v, src):
        out = []
        for g in range(T // G):
            r = HALO + p + g * G
            vg = _shuffle(_pack(v[g * G:(g + 1) * G]))
            for j in range(NB):
                bv_s[j, r:r + G, :] = vg[j]
            acc = [None] * NB
            for w in range(WIN):
                a = _after(step, piece(src, g - 1, w * G), attn[g][w]) if g else attn[g][w]
                for j in range(NB):
                    t = a * (bv_s[j, pl.ds(r - DIL * w, G), :] if w else vg[j])
                    acc[j] = t if acc[j] is None else acc[j] + t
            out.append(_unshuffle(acc))
        return jnp.concatenate(out, axis=0)

    def b_out(r, o):
        y = _dot(o.astype(BF16), bwo_v[...])
        ob_s[pl.ds(r, T), :] = y.astype(BF16)
        return y

    def b_finish(i):
        for j in range(NB):
            bk_s[j, 0:HALO, :] = bk_s[j, RB:RB + HALO, :]
            bv_s[j, 0:HALO, :] = bv_s[j, RB:RB + HALO, :]
        ob_copy(i).start()

    q_scale = DH ** -0.5 * LOG2E

    load["bx0"].wait()
    load["wk"].wait()
    load["wv"].start()
    xs = bx_v[0:RB, :]
    k = _dot(xs, wqkv_v[:, DB:2 * DB])
    b_keys(0, k[:T])
    b_keys(T, k[T:])
    load["wq"].wait()
    load["bwo"].start()
    q = _dot(xs, wqkv_v[:, 0:DB]) * q_scale
    load["wv"].wait()
    load["bx1"].start()
    v0 = _dot(xs[:T], wqkv_v[:, 2 * DB:])
    attn0 = b_weights(zero, 0, q[:T], v0, True)
    v1 = _dot(xs[T:], wqkv_v[:, 2 * DB:])
    attn1 = b_weights(zero, T, q[T:], v1, True)
    o0 = b_mix(zero, 0, attn0, v0, v1)
    load["bwo"].wait()
    for name in ("x", "c", "awq", "awk", "awv", "awo"):
        load[name].start()
    o1 = b_mix(zero, T, attn1, v1, b_out(0, o0))
    b_out(T, o1)
    b_finish(0)
    load["bx1"].wait()

    def b_chunk(i, carry):
        r0 = pl.multiple_of(i * RB, RB)
        pending = o = None
        for p in range(0, RB, T):
            xs = bx_v[pl.ds(r0 + p, T), :]
            k = _dot(xs, wqkv_v[:, DB:2 * DB])
            if pending is not None:
                o = b_mix(i, *pending, k)
                pending = None
            b_keys(p, k)
            q = _dot(xs, wqkv_v[:, 0:DB]) * q_scale
            v = _dot(xs, wqkv_v[:, 2 * DB:])
            attn = b_weights(i, p, q, v, False)
            if o is None:
                pending = (p, attn, v)
            else:
                o = b_mix(i, p, attn, v, b_out(r0 + p - T, o))
        b_out(r0 + RB - T, o)
        b_finish(i)
        return carry

    lax.fori_loop(1, S // RB, b_chunk, None)

    for name in ("x", "c", "awq", "awk", "awv"):
        load[name].wait()
    v_s = vc_s.at[H]
    nblk = S // T

    def head_weights(h, slot, part, parts):
        shift = (16 * (1 - h % 2)).astype(U32)

        def pick(ref, r0, r1):
            w = ref[pl.ds(h // 2 + r0 * (H // 2), r1 - r0, stride=H // 2), :]
            return pltpu.bitcast((w << shift) & U32(0xFFFF0000), F32)

        r0, r1 = part * M // parts, (part + 1) * M // parts
        _st(wq_h.at[slot], r0, r1, pick(wq_v, r0, r1))
        r0, r1 = part * DC // parts, (part + 1) * DC // parts
        _st(wkv_h.at[slot], r0, r1,
            jnp.concatenate([pick(wuk_v, r0, r1), pick(wuv_v, r0, r1)], axis=1))

    def project(slot, r0):
        q = _dot(x_v[r0:r0 + T, :], _ld(wq_h.at[slot], 0, M))
        _st(q_s, r0, r0 + T, q * (D ** -0.5 * LOG2E))
        wkv = _ld(wkv_h.at[slot], 0, DC)
        k = _dot(c_v[r0:r0 + T, :], wkv[:, :D])
        _st(k_s, r0, r0 + T, k)
        return q, k, _dot(c_v[r0:r0 + T, :], wkv[:, D:])

    def scores(r0):
        s = _dot_nt(_ld(q_s, r0, r0 + T), _ld(k_s, 0, r0 + T))
        s = [s[:, j:j + T] for j in range(0, r0 + T, T)]
        causal = (lax.broadcasted_iota(I32, (T, T), 1) <= lax.broadcasted_iota(I32, (T, T), 0))
        s[-1] = jnp.where(causal, s[-1], NEG)
        top = jnp.max(functools.reduce(jnp.maximum, s), axis=1, keepdims=True)
        return s, jnp.broadcast_to(top, (T, T))

    def attend(h, r0, s, top, gates):
        groups = min(-(-len(s) // EXP_TILES), len(gates) + 1)
        per = -(-len(s) // groups)
        tops = [top] + [_after(h, g, top) for g in gates[:groups - 1]]
        p = [jnp.exp2(t - tops[j // per]) for j, t in enumerate(s)]
        total = jnp.sum(functools.reduce(jnp.add, p), axis=1, keepdims=True)
        ctx = _dot(jnp.concatenate(p, axis=1).astype(BF16), _ld(v_s, 0, r0 + T))
        _st(vc_s.at[h], r0, r0 + T, ctx * (1.0 / total))

    head_weights(zero, 0, 0, 1)
    for n in range(nblk):
        head_weights(zero + 1, 1, n, nblk)
        _st(v_s, n * T, (n + 1) * T, project(0, n * T)[2])

    def head(h, carry):
        slot = (h + 1) % 2
        for n, r0 in enumerate(range(S - T, -1, -T)):
            s, top = scores(r0)
            head_weights(jnp.minimum(h + 2, H - 1), 1 - slot, n, nblk)
            qkv = project(slot, r0)
            attend(h, r0, s, top, qkv)
            _st(v_s, r0, r0 + T, qkv[2])
        return carry

    lax.fori_loop(0, H - 1, head, None)
    ahead = scores(S - T)
    for r0 in range(S - T, -1, -T):
        cur = ahead
        if r0:
            ahead = scores(r0 - T)
        attend(zero + (H - 1), r0, *cur, ())

    load["awo"].wait()

    def oa_copy(i):
        r0 = pl.multiple_of(i * RO, RO)
        return pltpu.make_async_copy(
            oa_s.at[pl.ds(r0, RO), :], out_hbm.at[pl.ds(r0, RO), pl.ds(0, M)], oa_sem.at[i])

    def o_chunk(i, carry):
        rw = pl.multiple_of(i * (RO // 2), RO // 2)
        ctx = jnp.concatenate(
            [pltpu.bitcast(vc_s[h, pl.ds(rw, RO // 2), :], BF16) for h in range(H)], axis=1)
        oa_s[pl.ds(pl.multiple_of(i * RO, RO), RO), :] = _dot(ctx, wo_v[...]).astype(BF16)
        oa_copy(i).start()
        return carry

    lax.fori_loop(0, S // RO, o_chunk, None)
    for i in range(S // RB):
        ob_copy(i).wait()
    for i in range(S // RO):
        oa_copy(i).wait()


@jax.jit
def pallas_concat_heads__compressed_kv_cla__sliding_local_dilated__prompt_kernel(
    A_x: jax.Array,
    A_c_kv: jax.Array,
    A_w_q: jax.Array,
    A_w_uk: jax.Array,
    A_w_uv: jax.Array,
    A_w_o: jax.Array,
    B_x: jax.Array,
    B_wqkv: jax.Array,
    B_wo: jax.Array,
):
    scratch = [
        pltpu.VMEM((S, M), BF16),
        pltpu.VMEM((S, DC), BF16),
        pltpu.VMEM((M * H // 2, D), U32),
        pltpu.VMEM((DC * H // 2, D), U32),
        pltpu.VMEM((DC * H // 2, D), U32),
        pltpu.VMEM((H * D, M), BF16),
        pltpu.VMEM((S, DB), BF16),
        pltpu.VMEM((DB, 3 * DB), BF16),
        pltpu.VMEM((DB, DB), BF16),
        pltpu.VMEM((2, M // 2, D), U32),
        pltpu.VMEM((2, DC // 2, 2 * D), U32),
        pltpu.VMEM((S // 2, D), U32),
        pltpu.VMEM((S // 2, D), U32),
        pltpu.VMEM((H + 1, S // 2, D), U32),
        pltpu.VMEM((NB, RB + HALO, T), F32),
        pltpu.VMEM((NB, RB + HALO, T), F32),
        pltpu.VMEM((S, DB), BF16),
        pltpu.VMEM((S, M), BF16),
        pltpu.SemaphoreType.DMA((12,)),
        pltpu.SemaphoreType.DMA((S // RB,)),
        pltpu.SemaphoreType.DMA((S // RO,)),
    ]
    out = pl.pallas_call(
        _kernel,
        grid=(1,),
        out_shape=jax.ShapeDtypeStruct((S, M + DB), BF16),
        in_specs=[pl.BlockSpec(memory_space=pl.ANY)] * 9,
        out_specs=pl.BlockSpec(memory_space=pl.ANY),
        scratch_shapes=scratch,
        compiler_params=pltpu.CompilerParams(vmem_limit_bytes=120 * 1024 * 1024),
        name="mla_local_concat",
    )(
        A_x.reshape(S, M),
        A_c_kv.reshape(S, DC),
        A_w_q.reshape(M * H, D),
        A_w_uk.reshape(DC * H, D),
        A_w_uv.reshape(DC * H, D),
        A_w_o.reshape(H * D, M),
        B_x.reshape(S, DB),
        B_wqkv,
        B_wo,
    )
    return out.reshape(1, S, M + DB)
```

```python
import functools
import math

import jax
import jax.numpy as jnp
from jax import lax
import jax.experimental.pallas as pl
import jax.experimental.pallas.tpu as pltpu

BF16 = jnp.bfloat16
F32 = jnp.float32
U32 = jnp.uint32
I32 = jnp.int32

T = 128
G = 16
LOG2E = math.log2(math.e)
NEG = -1e9 * LOG2E

S = 2048
M = 1024
H = 32
D = 128
DC = 512
EXP_TILES = 4
EARLY = 2
RO = 256
DB = 1024
DH = 32
NB = DB // T
WIN = 8
DIL = 2
HALO = 16
RB = 256


def _dot(a, b):
    return lax.dot_general(a, b, (((1,), (0,)), ((), ())), preferred_element_type=F32)


def _dot_nt(a, b):
    return lax.dot_general(a, b, (((1,), (1,)), ((), ())), preferred_element_type=F32)


def _ld(ref, r0, r1):
    return pltpu.bitcast(ref[r0 // 2:r1 // 2, :], BF16)


def _st(ref, r0, r1, val):
    ref[r0 // 2:r1 // 2, :] = pltpu.bitcast(val.astype(BF16), U32)


def _after(step, src, val):
    return jnp.where(jnp.broadcast_to(step, val.shape) < 0, src, val)


def _exchange(tiles):
    lane = lax.broadcasted_iota(I32, tiles[0].shape, 1)
    for bit in (1, 2, 4):
        pick = (lane & bit) != 0
        tiles = [jnp.where(pick, tiles[k ^ bit], tiles[k]) for k in range(NB)]
    return tiles


def _permute_lanes(tiles):
    lane = lax.broadcasted_iota(I32, (8, T), 1)
    base = ((lane >> 2) & 0x18) | ((lane << 2) & 0x60) | (lane & 7)
    return [
        jnp.concatenate(
            [jnp.take_along_axis(t[r:r + 8], base ^ k, axis=1) for r in range(0, t.shape[0], 8)],
            axis=0)
        for k, t in enumerate(tiles)
    ]


def _pack(y):
    w = pltpu.pack_elementwise([y[0:8], y[8:16]], packed_dtype=BF16)
    return [w[:, j * T:(j + 1) * T] for j in range(NB)]


def _shuffle(words):
    return [
        jnp.concatenate(
            [pltpu.unpack_elementwise(a, index=t, packed_dtype=BF16, unpacked_dtype=F32)
             for t in (0, 1)], axis=0)
        for a in _permute_lanes(_exchange(words))
    ]


def _unshuffle(tiles):
    return jnp.concatenate(_exchange(_permute_lanes(tiles)), axis=1)


def _kernel(x_hbm, c_hbm, wq_hbm, wuk_hbm, wuv_hbm, wo_hbm, bx_hbm, wqkv_hbm, bwo_hbm,
            out_hbm,
            x_v, c_v, wq_v, wuk_v, wuv_v, wo_v, bx_v, wqkv_v, bwo_v,
            wq_h, wuk_h, wuv_h, q_s, k_s, vc_s, bk_s, bv_s, part_s, ob_s, oa_s,
            in_sem, ob_sem, oa_sem):
    zero = pl.program_id(0)

    def block(src, dst, rows=slice(None), cols=slice(None)):
        return [(src.bitcast(U32).at[rows, cols], dst.at[rows, cols])]

    def head_pairs(src, dst):
        return [(src.bitcast(U32).at[:, hp, 0], dst.at[hp]) for hp in range(H // 2)]

    copies = dict(
        bx0=block(bx_hbm, bx_v, rows=pl.ds(0, RB // 2)),
        wk=block(wqkv_hbm, wqkv_v, cols=pl.ds(DB, DB)),
        wq=block(wqkv_hbm, wqkv_v, cols=pl.ds(0, DB)),
        wv=block(wqkv_hbm, wqkv_v, cols=pl.ds(2 * DB, DB)),
        bwo=block(bwo_hbm, bwo_v),
        bx1=block(bx_hbm, bx_v, rows=pl.ds(RB // 2, (S - RB) // 2)),
        a=(block(x_hbm, x_v) + block(c_hbm, c_v) + head_pairs(wq_hbm, wq_v)
           + head_pairs(wuk_hbm, wuk_v) + head_pairs(wuv_hbm, wuv_v)),
        awo=block(wo_hbm, wo_v),
    )
    copies = {name: [pltpu.make_async_copy(src, dst, in_sem.at[n]) for src, dst in group]
              for n, (name, group) in enumerate(copies.items())}

    def start(*names):
        for name in names:
            for cp in copies[name]:
                cp.start()

    def wait(*names):
        for name in names:
            for cp in copies[name]:
                cp.wait()

    start("bx0", "wk", "wq")

    for j in range(NB):
        bk_s[j, 0:HALO, :] = jnp.zeros((HALO, T), F32)
        bv_s[j, 0:HALO, :] = jnp.zeros((HALO, T), F32)

    def ob_copy(i):
        r0 = pl.multiple_of(i * RB, RB)
        return pltpu.make_async_copy(
            ob_s.at[pl.ds(r0, RB), :], out_hbm.at[pl.ds(r0, RB), pl.ds(M, DB)], ob_sem.at[i])

    def piece(src, col, row, rows=G):
        return src[row:row + rows, col * T:(col + 1) * T]

    def b_proj(xs, which):
        return _dot(xs, pltpu.bitcast(wqkv_v[:, which * DB:(which + 1) * DB], BF16))

    def b_keys(p, k):
        for g in range(T // G):
            r = HALO + p + g * G
            for j, t in enumerate(_shuffle(_pack(k[g * G:(g + 1) * G]))):
                bk_s[j, r:r + G, :] = t

    def b_weights(step, p, q, src, first):
        attn = []
        for g in range(T // G):
            r = HALO + p + g * G
            words = _pack(q[g * G:(g + 1) * G] * (DH ** -0.5 * LOG2E))
            if g:
                gate = pltpu.bitcast(piece(src, g - 1, T - 8, 8), U32)
                words = [_after(step, gate, a) for a in words]
            qg = _shuffle(words)
            logits = [None] * WIN
            for j in range(NB):
                qj = _after(step, piece(src, g, j * G), qg[j])
                for w in range(WIN):
                    t = qj * bk_s[j, pl.ds(r - DIL * w, G), :]
                    logits[w] = t if logits[w] is None else logits[w] + t
            for w in range(WIN):
                t = logits[w] + pltpu.roll(logits[w], 64, 1)
                t = t + pltpu.roll(t, 32, 1)
                if first and g == 0 and w:
                    t = jnp.where(lax.broadcasted_iota(I32, (G, T), 0) >= DIL * w, t, NEG)
                logits[w] = t
            top = functools.reduce(jnp.maximum, logits)
            e = [jnp.exp2(t - top) for t in logits]
            inv = 1.0 / functools.reduce(jnp.add, e)
            attn.append([t * inv for t in e])
        return attn

    def b_mix(step, p, attn, v, src):
        out = []
        for g in range(T // G):
            r = HALO + p + g * G
            vg = _shuffle(_pack(v[g * G:(g + 1) * G]))
            for j in range(NB):
                bv_s[j, r:r + G, :] = vg[j]
            acc = [None] * NB
            for w in range(WIN):
                a = _after(step, piece(src, g - 1, w * G), attn[g][w]) if g else attn[g][w]
                for j in range(NB):
                    t = a * (bv_s[j, pl.ds(r - DIL * w, G), :] if w else vg[j])
                    acc[j] = t if acc[j] is None else acc[j] + t
            out.append(_unshuffle(acc))
        return jnp.concatenate(out, axis=0)

    def b_out(r, o):
        y = _dot(o.astype(BF16), pltpu.bitcast(bwo_v[...], BF16))
        ob_s[pl.ds(r, T), :] = y.astype(BF16)
        return y

    def b_finish(i):
        for j in range(NB):
            bk_s[j, 0:HALO, :] = bk_s[j, RB:RB + HALO, :]
            bv_s[j, 0:HALO, :] = bv_s[j, RB:RB + HALO, :]
        ob_copy(i).start()

    wait("bx0", "wk")
    start("wv")
    k = b_proj(_ld(bx_v, 0, RB), 1)
    wait("wq")
    start("bwo", "bx1")
    b_keys(0, k[:T])
    q0 = b_proj(_ld(bx_v, 0, T), 0)
    b_keys(T, k[T:])
    wait("wv", "bwo")
    start("a", "awo")
    v0 = b_proj(_ld(bx_v, 0, T), 2)
    attn0 = b_weights(zero, 0, q0, v0, True)
    q1 = b_proj(_ld(bx_v, T, RB), 0)
    o0 = b_mix(zero, 0, attn0, v0, q1)
    v1 = b_proj(_ld(bx_v, T, RB), 2)
    attn1 = b_weights(zero, T, q1, v1, False)
    b_out(T, b_mix(zero, T, attn1, v1, b_out(0, o0)))
    b_finish(0)
    wait("bx1")

    def b_chunk(i, carry):
        r0 = pl.multiple_of(i * RB, RB)
        rw = pl.multiple_of(i * (RB // 2), RB // 2)
        pending = o = None
        for p in range(0, RB, T):
            xs = pltpu.bitcast(bx_v[pl.ds(rw + p // 2, T // 2), :], BF16)
            k = b_proj(xs, 1)
            if pending is not None:
                o = b_mix(i, *pending, k)
                pending = None
            b_keys(p, k)
            q = b_proj(xs, 0)
            v = b_proj(xs, 2)
            attn = b_weights(i, p, q, v, False)
            if o is None:
                pending = (p, attn, v)
            else:
                o = b_mix(i, p, attn, v, b_out(r0 + p - T, o))
        b_out(r0 + RB - T, o)
        b_finish(i)
        return carry

    lax.fori_loop(1, S // RB, b_chunk, None)

    wait("a", "awo")
    v_s = vc_s.at[H]
    nblk = S // T

    def head_weights(pair, odd, part, parts):
        for src, dst in ((wq_v, wq_h), (wuk_v, wuk_h), (wuv_v, wuv_h)):
            n = dst.shape[1] // parts
            lo = src[pair, pl.ds(2 * n * part, n, stride=2), :]
            hi = src[pair, pl.ds(2 * n * part + 1, n, stride=2), :]
            if odd:
                w = (lo >> 16) | (hi & U32(0xFFFF0000))
            else:
                w = (lo & U32(0xFFFF)) | (hi << 16)
            dst[odd, n * part:n * (part + 1), :] = w

    def project(odd, r0):
        q = _dot(_ld(x_v, r0, r0 + T), _ld(wq_h.at[odd], 0, M))
        _st(q_s, r0, r0 + T, q * (D ** -0.5 * LOG2E))
        k = _dot(_ld(c_v, r0, r0 + T), _ld(wuk_h.at[odd], 0, DC))
        _st(k_s, r0, r0 + T, k)
        return q, k, _dot(_ld(c_v, r0, r0 + T), _ld(wuv_h.at[odd], 0, DC))

    def scores(r0):
        s = _dot_nt(_ld(q_s, r0, r0 + T), _ld(k_s, 0, r0 + T))
        s = [s[:, j:j + T] for j in range(0, r0 + T, T)]
        causal = (lax.broadcasted_iota(I32, (T, T), 1) <= lax.broadcasted_iota(I32, (T, T), 0))
        s[-1] = jnp.where(causal, s[-1], NEG)
        top = jnp.max(functools.reduce(jnp.maximum, s), axis=1, keepdims=True)
        return s, jnp.broadcast_to(top, (T, T))

    def attend(h, r0, s, top, gates):
        groups = min(-(-len(s) // EXP_TILES), len(gates) + 1)
        per = -(-len(s) // groups)
        tops = [top] + [_after(h, g, top) for g in gates[:groups - 1]]
        p = [jnp.exp2(t - tops[j // per]) for j, t in enumerate(s)]
        total = jnp.sum(functools.reduce(jnp.add, p), axis=1, keepdims=True)
        ctx = _dot(jnp.concatenate(p, axis=1).astype(BF16), _ld(v_s, 0, r0 + T))
        _st(vc_s.at[h], r0, r0 + T, ctx * (1.0 / total))

    def head(h, odd, repack=True):
        for n, r0 in enumerate(range(S - T, -1, -T)):
            s, top = scores(r0)
            if repack:
                head_weights(h // 2 + 1, odd, n, nblk)
            qkv = project(1 - odd, r0)
            attend(h, r0, s, top, qkv)
            _st(v_s, r0, r0 + T, qkv[2])

    head_weights(0, 0, 0, 1)
    for n in range(nblk):
        head_weights(0, 1, n, nblk)
        _st(v_s, n * T, (n + 1) * T, project(0, n * T)[2])

    def head_pair(i, carry):
        head(2 * i, 0)
        head(2 * i + 1, 1)
        return carry

    lax.fori_loop(0, H // 2 - 1, head_pair, None)

    head(zero + (H - 2), 0, repack=False)
    for r0 in range(S - T, -1, -T):
        s, top = scores(r0)
        ctx = jnp.concatenate([_ld(vc_s.at[h], r0, r0 + T) for h in range(EARLY)], axis=1)
        part = _dot(ctx, _ld(wo_v, 0, EARLY * D))
        part_s[r0:r0 + T, :] = part
        attend(zero + (H - 1), r0, s, top, [part[:, c:c + T] for c in range(3 * T, M, 2 * T)])

    def oa_copy(i):
        r0 = pl.multiple_of(i * RO, RO)
        return pltpu.make_async_copy(
            oa_s.at[pl.ds(r0, RO), :], out_hbm.at[pl.ds(r0, RO), pl.ds(0, M)], oa_sem.at[i])

    def o_chunk(i, carry):
        rows = pl.ds(pl.multiple_of(i * RO, RO), RO)
        words = pl.ds(pl.multiple_of(i * (RO // 2), RO // 2), RO // 2)
        ctx = jnp.concatenate(
            [pltpu.bitcast(vc_s[h, words, :], BF16) for h in range(EARLY, H)], axis=1)
        oa_s[rows, :] = (part_s[rows, :] + _dot(ctx, _ld(wo_v, EARLY * D, H * D))).astype(BF16)
        oa_copy(i).start()
        return carry

    lax.fori_loop(0, S // RO, o_chunk, None)
    for i in range(S // RB):
        ob_copy(i).wait()
    for i in range(S // RO):
        oa_copy(i).wait()


@jax.jit
def pallas_concat_heads__compressed_kv_cla__sliding_local_dilated__prompt_kernel(
    A_x: jax.Array,
    A_c_kv: jax.Array,
    A_w_q: jax.Array,
    A_w_uk: jax.Array,
    A_w_uv: jax.Array,
    A_w_o: jax.Array,
    B_x: jax.Array,
    B_wqkv: jax.Array,
    B_wo: jax.Array,
):
    scratch = [
        pltpu.VMEM((S // 2, M), U32),
        pltpu.VMEM((S // 2, DC), U32),
        pltpu.VMEM((H // 2, M, D), U32),
        pltpu.VMEM((H // 2, DC, D), U32),
        pltpu.VMEM((H // 2, DC, D), U32),
        pltpu.VMEM((H * D // 2, M), U32),
        pltpu.VMEM((S // 2, DB), U32),
        pltpu.VMEM((DB // 2, 3 * DB), U32),
        pltpu.VMEM((DB // 2, DB), U32),
        pltpu.VMEM((2, M // 2, D), U32),
        pltpu.VMEM((2, DC // 2, D), U32),
        pltpu.VMEM((2, DC // 2, D), U32),
        pltpu.VMEM((S // 2, D), U32),
        pltpu.VMEM((S // 2, D), U32),
        pltpu.VMEM((H + 1, S // 2, D), U32),
        pltpu.VMEM((NB, RB + HALO, T), F32),
        pltpu.VMEM((NB, RB + HALO, T), F32),
        pltpu.VMEM((S, M), F32),
        pltpu.VMEM((S, DB), BF16),
        pltpu.VMEM((S, M), BF16),
        pltpu.SemaphoreType.DMA((8,)),
        pltpu.SemaphoreType.DMA((S // RB,)),
        pltpu.SemaphoreType.DMA((S // RO,)),
    ]
    out = pl.pallas_call(
        _kernel,
        grid=(1,),
        out_shape=jax.ShapeDtypeStruct((S, M + DB), BF16),
        in_specs=[pl.BlockSpec(memory_space=pl.ANY)] * 9,
        out_specs=pl.BlockSpec(memory_space=pl.ANY),
        scratch_shapes=scratch,
        compiler_params=pltpu.CompilerParams(vmem_limit_bytes=120 * 1024 * 1024),
        name="mla_local_concat",
    )(
        A_x.reshape(S, M),
        A_c_kv.reshape(S, DC),
        A_w_q.reshape(M, H // 2, 2, D),
        A_w_uk.reshape(DC, H // 2, 2, D),
        A_w_uv.reshape(DC, H // 2, 2, D),
        A_w_o.reshape(H * D, M),
        B_x.reshape(S, DB),
        B_wqkv,
        B_wo,
    )
    return out.reshape(1, S, M + DB)
```

```python
import functools
import math

import jax
import jax.numpy as jnp
from jax import lax
import jax.experimental.pallas as pl
import jax.experimental.pallas.tpu as pltpu

BF16 = jnp.bfloat16
F32 = jnp.float32
U32 = jnp.uint32
I32 = jnp.int32

T = 128
G = 16
LOG2E = math.log2(math.e)
NEG = -1e9 * LOG2E

S = 2048
M = 1024
H = 32
D = 128
DC = 512
EXP_TILES = 4
EARLY = 2
RO = 256
DB = 1024
DH = 32
NB = DB // T
WIN = 8
DIL = 2
HALO = 16
RA = 512
RB = 256


def _dot(a, b):
    return lax.dot_general(a, b, (((1,), (0,)), ((), ())), preferred_element_type=F32)


def _dot_nt(a, b):
    return lax.dot_general(a, b, (((1,), (1,)), ((), ())), preferred_element_type=F32)


def _ld(ref, r0, r1):
    return pltpu.bitcast(ref[r0 // 2:r1 // 2, :], BF16)


def _st(ref, r0, r1, val):
    ref[r0 // 2:r1 // 2, :] = pltpu.bitcast(val.astype(BF16), U32)


def _after(nonneg, src, val):
    return jnp.where(jnp.tile(nonneg, (val.shape[0] // 8, 1)) < 0, src, val)


def _exchange(tiles):
    lane = lax.broadcasted_iota(I32, tiles[0].shape, 1)
    for bit in (1, 2, 4):
        pick = (lane & bit) != 0
        tiles = [jnp.where(pick, tiles[k ^ bit], tiles[k]) for k in range(NB)]
    return tiles


def _permute_lanes(tiles):
    lane = lax.broadcasted_iota(I32, (8, T), 1)
    base = ((lane >> 2) & 0x18) | ((lane << 2) & 0x60) | (lane & 7)
    return [
        jnp.concatenate(
            [jnp.take_along_axis(t[r:r + 8], base ^ k, axis=1) for r in range(0, t.shape[0], 8)],
            axis=0)
        for k, t in enumerate(tiles)
    ]


def _pack(y):
    w = pltpu.pack_elementwise([y[0:8], y[8:16]], packed_dtype=BF16)
    return [w[:, j * T:(j + 1) * T] for j in range(NB)]


def _shuffle(words):
    return [
        jnp.concatenate(
            [pltpu.unpack_elementwise(a, index=t, packed_dtype=BF16, unpacked_dtype=F32)
             for t in (0, 1)], axis=0)
        for a in _permute_lanes(_exchange(words))
    ]


def _unshuffle(tiles):
    return jnp.concatenate(_exchange(_permute_lanes(tiles)), axis=1)


def _kernel(x_hbm, c_hbm, wq_hbm, wuk_hbm, wuv_hbm, wo_hbm, bx_hbm, wqkv_hbm, bwo_hbm,
            out_hbm,
            x_v, c_v, wq_v, wuk_v, wuv_v, wo_v, bx_v, wqkv_v, bwo_v,
            wq_h, wuk_h, wuv_h, q_s, k_s, vc_s, bk_s, bv_s, part_s, ob_s, oa_s,
            in_sem, ob_sem, oa_sem):
    def block(src, dst, rows=slice(None), cols=slice(None)):
        return [(src.bitcast(U32).at[rows, cols], dst.at[rows, cols])]

    def head_pairs(src, dst):
        return [(src.bitcast(U32).at[:, hp, 0], dst.at[hp]) for hp in range(H // 2)]

    half = RA // 2
    b_loads = dict(
        first=(block(bx_hbm, bx_v, rows=pl.ds(0, half // 2))
               + block(wqkv_hbm, wqkv_v, cols=pl.ds(DB, DB // 4))),
        bx0=block(bx_hbm, bx_v, rows=pl.ds(half // 2, half // 2)),
        wk1=block(wqkv_hbm, wqkv_v, cols=pl.ds(DB + DB // 4, DB // 4)),
        wk2=block(wqkv_hbm, wqkv_v, cols=pl.ds(DB + DB // 2, DB // 2)),
        wq=block(wqkv_hbm, wqkv_v, cols=pl.ds(0, DB)),
        wv=block(wqkv_hbm, wqkv_v, cols=pl.ds(2 * DB, DB)),
    )
    b_later = dict(
        bwo=block(bwo_hbm, bwo_v),
        bx1=block(bx_hbm, bx_v, rows=pl.ds(RA // 2, (S - RA) // 2)),
    )
    a_loads = dict(
        x=block(x_hbm, x_v) + block(c_hbm, c_v),
        awq=head_pairs(wq_hbm, wq_v),
        awkv=head_pairs(wuk_hbm, wuk_v) + head_pairs(wuv_hbm, wuv_v),
        awo=block(wo_hbm, wo_v),
    )
    copies = {name: [pltpu.make_async_copy(src, dst, in_sem.at[n]) for src, dst in group]
              for n, (name, group) in enumerate({**b_loads, **b_later, **a_loads}.items())}

    def start(*names):
        for name in names:
            for cp in copies[name]:
                cp.start()

    def wait(*names):
        for name in names:
            for cp in copies[name]:
                cp.wait()

    start(*b_loads)

    for j in range(NB):
        bk_s[j, 0:HALO, :] = jnp.zeros((HALO, T), F32)
        bv_s[j, 0:HALO, :] = jnp.zeros((HALO, T), F32)

    def ob_copy(r0, rows):
        return pltpu.make_async_copy(
            ob_s.at[pl.ds(r0, rows), :], out_hbm.at[pl.ds(r0, rows), pl.ds(M, DB)],
            ob_sem.at[r0 // RB])

    def nonneg():
        return pltpu.bitcast(bx_v[0:8, 0:T] >> 1, I32)

    def piece(src, col, row, rows=G):
        return src[row:row + rows, col * T:(col + 1) * T]

    def b_proj(xs, c0, width=DB):
        return _dot(xs, pltpu.bitcast(wqkv_v[:, c0:c0 + width], BF16))

    def b_keys(p, k, src=None):
        for g in range(T // G):
            r = HALO + p + g * G
            words = _pack(k[g * G:(g + 1) * G])
            if src is not None:
                gate = pltpu.bitcast(piece(src, NB - 1, g * G, 8), U32)
                words = [_after(nonneg(), gate, a) for a in words]
            for j, t in enumerate(_shuffle(words)):
                bk_s[j, r:r + G, :] = t

    def b_weights(p, q, src, first):
        attn = []
        for g in range(T // G):
            r = HALO + p + g * G
            words = _pack(q[g * G:(g + 1) * G] * (DH ** -0.5 * LOG2E))
            if g:
                gate = pltpu.bitcast(piece(src, g - 1, T - 8, 8), U32)
                words = [_after(nonneg(), gate, a) for a in words]
            qg = _shuffle(words)
            logits = [None] * WIN
            for j in range(NB):
                qj = _after(nonneg(), piece(src, g, j * G), qg[j])
                for w in range(WIN):
                    t = qj * bk_s[j, pl.ds(r - DIL * w, G), :]
                    logits[w] = t if logits[w] is None else logits[w] + t
            for w in range(WIN):
                t = logits[w] + pltpu.roll(logits[w], 64, 1)
                t = t + pltpu.roll(t, 32, 1)
                if first and g == 0 and w:
                    t = jnp.where(lax.broadcasted_iota(I32, (G, T), 0) >= DIL * w, t, NEG)
                logits[w] = t
            top = functools.reduce(jnp.maximum, logits)
            e = [jnp.exp2(t - top) for t in logits]
            inv = 1.0 / functools.reduce(jnp.add, e)
            attn.append([t * inv for t in e])
        return attn

    def b_mix(p, attn, v, src):
        out = []
        for g in range(T // G):
            r = HALO + p + g * G
            vg = _shuffle(_pack(v[g * G:(g + 1) * G]))
            for j in range(NB):
                bv_s[j, r:r + G, :] = vg[j]
            acc = [None] * NB
            for w in range(WIN):
                a = _after(nonneg(), piece(src, g - 1, w * G), attn[g][w]) if g else attn[g][w]
                for j in range(NB):
                    t = a * (bv_s[j, pl.ds(r - DIL * w, G), :] if w else vg[j])
                    acc[j] = t if acc[j] is None else acc[j] + t
            out.append(_unshuffle(acc))
        return jnp.concatenate(out, axis=0)

    def b_out(r, o):
        y = _dot(o.astype(BF16), pltpu.bitcast(bwo_v[...], BF16))
        ob_s[pl.ds(r, T), :] = y.astype(BF16)
        return y

    def b_finish(r0, rows):
        for j in range(NB):
            bk_s[j, 0:HALO, :] = bk_s[j, rows:rows + HALO, :]
            bv_s[j, 0:HALO, :] = bv_s[j, rows:rows + HALO, :]
        ob_copy(r0, rows).start()

    wait("first")
    k_top = b_proj(_ld(bx_v, 0, half), DB, DB // 4)
    wait("bx0")
    k = [jnp.concatenate([k_top, b_proj(_ld(bx_v, half, RA), DB, DB // 4)], axis=0)]
    wait("wk1")
    k.append(b_proj(_ld(bx_v, 0, RA), DB + DB // 4, DB // 4))
    wait("wk2")
    k.append(b_proj(_ld(bx_v, 0, RA), DB + DB // 2, DB // 2))
    k = jnp.concatenate(k, axis=1)
    wait("wq")
    start(*b_later)
    xs = [functools.partial(_ld, bx_v, p, p + T) for p in range(0, RA, T)]
    q = [b_proj(xs[0](), 0), b_proj(xs[1](), 0)]
    b_keys(0, k[:T])
    b_keys(T, k[T:2 * T], q[0])
    wait("wv")
    v = b_proj(xs[0](), 2 * DB)
    attn = b_weights(0, q[0], v, True)
    q.append(b_proj(xs[2](), 0))
    o = b_mix(0, attn, v, q[2])
    wait("bwo")
    for n in range(1, RA // T):
        if n + 2 < RA // T:
            q.append(b_proj(xs[n + 2](), 0))
            for u in range(n + 1, RA // T):
                b_keys(u * T, k[u * T:(u + 1) * T])
        v = b_proj(xs[n](), 2 * DB)
        attn = b_weights(n * T, q[n], v, False)
        o = b_mix(n * T, attn, v, b_out((n - 1) * T, o))
    b_out(RA - T, o)
    b_finish(0, RA)
    wait("bx1")

    def b_chunk(i, carry):
        r0 = pl.multiple_of(i * RB, RB)
        rw = pl.multiple_of(i * (RB // 2), RB // 2)
        pending = o = None
        for p in range(0, RB, T):
            xs = pltpu.bitcast(bx_v[pl.ds(rw + p // 2, T // 2), :], BF16)
            k = b_proj(xs, DB)
            if pending is not None:
                o = b_mix(*pending, k)
                pending = None
            b_keys(p, k)
            q = b_proj(xs, 0)
            v = b_proj(xs, 2 * DB)
            attn = b_weights(p, q, v, False)
            if o is None:
                pending = (p, attn, v)
            else:
                o = b_mix(p, attn, v, b_out(r0 + p - T, o))
        b_out(r0 + RB - T, o)
        b_finish(r0, RB)
        for n, name in enumerate(a_loads):
            pl.when(i == RA // RB + n)(functools.partial(start, name))
        return carry

    lax.fori_loop(RA // RB, S // RB, b_chunk, None)

    wait(*a_loads)
    v_s = vc_s.at[H]
    nblk = S // T

    def head_weights(pair, odd, part, parts):
        for src, dst in ((wq_v, wq_h), (wuk_v, wuk_h), (wuv_v, wuv_h)):
            n = dst.shape[1] // parts
            lo = src[pair, pl.ds(2 * n * part, n, stride=2), :]
            hi = src[pair, pl.ds(2 * n * part + 1, n, stride=2), :]
            if odd:
                w = (lo >> 16) | (hi & U32(0xFFFF0000))
            else:
                w = (lo & U32(0xFFFF)) | (hi << 16)
            dst[odd, n * part:n * (part + 1), :] = w

    def project(odd, r0):
        q = _dot(_ld(x_v, r0, r0 + T), _ld(wq_h.at[odd], 0, M))
        _st(q_s, r0, r0 + T, q * (D ** -0.5 * LOG2E))
        k = _dot(_ld(c_v, r0, r0 + T), _ld(wuk_h.at[odd], 0, DC))
        _st(k_s, r0, r0 + T, k)
        return q, k, _dot(_ld(c_v, r0, r0 + T), _ld(wuv_h.at[odd], 0, DC))

    def scores(r0):
        s = _dot_nt(_ld(q_s, r0, r0 + T), _ld(k_s, 0, r0 + T))
        s = [s[:, j:j + T] for j in range(0, r0 + T, T)]
        causal = (lax.broadcasted_iota(I32, (T, T), 1) <= lax.broadcasted_iota(I32, (T, T), 0))
        s[-1] = jnp.where(causal, s[-1], NEG)
        top = jnp.max(functools.reduce(jnp.maximum, s), axis=1, keepdims=True)
        return s, jnp.broadcast_to(top, (T, T))

    def attend(h, r0, s, top, gates):
        groups = min(-(-len(s) // EXP_TILES), len(gates) + 1)
        per = -(-len(s) // groups)
        tops = [top] + [_after(nonneg(), g, top) for g in gates[:groups - 1]]
        p = [jnp.exp2(t - tops[j // per]) for j, t in enumerate(s)]
        total = jnp.sum(functools.reduce(jnp.add, p), axis=1, keepdims=True)
        ctx = _dot(jnp.concatenate(p, axis=1).astype(BF16), _ld(v_s, 0, r0 + T))
        _st(vc_s.at[h], r0, r0 + T, ctx * (1.0 / total))

    def head(h, odd, repack=True):
        for n, r0 in enumerate(range(S - T, -1, -T)):
            s, top = scores(r0)
            if repack:
                head_weights(h // 2 + 1, odd, n, nblk)
            qkv = project(1 - odd, r0)
            attend(h, r0, s, top, qkv)
            _st(v_s, r0, r0 + T, qkv[2])

    head_weights(0, 0, 0, 1)
    for n in range(nblk):
        head_weights(0, 1, n, nblk)
        _st(v_s, n * T, (n + 1) * T, project(0, n * T)[2])

    def head_pair(i, carry):
        head(2 * i, 0)
        head(2 * i + 1, 1)
        return carry + 2

    last = lax.fori_loop(0, H // 2 - 1, head_pair, 1)

    head(last - 1, 0, repack=False)
    for r0 in range(S - T, -1, -T):
        s, top = scores(r0)
        ctx = jnp.concatenate([_ld(vc_s.at[h], r0, r0 + T) for h in range(EARLY)], axis=1)
        part = _dot(ctx, _ld(wo_v, 0, EARLY * D))
        part_s[r0:r0 + T, :] = part
        attend(last, r0, s, top, [part[:, c:c + T] for c in range(3 * T, M, 2 * T)])

    def oa_copy(i):
        r0 = pl.multiple_of(i * RO, RO)
        return pltpu.make_async_copy(
            oa_s.at[pl.ds(r0, RO), :], out_hbm.at[pl.ds(r0, RO), pl.ds(0, M)], oa_sem.at[i])

    def o_chunk(i, carry):
        rows = pl.ds(pl.multiple_of(i * RO, RO), RO)
        words = pl.ds(pl.multiple_of(i * (RO // 2), RO // 2), RO // 2)
        ctx = jnp.concatenate(
            [pltpu.bitcast(vc_s[h, words, :], BF16) for h in range(EARLY, H)], axis=1)
        oa_s[rows, :] = (part_s[rows, :] + _dot(ctx, _ld(wo_v, EARLY * D, H * D))).astype(BF16)
        oa_copy(i).start()
        return carry

    lax.fori_loop(0, S // RO, o_chunk, None)
    ob_copy(0, RA).wait()
    for r0 in range(RA, S, RB):
        ob_copy(r0, RB).wait()
    for i in range(S // RO):
        oa_copy(i).wait()


@jax.jit
def pallas_concat_heads__compressed_kv_cla__sliding_local_dilated__prompt_kernel(
    A_x: jax.Array,
    A_c_kv: jax.Array,
    A_w_q: jax.Array,
    A_w_uk: jax.Array,
    A_w_uv: jax.Array,
    A_w_o: jax.Array,
    B_x: jax.Array,
    B_wqkv: jax.Array,
    B_wo: jax.Array,
):
    scratch = [
        pltpu.VMEM((S // 2, M), U32),
        pltpu.VMEM((S // 2, DC), U32),
        pltpu.VMEM((H // 2, M, D), U32),
        pltpu.VMEM((H // 2, DC, D), U32),
        pltpu.VMEM((H // 2, DC, D), U32),
        pltpu.VMEM((H * D // 2, M), U32),
        pltpu.VMEM((S // 2, DB), U32),
        pltpu.VMEM((DB // 2, 3 * DB), U32),
        pltpu.VMEM((DB // 2, DB), U32),
        pltpu.VMEM((2, M // 2, D), U32),
        pltpu.VMEM((2, DC // 2, D), U32),
        pltpu.VMEM((2, DC // 2, D), U32),
        pltpu.VMEM((S // 2, D), U32),
        pltpu.VMEM((S // 2, D), U32),
        pltpu.VMEM((H + 1, S // 2, D), U32),
        pltpu.VMEM((NB, RA + HALO, T), F32),
        pltpu.VMEM((NB, RA + HALO, T), F32),
        pltpu.VMEM((S, M), F32),
        pltpu.VMEM((S, DB), BF16),
        pltpu.VMEM((S, M), BF16),
        pltpu.SemaphoreType.DMA((12,)),
        pltpu.SemaphoreType.DMA((S // RB,)),
        pltpu.SemaphoreType.DMA((S // RO,)),
    ]
    out = pl.pallas_call(
        _kernel,
        grid=(1,),
        out_shape=jax.ShapeDtypeStruct((S, M + DB), BF16),
        in_specs=[pl.BlockSpec(memory_space=pl.ANY)] * 9,
        out_specs=pl.BlockSpec(memory_space=pl.ANY),
        scratch_shapes=scratch,
        compiler_params=pltpu.CompilerParams(vmem_limit_bytes=120 * 1024 * 1024),
        name="mla_local_concat",
    )(
        A_x.reshape(S, M),
        A_c_kv.reshape(S, DC),
        A_w_q.reshape(M, H // 2, 2, D),
        A_w_uk.reshape(DC, H // 2, 2, D),
        A_w_uv.reshape(DC, H // 2, 2, D),
        A_w_o.reshape(H * D, M),
        B_x.reshape(S, DB),
        B_wqkv,
        B_wo,
    )
    return out.reshape(1, S, M + DB)
```

```python
import functools
import math

import jax
import jax.numpy as jnp
from jax import lax
import jax.experimental.pallas as pl
import jax.experimental.pallas.tpu as pltpu

BF16 = jnp.bfloat16
F32 = jnp.float32
U32 = jnp.uint32
I32 = jnp.int32

T = 128
G = 16
LOG2E = math.log2(math.e)
NEG = -1e9 * LOG2E

S = 2048
M = 1024
H = 32
D = 128
DC = 512
EXP_TILES = 4
EARLY = 2
RO = 256
DB = 1024
DH = 32
NB = DB // T
WIN = 8
DIL = 2
HALO = 16
RA = 512
RB = 256
RW = 32


def _dot(a, b):
    return lax.dot_general(a, b, (((1,), (0,)), ((), ())), preferred_element_type=F32)


def _dot_nt(a, b):
    return lax.dot_general(a, b, (((1,), (1,)), ((), ())), preferred_element_type=F32)


def _ld(ref, r0, r1):
    return pltpu.bitcast(ref[r0 // 2:r1 // 2, :], BF16)


def _st(ref, r0, r1, val):
    ref[r0 // 2:r1 // 2, :] = pltpu.bitcast(val.astype(BF16), U32)


def _after(nonneg, src, val):
    return jnp.where(jnp.tile(nonneg, (val.shape[0] // 8, 1)) < 0, src, val)


def _exchange(tiles):
    lane = lax.broadcasted_iota(I32, tiles[0].shape, 1)
    for bit in (1, 2, 4):
        pick = (lane & bit) != 0
        tiles = [jnp.where(pick, tiles[k ^ bit], tiles[k]) for k in range(NB)]
    return tiles


def _permute_lanes(tiles):
    lane = lax.broadcasted_iota(I32, (8, T), 1)
    base = ((lane >> 2) & 0x18) | ((lane << 2) & 0x60) | (lane & 7)
    return [
        jnp.concatenate(
            [jnp.take_along_axis(t[r:r + 8], base ^ k, axis=1) for r in range(0, t.shape[0], 8)],
            axis=0)
        for k, t in enumerate(tiles)
    ]


def _tiles(a):
    return [a[:, j * T:(j + 1) * T] for j in range(NB)]


def _shuffle(tiles):
    return _permute_lanes(_exchange(tiles))


def _shuffle_rows(y, hold=lambda words: words):
    words = hold(_tiles(pltpu.pack_elementwise([y[0:8], y[8:16]], packed_dtype=BF16)))
    return [
        jnp.concatenate(
            [pltpu.unpack_elementwise(a, index=t, packed_dtype=BF16, unpacked_dtype=F32)
             for t in (0, 1)], axis=0)
        for a in _shuffle(words)
    ]


def _unshuffle(tiles):
    return jnp.concatenate(_exchange(_permute_lanes(tiles)), axis=1)


def _kernel(x_hbm, c_hbm, wq_hbm, wuk_hbm, wuv_hbm, wo_hbm, bx_hbm, wqkv_hbm, bwo_hbm,
            out_hbm,
            x_v, c_v, wq_v, wuk_v, wuv_v, wo_v, bx_v, wqkv_v, bwo_v,
            wq_h, wuk_h, wuv_h, q_s, k_s, vc_s, wsh_s, bk_s, bv_s, part_s, ob_s, oa_s,
            in_sem, ob_sem, oa_sem):
    def block(src, dst, rows=slice(None), cols=slice(None)):
        return [(src.bitcast(U32).at[rows, cols], dst.at[rows, cols])]

    def head_pairs(src, dst):
        return [(src.bitcast(U32).at[:, hp, 0], dst.at[hp]) for hp in range(H // 2)]

    half = RA // 2
    b_loads = dict(
        first=(block(bx_hbm, bx_v, rows=pl.ds(0, half // 2))
               + block(wqkv_hbm, wqkv_v, cols=pl.ds(DB, DB // 4))),
        bx0=block(bx_hbm, bx_v, rows=pl.ds(half // 2, half // 2)),
        wk1=block(wqkv_hbm, wqkv_v, cols=pl.ds(DB + DB // 4, DB // 4)),
        wk2=block(wqkv_hbm, wqkv_v, cols=pl.ds(DB + DB // 2, DB // 2)),
        wq=block(wqkv_hbm, wqkv_v, cols=pl.ds(0, DB)),
        wv=block(wqkv_hbm, wqkv_v, cols=pl.ds(2 * DB, DB)),
    )
    b_later = dict(
        bwo=block(bwo_hbm, bwo_v),
        bx1=block(bx_hbm, bx_v, rows=pl.ds(RA // 2, (S - RA) // 2)),
    )
    a_loads = dict(
        x=block(x_hbm, x_v) + block(c_hbm, c_v),
        awq=head_pairs(wq_hbm, wq_v),
        awkv=head_pairs(wuk_hbm, wuk_v) + head_pairs(wuv_hbm, wuv_v),
        awo=block(wo_hbm, wo_v),
    )
    copies = {name: [pltpu.make_async_copy(src, dst, in_sem.at[n]) for src, dst in group]
              for n, (name, group) in enumerate({**b_loads, **b_later, **a_loads}.items())}

    def start(*names):
        for name in names:
            for cp in copies[name]:
                cp.start()

    def wait(*names):
        for name in names:
            for cp in copies[name]:
                cp.wait()

    start(*b_loads)

    for j in range(NB):
        bk_s[j, 0:HALO, :] = jnp.zeros((HALO, T), F32)
        bv_s[j, 0:HALO, :] = jnp.zeros((HALO, T), F32)

    def ob_copy(r0, rows):
        return pltpu.make_async_copy(
            ob_s.at[pl.ds(r0, rows), :], out_hbm.at[pl.ds(r0, rows), pl.ds(M, DB)],
            ob_sem.at[r0 // RB])

    def nonneg():
        return pltpu.bitcast(bx_v[0:8, 0:T] >> 1, I32)

    def piece(src, col, row, rows=G):
        return src[row:row + rows, col * T:(col + 1) * T]

    def hold(src, col, row):
        gate = pltpu.bitcast(piece(src, col, row, 8), U32)
        return lambda words: [
            _after(nonneg(), jnp.tile(gate, (a.shape[0] // 8, 1)), a) for a in words]

    def b_proj(xs, c0, width=DB, w_ref=wqkv_v):
        return _dot(xs, pltpu.bitcast(w_ref[:, c0:c0 + width], BF16))

    def b_shuffle_weights(c0, gates, r0=0):
        for n, gate in enumerate(gates):
            rows = slice(r0 + n * RW, r0 + (n + 1) * RW)
            for j, t in enumerate(_shuffle(gate(_tiles(wqkv_v[rows, c0:c0 + DB])))):
                wsh_s[rows, c0 + j * T:c0 + (j + 1) * T] = t

    def b_keys(p, k, raw, src=None):
        for g in range(T // G):
            r = HALO + p + g * G
            kg = k[g * G:(g + 1) * G]
            if not raw:
                kg = _tiles(kg)
            elif src is None:
                kg = _shuffle_rows(kg)
            else:
                kg = _shuffle_rows(kg, hold(src, NB - 1, g * G))
            for j in range(NB):
                bk_s[j, r:r + G, :] = kg[j]

    def b_weights(p, q, src, raw, first=False):
        attn = []
        for g in range(T // G):
            r = HALO + p + g * G
            qg = q[g * G:(g + 1) * G] * (DH ** -0.5 * LOG2E)
            if not raw:
                qg = _tiles(qg)
            elif g:
                qg = _shuffle_rows(qg, hold(src, g - 1, T - 8))
            else:
                qg = _shuffle_rows(qg)
            logits = [None] * WIN
            for j in range(NB):
                qj = _after(nonneg(), piece(src, g, j * G), qg[j])
                for w in range(WIN):
                    t = qj * bk_s[j, pl.ds(r - DIL * w, G), :]
                    logits[w] = t if logits[w] is None else logits[w] + t
            for w in range(WIN):
                t = logits[w] + pltpu.roll(logits[w], 64, 1)
                t = t + pltpu.roll(t, 32, 1)
                if first and g == 0 and w:
                    t = jnp.where(lax.broadcasted_iota(I32, (G, T), 0) >= DIL * w, t, NEG)
                logits[w] = t
            top = functools.reduce(jnp.maximum, logits)
            e = [jnp.exp2(t - top) for t in logits]
            inv = 1.0 / functools.reduce(jnp.add, e)
            attn.append([t * inv for t in e])
        return attn

    def b_mix(p, attn, v, src, raw):
        out = []
        for g in range(T // G):
            r = HALO + p + g * G
            vg = (_shuffle_rows if raw else _tiles)(v[g * G:(g + 1) * G])
            for j in range(NB):
                bv_s[j, r:r + G, :] = vg[j]
            acc = [None] * NB
            for w in range(WIN):
                a = _after(nonneg(), piece(src, g - 1, w * G), attn[g][w]) if g else attn[g][w]
                for j in range(NB):
                    t = a * (bv_s[j, pl.ds(r - DIL * w, G), :] if w else vg[j])
                    acc[j] = t if acc[j] is None else acc[j] + t
            out.append(_unshuffle(acc))
        return jnp.concatenate(out, axis=0)

    def b_out(r, o):
        y = _dot(o.astype(BF16), pltpu.bitcast(bwo_v[...], BF16))
        ob_s[pl.ds(r, T), :] = y.astype(BF16)
        return y

    def b_finish(r0, rows):
        for j in range(NB):
            bk_s[j, 0:HALO, :] = bk_s[j, rows:rows + HALO, :]
            bv_s[j, 0:HALO, :] = bv_s[j, rows:rows + HALO, :]
        ob_copy(r0, rows).start()

    wait("first")
    k_top = b_proj(_ld(bx_v, 0, half), DB, DB // 4)
    wait("bx0")
    k = [jnp.concatenate([k_top, b_proj(_ld(bx_v, half, RA), DB, DB // 4)], axis=0)]
    wait("wk1")
    k.append(b_proj(_ld(bx_v, 0, RA), DB + DB // 4, DB // 4))
    wait("wk2")
    k.append(b_proj(_ld(bx_v, 0, RA), DB + DB // 2, DB // 2))
    b_shuffle_weights(DB, [hold(k[-1], c, r) for c in range(NB // 2) for r in range(0, RA, T)])
    k = jnp.concatenate(k, axis=1)
    wait("wq")
    start(*b_later)
    xs = [functools.partial(_ld, bx_v, p, p + T) for p in range(0, RA, T)]
    q = [b_proj(xs[0](), 0), b_proj(xs[1](), 0)]
    b_keys(0, k[:T], True)
    b_keys(T, k[T:2 * T], True, q[0])
    b_shuffle_weights(0, [hold(q[0], c, 0) for c in range(3, NB)]
                      + [hold(q[1], c // 2, c % 2 * (T - G)) for c in range(11)])
    wait("wv")
    v = b_proj(xs[0](), 2 * DB)
    attn = b_weights(0, q[0], v, True, first=True)
    q.append(b_proj(xs[2](), 0))
    o = b_mix(0, attn, v, q[2], True)
    wait("bwo")
    q.append(b_proj(xs[3](), 0))
    b_keys(2 * T, k[2 * T:3 * T], True)
    b_keys(3 * T, k[3 * T:], True)
    b_shuffle_weights(2 * DB, [hold(q[3], c, 0) for c in range(3, 7)])
    for n in range(1, RA // T):
        v = b_proj(xs[n](), 2 * DB)
        attn = b_weights(n * T, q[n], v, True)
        o = b_mix(n * T, attn, v, b_out((n - 1) * T, o), True)
    y = b_out(RA - T, o)
    b_shuffle_weights(2 * DB, [hold(y, c // 2, c % 2 * (T - G)) for c in range(12)], 4 * RW)
    b_finish(0, RA)
    wait("bx1")

    def b_chunk(i, carry):
        r0 = pl.multiple_of(i * RB, RB)
        rw = pl.multiple_of(i * (RB // 2), RB // 2)
        pending = o = None
        for p in range(0, RB, T):
            xs = pltpu.bitcast(bx_v[pl.ds(rw + p // 2, T // 2), :], BF16)
            k = b_proj(xs, DB, w_ref=wsh_s)
            if pending is not None:
                o = b_mix(*pending, k, False)
                pending = None
            b_keys(p, k, False)
            q = b_proj(xs, 0, w_ref=wsh_s)
            v = b_proj(xs, 2 * DB, w_ref=wsh_s)
            attn = b_weights(p, q, v, False)
            if o is None:
                pending = (p, attn, v)
            else:
                o = b_mix(p, attn, v, b_out(r0 + p - T, o), False)
        b_out(r0 + RB - T, o)
        b_finish(r0, RB)
        for n, name in enumerate(a_loads):
            pl.when(i == RA // RB + n)(functools.partial(start, name))
        return carry

    lax.fori_loop(RA // RB, S // RB, b_chunk, None)

    wait(*a_loads)
    v_s = vc_s.at[H]
    nblk = S // T

    def head_weights(pair, odd, part, parts):
        for src, dst in ((wq_v, wq_h), (wuk_v, wuk_h), (wuv_v, wuv_h)):
            n = dst.shape[1] // parts
            lo = src[pair, pl.ds(2 * n * part, n, stride=2), :]
            hi = src[pair, pl.ds(2 * n * part + 1, n, stride=2), :]
            if odd:
                w = (lo >> 16) | (hi & U32(0xFFFF0000))
            else:
                w = (lo & U32(0xFFFF)) | (hi << 16)
            dst[odd, n * part:n * (part + 1), :] = w

    def project(odd, r0):
        q = _dot(_ld(x_v, r0, r0 + T), _ld(wq_h.at[odd], 0, M))
        _st(q_s, r0, r0 + T, q * (D ** -0.5 * LOG2E))
        k = _dot(_ld(c_v, r0, r0 + T), _ld(wuk_h.at[odd], 0, DC))
        _st(k_s, r0, r0 + T, k)
        return q, k, _dot(_ld(c_v, r0, r0 + T), _ld(wuv_h.at[odd], 0, DC))

    def scores(r0):
        s = _dot_nt(_ld(q_s, r0, r0 + T), _ld(k_s, 0, r0 + T))
        s = [s[:, j:j + T] for j in range(0, r0 + T, T)]
        causal = (lax.broadcasted_iota(I32, (T, T), 1) <= lax.broadcasted_iota(I32, (T, T), 0))
        s[-1] = jnp.where(causal, s[-1], NEG)
        top = jnp.max(functools.reduce(jnp.maximum, s), axis=1, keepdims=True)
        return s, jnp.broadcast_to(top, (T, T))

    def attend(h, r0, s, top, gates):
        groups = min(-(-len(s) // EXP_TILES), len(gates) + 1)
        per = -(-len(s) // groups)
        tops = [top] + [_after(nonneg(), g, top) for g in gates[:groups - 1]]
        p = [jnp.exp2(t - tops[j // per]) for j, t in enumerate(s)]
        total = jnp.sum(functools.reduce(jnp.add, p), axis=1, keepdims=True)
        ctx = _dot(jnp.concatenate(p, axis=1).astype(BF16), _ld(v_s, 0, r0 + T))
        _st(vc_s.at[h], r0, r0 + T, ctx * (1.0 / total))

    def head(h, odd, repack=True):
        for n, r0 in enumerate(range(S - T, -1, -T)):
            s, top = scores(r0)
            if repack:
                head_weights(h // 2 + 1, odd, n, nblk)
            qkv = project(1 - odd, r0)
            attend(h, r0, s, top, qkv)
            _st(v_s, r0, r0 + T, qkv[2])

    head_weights(0, 0, 0, 1)
    for n in range(nblk):
        head_weights(0, 1, n, nblk)
        _st(v_s, n * T, (n + 1) * T, project(0, n * T)[2])

    def head_pair(i, carry):
        head(2 * i, 0)
        head(2 * i + 1, 1)
        return carry + 2

    last = lax.fori_loop(0, H // 2 - 1, head_pair, 1)

    head(last - 1, 0, repack=False)
    for r0 in range(S - T, -1, -T):
        s, top = scores(r0)
        ctx = jnp.concatenate([_ld(vc_s.at[h], r0, r0 + T) for h in range(EARLY)], axis=1)
        part = _dot(ctx, _ld(wo_v, 0, EARLY * D))
        part_s[r0:r0 + T, :] = part
        attend(last, r0, s, top, [part[:, c:c + T] for c in range(3 * T, M, 2 * T)])

    def oa_copy(i):
        r0 = pl.multiple_of(i * RO, RO)
        return pltpu.make_async_copy(
            oa_s.at[pl.ds(r0, RO), :], out_hbm.at[pl.ds(r0, RO), pl.ds(0, M)], oa_sem.at[i])

    def o_chunk(i, carry):
        rows = pl.ds(pl.multiple_of(i * RO, RO), RO)
        words = pl.ds(pl.multiple_of(i * (RO // 2), RO // 2), RO // 2)
        ctx = jnp.concatenate(
            [pltpu.bitcast(vc_s[h, words, :], BF16) for h in range(EARLY, H)], axis=1)
        oa_s[rows, :] = (part_s[rows, :] + _dot(ctx, _ld(wo_v, EARLY * D, H * D))).astype(BF16)
        oa_copy(i).start()
        return carry

    lax.fori_loop(0, S // RO, o_chunk, None)
    ob_copy(0, RA).wait()
    for r0 in range(RA, S, RB):
        ob_copy(r0, RB).wait()
    for i in range(S // RO):
        oa_copy(i).wait()


@jax.jit
def pallas_concat_heads__compressed_kv_cla__sliding_local_dilated__prompt_kernel(
    A_x: jax.Array,
    A_c_kv: jax.Array,
    A_w_q: jax.Array,
    A_w_uk: jax.Array,
    A_w_uv: jax.Array,
    A_w_o: jax.Array,
    B_x: jax.Array,
    B_wqkv: jax.Array,
    B_wo: jax.Array,
):
    scratch = [
        pltpu.VMEM((S // 2, M), U32),
        pltpu.VMEM((S // 2, DC), U32),
        pltpu.VMEM((H // 2, M, D), U32),
        pltpu.VMEM((H // 2, DC, D), U32),
        pltpu.VMEM((H // 2, DC, D), U32),
        pltpu.VMEM((H * D // 2, M), U32),
        pltpu.VMEM((S // 2, DB), U32),
        pltpu.VMEM((DB // 2, 3 * DB), U32),
        pltpu.VMEM((DB // 2, DB), U32),
        pltpu.VMEM((2, M // 2, D), U32),
        pltpu.VMEM((2, DC // 2, D), U32),
        pltpu.VMEM((2, DC // 2, D), U32),
        pltpu.VMEM((S // 2, D), U32),
        pltpu.VMEM((S // 2, D), U32),
        pltpu.VMEM((H + 1, S // 2, D), U32),
        pltpu.VMEM((DB // 2, 3 * DB), U32),
        pltpu.VMEM((NB, RA + HALO, T), F32),
        pltpu.VMEM((NB, RA + HALO, T), F32),
        pltpu.VMEM((S, M), F32),
        pltpu.VMEM((S, DB), BF16),
        pltpu.VMEM((S, M), BF16),
        pltpu.SemaphoreType.DMA((12,)),
        pltpu.SemaphoreType.DMA((S // RB,)),
        pltpu.SemaphoreType.DMA((S // RO,)),
    ]
    out = pl.pallas_call(
        _kernel,
        grid=(1,),
        out_shape=jax.ShapeDtypeStruct((S, M + DB), BF16),
        in_specs=[pl.BlockSpec(memory_space=pl.ANY)] * 9,
        out_specs=pl.BlockSpec(memory_space=pl.ANY),
        scratch_shapes=scratch,
        compiler_params=pltpu.CompilerParams(vmem_limit_bytes=120 * 1024 * 1024),
        name="mla_local_concat",
    )(
        A_x.reshape(S, M),
        A_c_kv.reshape(S, DC),
        A_w_q.reshape(M, H // 2, 2, D),
        A_w_uk.reshape(DC, H // 2, 2, D),
        A_w_uv.reshape(DC, H // 2, 2, D),
        A_w_o.reshape(H * D, M),
        B_x.reshape(S, DB),
        B_wqkv,
        B_wo,
    )
    return out.reshape(1, S, M + DB)
```

```python
import functools
import math

import jax
import jax.numpy as jnp
from jax import lax
import jax.experimental.pallas as pl
import jax.experimental.pallas.tpu as pltpu

BF16 = jnp.bfloat16
F32 = jnp.float32
U32 = jnp.uint32
I32 = jnp.int32

T = 128
G = 16
LOG2E = math.log2(math.e)
NEG = -1e9 * LOG2E

S = 2048
M = 1024
H = 32
D = 128
DC = 512
PAIRS = H // 2
Q_SCALE = D ** -0.5 * LOG2E
CR = 512
XR = 512
EXP_TILES = 4
EARLY = 2
DB = 1024
DH = 32
NB = DB // T
WIN = 8
DIL = 2
HALO = 16
SLAB = DB // 2 // PAIRS
RC = 256


def _dot(a, b):
    return lax.dot_general(a, b, (((1,), (0,)), ((), ())), preferred_element_type=F32)


def _dot_nt(a, b):
    return lax.dot_general(a, b, (((1,), (1,)), ((), ())), preferred_element_type=F32)


def _ld(ref, r0, r1):
    return pltpu.bitcast(ref[r0 // 2:r1 // 2, :], BF16)


def _band(ref, n, size):
    return ref.at[pl.ds(pl.multiple_of(n * (size // 2), size // 2), size // 2)]


def _st(ref, r0, r1, val):
    ref[r0 // 2:r1 // 2, :] = pltpu.bitcast(val.astype(BF16), U32)


def _exchange(tiles):
    lane = lax.broadcasted_iota(I32, tiles[0].shape, 1)
    for bit in (1, 2, 4):
        pick = (lane & bit) != 0
        tiles = [jnp.where(pick, tiles[k ^ bit], tiles[k]) for k in range(NB)]
    return tiles


def _permute_lanes(tiles):
    lane = lax.broadcasted_iota(I32, (8, T), 1)
    base = ((lane >> 2) & 0x18) | ((lane << 2) & 0x60) | (lane & 7)
    return [
        jnp.concatenate(
            [jnp.take_along_axis(t[r:r + 8], base ^ k, axis=1) for r in range(0, t.shape[0], 8)],
            axis=0)
        for k, t in enumerate(tiles)
    ]


def _tiles(a):
    return [a[:, j * T:(j + 1) * T] for j in range(NB)]


def _shuffle(a):
    return _permute_lanes(_exchange(_tiles(a)))


def _unshuffle(tiles):
    return jnp.concatenate(_exchange(_permute_lanes(tiles)), axis=1)


def _kernel(x_hbm, c_hbm, wq_hbm, wuk_hbm, wuv_hbm, wo_hbm, bx_hbm, wqkv_hbm, bwo_hbm,
            out_hbm,
            x_v, c_v, wq_v, wuk_v, wuv_v, wo_v, bx_v, wqkv_v, bwo_v,
            wq_h, wuk_h, wuv_h, q_s, k_s, vc_s, part_s, wsh_s, bk_s, bv_s, out_s,
            c_sem, x_sem, in_sem, out_sem):

    def rows(src, dst, r0, n, sem):
        return pltpu.make_async_copy(
            src.bitcast(U32).at[pl.ds(r0, n)], dst.at[pl.ds(r0, n)], sem)

    def pair(src, dst, hp, sem):
        return pltpu.make_async_copy(src.bitcast(U32).at[:, hp, 0], dst.at[hp], sem)

    def head_pairs(p0, p1, sem):
        return [pair(src, dst, hp, sem) for hp in range(p0, p1)
                for src, dst in ((wq_hbm, wq_v), (wuk_hbm, wuk_v), (wuv_hbm, wuv_v))]

    def wqkv_slabs(i0, i1, sem):
        return [rows(wqkv_hbm, wqkv_v, i0 * SLAB, (i1 - i0) * SLAB, sem)]

    def start(copies):
        for cp in copies:
            cp.start()

    def wait(copies):
        for cp in copies:
            cp.wait()

    def c_copies(n):
        return [rows(c_hbm, c_v, pl.multiple_of(n * (CR // 2), CR // 2), CR // 2, c_sem.at[n])]

    def x_copies(n):
        return [rows(x_hbm, x_v, pl.multiple_of(n * (XR // 2), XR // 2), XR // 2, x_sem.at[n])]

    wkv_first = [pair(wuk_hbm, wuk_v, 0, in_sem.at[0]), pair(wuv_hbm, wuv_v, 0, in_sem.at[0])]
    wq_first = [pair(wq_hbm, wq_v, 0, in_sem.at[1])]
    step0 = head_pairs(1, 3, in_sem.at[2]) + wqkv_slabs(0, 1, in_sem.at[2])
    step1 = head_pairs(3, 6, in_sem.at[3]) + wqkv_slabs(1, 4, in_sem.at[3])
    step4 = head_pairs(6, PAIRS, in_sem.at[4]) + wqkv_slabs(4, PAIRS, in_sem.at[4])
    others = [rows(src, dst, 0, dst.shape[0], in_sem.at[5])
              for src, dst in ((wo_hbm, wo_v), (bx_hbm, bx_v), (bwo_hbm, bwo_v))]
    start(wkv_first)
    for n in range(S // CR):
        start(c_copies(n))
    start(wq_first)
    for n in range(S // XR):
        start(x_copies(n))
    start(step0 + step1 + step4 + others)

    def after(src, val):
        nonneg = pltpu.bitcast(c_v[0:8, 0:T] >> 1, I32)
        return jnp.where(jnp.tile(nonneg, (val.shape[0] // 8, 1)) < 0, src, val)

    nblk = S // T

    def repack(src, dst, hp, odd, part=0, parts=1):
        n = dst.shape[1] // parts
        lo = src[hp, pl.ds(2 * n * part, n, stride=2), :]
        hi = src[hp, pl.ds(2 * n * part + 1, n, stride=2), :]
        if odd:
            w = (lo >> 16) | (hi & U32(0xFFFF0000))
        else:
            w = (lo & U32(0xFFFF)) | (hi << 16)
        dst[odd, n * part:n * (part + 1), :] = w

    def repack_head(*args):
        for src, dst in ((wq_v, wq_h), (wuk_v, wuk_h), (wuv_v, wuv_h)):
            repack(src, dst, *args)

    def project_q(odd, r0, r1):
        q = _dot(_ld(x_v, r0, r1), _ld(wq_h.at[odd], 0, M))
        _st(q_s.at[odd], r0, r1, q * Q_SCALE)
        return q

    def project_kv(odd, r0, r1):
        k = _dot(_ld(c_v, r0, r1), _ld(wuk_h.at[odd], 0, DC))
        _st(k_s.at[odd], r0, r1, k)
        return k, _dot(_ld(c_v, r0, r1), _ld(wuv_h.at[odd], 0, DC))

    def scores(odd, r0):
        s = _dot_nt(_ld(q_s.at[odd], r0, r0 + T), _ld(k_s.at[odd], 0, r0 + T))
        s = [s[:, j:j + T] for j in range(0, r0 + T, T)]
        causal = (lax.broadcasted_iota(I32, (T, T), 1) <= lax.broadcasted_iota(I32, (T, T), 0))
        s[-1] = jnp.where(causal, s[-1], NEG)
        top = jnp.max(functools.reduce(jnp.maximum, s), axis=1, keepdims=True)
        return s, jnp.broadcast_to(top, (T, T))

    def attend(h, odd, r0, s, top, gates):
        groups = min(-(-len(s) // EXP_TILES), len(gates) + 1)
        per = -(-len(s) // groups)
        tops = [top] + [after(g, top) for g in gates[:groups - 1]]
        p = [jnp.exp2(t - tops[j // per]) for j, t in enumerate(s)]
        total = jnp.sum(functools.reduce(jnp.add, p), axis=1, keepdims=True)
        ctx = _dot(jnp.concatenate(p, axis=1).astype(BF16), _ld(vc_s.at[H + odd], 0, r0 + T))
        _st(vc_s.at[h], r0, r0 + T, ctx * (1.0 / total))

    def shuffle_weights(i, n, gate):
        per = SLAB // 8
        if n < 3 * per:
            r = pl.ds(pl.multiple_of(i * SLAB, 8) + n % per * 8, 8)
            c0 = n // per * DB
            gate = pltpu.bitcast(gate[0:8], U32)
            w = jnp.concatenate([after(gate, t) for t in _tiles(wqkv_v[r, c0:c0 + DB])], axis=1)
            for j, t in enumerate(_shuffle(w)):
                wsh_s[r, c0 + j * T:c0 + (j + 1) * T] = t

    def first_kv(n, carry):
        wait(c_copies(n))
        for odd in range(2):
            for w, dst in ((wuk_h, k_s.at[odd]), (wuv_h, vc_s.at[H + odd])):
                y = _dot(_ld(_band(c_v, n, CR), 0, CR), _ld(w.at[odd], 0, DC))
                _st(_band(dst, n, CR), 0, CR, y)
        return carry

    def first_q(n, carry):
        wait(x_copies(n))
        for odd in range(2):
            y = _dot(_ld(_band(x_v, n, XR), 0, XR), _ld(wq_h.at[odd], 0, M))
            _st(_band(q_s.at[odd], n, XR), 0, XR, y * Q_SCALE)
        return carry

    wait(wkv_first)
    for odd in range(2):
        repack(wuk_v, wuk_h, 0, odd)
        repack(wuv_v, wuv_h, 0, odd)
    lax.fori_loop(0, S // CR, first_kv, None)
    wait(wq_first)
    for odd in range(2):
        repack(wq_v, wq_h, 0, odd)
    lax.fori_loop(0, S // XR, first_q, None)
    wait(step0)
    repack_head(1, 0)

    def head_pair(i, carry):
        pl.when(i == 1)(lambda: wait(step1))
        pl.when(i == 4)(lambda: wait(step4))
        for odd in range(2):
            for n, r0 in enumerate(range(S - T, -1, -T)):
                s, top = scores(odd, r0)
                repack_head(jnp.minimum(i + 1 + odd, PAIRS - 1), 1 - odd, n, nblk)
                q = project_q(odd, r0, r0 + T)
                k, v = project_kv(odd, r0, r0 + T)
                attend(2 * i + odd, odd, r0, s, top, (q, k, v))
                _st(vc_s.at[H + odd], r0, r0 + T, v)
                if n >= nblk // 2:
                    shuffle_weights(i, odd * (nblk // 2) + n - nblk // 2, q)
        return carry

    lax.fori_loop(0, PAIRS - 1, head_pair, None)

    def last_head(odd, carry):
        for n, r0 in enumerate(range(S - T, -1, -T)):
            s, top = scores(odd, r0)
            ctx = jnp.concatenate(
                [_ld(vc_s.at[odd * EARLY + h], r0, r0 + T) for h in range(EARLY)], axis=1)
            part = _dot(ctx, _ld(_band(wo_v, odd, EARLY * D), 0, EARLY * D))
            part_s[odd, r0:r0 + T, :] = part
            attend(H - 2 + odd, odd, r0, s, top, _tiles(part)[3::2])
            if n >= nblk // 4:
                shuffle_weights(PAIRS - 1, n - nblk // 4, part[:, :T])
        return carry

    wait(others)
    lax.fori_loop(0, 2, last_head, None)

    for j in range(NB):
        bk_s[j, 0:HALO, :] = jnp.zeros((HALO, T), F32)
        bv_s[j, 0:HALO, :] = jnp.zeros((HALO, T), F32)

    def piece(src, col, row):
        return src[row:row + G, col * T:(col + 1) * T]

    def b_proj(xs, which):
        return _dot(xs, pltpu.bitcast(wsh_s[:, which * DB:(which + 1) * DB], BF16))

    def b_weights(pos, p, q, src):
        attn = []
        for g in range(T // G):
            r = HALO + p + g * G
            logits = [None] * WIN
            for j in range(NB):
                qj = after(piece(src, g, j * G), piece(q, j, g * G)) * (DH ** -0.5 * LOG2E)
                for w in range(WIN):
                    t = qj * bk_s[j, pl.ds(r - DIL * w, G), :]
                    logits[w] = t if logits[w] is None else logits[w] + t
            for w in range(WIN):
                t = logits[w] + pltpu.roll(logits[w], 64, 1)
                t = t + pltpu.roll(t, 32, 1)
                if p == 0 and g == 0 and w:
                    t = jnp.where(pos + lax.broadcasted_iota(I32, (G, T), 0) >= DIL * w, t, NEG)
                logits[w] = t
            top = functools.reduce(jnp.maximum, logits)
            e = [jnp.exp2(t - top) for t in logits]
            inv = 1.0 / functools.reduce(jnp.add, e)
            attn.append([t * inv for t in e])
        return attn

    def b_mix(p, attn, src):
        out = []
        for g in range(T // G):
            r = HALO + p + g * G
            acc = [None] * NB
            for w in range(WIN):
                a = after(piece(src, g, w * G), attn[g][w])
                for j in range(NB):
                    t = a * bv_s[j, pl.ds(r - DIL * w, G), :]
                    acc[j] = t if acc[j] is None else acc[j] + t
            out.append(_unshuffle(acc))
        return jnp.concatenate(out, axis=0)

    def out_copy(r0, branch):
        at = (pl.ds(r0, T), pl.ds(branch * M, M))
        return pltpu.make_async_copy(out_s.at[at], out_hbm.at[at], out_sem)

    def chunk(i, carry):
        r0 = pl.multiple_of(i * RC, RC)
        w0 = pl.multiple_of(i * (RC // 2), RC // 2)
        for p in range(0, RC, T):
            r = pl.ds(r0 + p, T)
            words = pl.ds(w0 + p // 2, T // 2)
            xs = pltpu.bitcast(bx_v[words, :], BF16)
            for j, t in enumerate(_tiles(b_proj(xs, 1))):
                bk_s[j, HALO + p:HALO + p + T, :] = t
            q = b_proj(xs, 0)
            v = b_proj(xs, 2)
            for j, t in enumerate(_tiles(v)):
                bv_s[j, HALO + p:HALO + p + T, :] = t
            attn = b_weights(r0, p, q, v)
            a = part_s[0, r, :] + part_s[1, r, :]
            o = None
            for h0, h1 in ((2 * EARLY, H // 2), (H // 2, H)):
                ctx = jnp.concatenate(
                    [pltpu.bitcast(vc_s[h, words, :], BF16) for h in range(h0, h1)], axis=1)
                y = _dot(ctx, _ld(wo_v, h0 * D, h1 * D))
                a = a + y
                if o is None:
                    o = b_mix(p, attn, y)
            out_s[r, 0:M] = a.astype(BF16)
            out_copy(r0 + p, 0).start()
            out_s[r, M:] = _dot(o.astype(BF16), _ld(bwo_v, 0, DB)).astype(BF16)
            out_copy(r0 + p, 1).start()
        for j in range(NB):
            bk_s[j, 0:HALO, :] = bk_s[j, RC:RC + HALO, :]
            bv_s[j, 0:HALO, :] = bv_s[j, RC:RC + HALO, :]
        return carry

    lax.fori_loop(0, S // RC, chunk, None)
    pltpu.make_async_copy(out_s, out_hbm, out_sem).wait()


@jax.jit
def pallas_concat_heads__compressed_kv_cla__sliding_local_dilated__prompt_kernel(
    A_x: jax.Array,
    A_c_kv: jax.Array,
    A_w_q: jax.Array,
    A_w_uk: jax.Array,
    A_w_uv: jax.Array,
    A_w_o: jax.Array,
    B_x: jax.Array,
    B_wqkv: jax.Array,
    B_wo: jax.Array,
):
    scratch = [
        pltpu.VMEM((S // 2, M), U32),
        pltpu.VMEM((S // 2, DC), U32),
        pltpu.VMEM((PAIRS, M, D), U32),
        pltpu.VMEM((PAIRS, DC, D), U32),
        pltpu.VMEM((PAIRS, DC, D), U32),
        pltpu.VMEM((H * D // 2, M), U32),
        pltpu.VMEM((S // 2, DB), U32),
        pltpu.VMEM((DB // 2, 3 * DB), U32),
        pltpu.VMEM((DB // 2, DB), U32),
        pltpu.VMEM((2, M // 2, D), U32),
        pltpu.VMEM((2, DC // 2, D), U32),
        pltpu.VMEM((2, DC // 2, D), U32),
        pltpu.VMEM((2, S // 2, D), U32),
        pltpu.VMEM((2, S // 2, D), U32),
        pltpu.VMEM((H + 2, S // 2, D), U32),
        pltpu.VMEM((2, S, M), F32),
        pltpu.VMEM((DB // 2, 3 * DB), U32),
        pltpu.VMEM((NB, RC + HALO, T), F32),
        pltpu.VMEM((NB, RC + HALO, T), F32),
        pltpu.VMEM((S, M + DB), BF16),
        pltpu.SemaphoreType.DMA((S // CR,)),
        pltpu.SemaphoreType.DMA((S // XR,)),
        pltpu.SemaphoreType.DMA((6,)),
        pltpu.SemaphoreType.DMA,
    ]
    out = pl.pallas_call(
        _kernel,
        out_shape=jax.ShapeDtypeStruct((S, M + DB), BF16),
        in_specs=[pl.BlockSpec(memory_space=pl.ANY)] * 9,
        out_specs=pl.BlockSpec(memory_space=pl.ANY),
        scratch_shapes=scratch,
        compiler_params=pltpu.CompilerParams(vmem_limit_bytes=120 * 1024 * 1024),
        name="mla_local_concat",
    )(
        A_x.reshape(S, M),
        A_c_kv.reshape(S, DC),
        A_w_q.reshape(M, PAIRS, 2, D),
        A_w_uk.reshape(DC, PAIRS, 2, D),
        A_w_uv.reshape(DC, PAIRS, 2, D),
        A_w_o.reshape(H * D, M),
        B_x.reshape(S, DB),
        B_wqkv,
        B_wo,
    )
    return out.reshape(1, S, M + DB)
```

```python
import functools
import math

import jax
import jax.numpy as jnp
from jax import lax
import jax.experimental.pallas as pl
import jax.experimental.pallas.tpu as pltpu

BF16 = jnp.bfloat16
F32 = jnp.float32
U32 = jnp.uint32
I32 = jnp.int32

T = 128
G = 16
LOG2E = math.log2(math.e)
NEG = -1e9 * LOG2E

S = 2048
M = 1024
H = 32
D = 128
DC = 512
PAIRS = H // 2
Q_SCALE = D ** -0.5 * LOG2E
CR = 512
XR = 512
EXP_TILES = 4
EARLY = 2
LATE = 8
DB = 1024
DH = 32
NB = DB // T
WIN = 8
DIL = 2
HALO = 16
RW = 32
RC = 256


def _dot(a, b):
    return lax.dot_general(a, b, (((1,), (0,)), ((), ())), preferred_element_type=F32)


def _dot_nt(a, b):
    return lax.dot_general(a, b, (((1,), (1,)), ((), ())), preferred_element_type=F32)


def _ld(ref, r0, r1):
    return pltpu.bitcast(ref[r0 // 2:r1 // 2, :], BF16)


def _band(ref, n, size):
    return ref.at[pl.ds(pl.multiple_of(n * (size // 2), size // 2), size // 2)]


def _st(ref, r0, r1, val):
    ref[r0 // 2:r1 // 2, :] = pltpu.bitcast(val.astype(BF16), U32)


def _exchange(tiles):
    lane = lax.broadcasted_iota(I32, tiles[0].shape, 1)
    for bit in (1, 2, 4):
        pick = (lane & bit) != 0
        tiles = [jnp.where(pick, tiles[k ^ bit], tiles[k]) for k in range(NB)]
    return tiles


def _permute_lanes(tiles):
    lane = lax.broadcasted_iota(I32, (8, T), 1)
    base = ((lane >> 2) & 0x18) | ((lane << 2) & 0x60) | (lane & 7)
    return [
        jnp.concatenate(
            [jnp.take_along_axis(t[r:r + 8], base ^ k, axis=1) for r in range(0, t.shape[0], 8)],
            axis=0)
        for k, t in enumerate(tiles)
    ]


def _tiles(a):
    return [a[:, j * T:(j + 1) * T] for j in range(NB)]


def _unshuffle(tiles):
    return jnp.concatenate(_exchange(_permute_lanes(tiles)), axis=1)


def _kernel(x_hbm, c_hbm, wq_hbm, wuk_hbm, wuv_hbm, wo_hbm, bx_hbm, wqkv_hbm, bwo_hbm,
            out_hbm,
            x_v, c_v, wq_v, wuk_v, wuv_v, wo_v, bx_v, wqkv_v, bwo_v,
            wq_h, wuk_h, wuv_h, q_s, k_s, vc_s, part_s, wsh_s, bk_s, bv_s, out_s,
            c_sem, x_sem, in_sem, out_sem):

    def rows(src, dst, r0, n, sem):
        return pltpu.make_async_copy(
            src.bitcast(U32).at[pl.ds(r0, n)], dst.at[pl.ds(r0, n)], sem)

    def pair(src, dst, hp, sem):
        return pltpu.make_async_copy(src.bitcast(U32).at[:, hp, 0], dst.at[hp], sem)

    def head_pairs(p0, p1, sem):
        return [pair(src, dst, hp, sem) for hp in range(p0, p1)
                for src, dst in ((wq_hbm, wq_v), (wuk_hbm, wuk_v), (wuv_hbm, wuv_v))]

    def start(copies):
        for cp in copies:
            cp.start()

    def wait(copies):
        for cp in copies:
            cp.wait()

    def c_copies(n):
        return [rows(c_hbm, c_v, pl.multiple_of(n * (CR // 2), CR // 2), CR // 2, c_sem.at[n])]

    def x_copies(n):
        return [rows(x_hbm, x_v, pl.multiple_of(n * (XR // 2), XR // 2), XR // 2, x_sem.at[n])]

    wkv_first = [pair(wuk_hbm, wuk_v, 0, in_sem.at[0]), pair(wuv_hbm, wuv_v, 0, in_sem.at[0])]
    wq_first = [pair(wq_hbm, wq_v, 0, in_sem.at[1])]
    step0 = head_pairs(1, 3, in_sem.at[2])
    step1 = head_pairs(3, 6, in_sem.at[3])
    step4 = head_pairs(6, PAIRS, in_sem.at[4])
    others = [rows(src, dst, 0, dst.shape[0], in_sem.at[5])
              for src, dst in ((wo_hbm, wo_v), (bx_hbm, bx_v), (wqkv_hbm, wqkv_v),
                               (bwo_hbm, bwo_v))]
    start(wkv_first)
    for n in range(S // CR):
        start(c_copies(n))
    start(wq_first)
    for n in range(S // XR):
        start(x_copies(n))
    start(step0 + step1 + step4 + others)

    def after(src, val):
        nonneg = pltpu.bitcast(c_v[0:8, 0:T] >> 1, I32)
        return jnp.where(jnp.tile(nonneg, (val.shape[0] // 8, 1)) < 0, src, val)

    nblk = S // T

    def repack(src, dst, hp, odd, part=0, parts=1):
        n = dst.shape[1] // parts
        lo = src[hp, pl.ds(2 * n * part, n, stride=2), :]
        hi = src[hp, pl.ds(2 * n * part + 1, n, stride=2), :]
        if odd:
            w = (lo >> 16) | (hi & U32(0xFFFF0000))
        else:
            w = (lo & U32(0xFFFF)) | (hi << 16)
        dst[odd, n * part:n * (part + 1), :] = w

    def repack_head(*args):
        for src, dst in ((wq_v, wq_h), (wuk_v, wuk_h), (wuv_v, wuv_h)):
            repack(src, dst, *args)

    def project_q(odd, r0, r1):
        q = _dot(_ld(x_v, r0, r1), _ld(wq_h.at[odd], 0, M))
        _st(q_s.at[odd], r0, r1, q * Q_SCALE)
        return q

    def project_kv(odd, r0, r1):
        k = _dot(_ld(c_v, r0, r1), _ld(wuk_h.at[odd], 0, DC))
        _st(k_s.at[odd], r0, r1, k)
        return k, _dot(_ld(c_v, r0, r1), _ld(wuv_h.at[odd], 0, DC))

    def scores(odd, r0):
        s = _dot_nt(_ld(q_s.at[odd], r0, r0 + T), _ld(k_s.at[odd], 0, r0 + T))
        s = [s[:, j:j + T] for j in range(0, r0 + T, T)]
        causal = (lax.broadcasted_iota(I32, (T, T), 1) <= lax.broadcasted_iota(I32, (T, T), 0))
        s[-1] = jnp.where(causal, s[-1], NEG)
        top = jnp.max(functools.reduce(jnp.maximum, s), axis=1, keepdims=True)
        return s, jnp.broadcast_to(top, (T, T))

    def attend(h, odd, r0, s, top, gates):
        groups = min(-(-len(s) // EXP_TILES), len(gates) + 1)
        per = -(-len(s) // groups)
        tops = [top] + [after(g, top) for g in gates[:groups - 1]]
        p = [jnp.exp2(t - tops[j // per]) for j, t in enumerate(s)]
        total = jnp.sum(functools.reduce(jnp.add, p), axis=1, keepdims=True)
        ctx = _dot(jnp.concatenate(p, axis=1).astype(BF16), _ld(vc_s.at[H + odd], 0, r0 + T))
        _st(vc_s.at[h], r0, r0 + T, ctx * (1.0 / total))

    def first_kv(n, carry):
        wait(c_copies(n))
        for odd in range(2):
            for w, dst in ((wuk_h, k_s.at[odd]), (wuv_h, vc_s.at[H + odd])):
                y = _dot(_ld(_band(c_v, n, CR), 0, CR), _ld(w.at[odd], 0, DC))
                _st(_band(dst, n, CR), 0, CR, y)
        return carry

    def first_q(n, carry):
        wait(x_copies(n))
        for odd in range(2):
            y = _dot(_ld(_band(x_v, n, XR), 0, XR), _ld(wq_h.at[odd], 0, M))
            _st(_band(q_s.at[odd], n, XR), 0, XR, y * Q_SCALE)
        return carry

    wait(wkv_first)
    for odd in range(2):
        repack(wuk_v, wuk_h, 0, odd)
        repack(wuv_v, wuv_h, 0, odd)
    lax.fori_loop(0, S // CR, first_kv, None)
    wait(wq_first)
    for odd in range(2):
        repack(wq_v, wq_h, 0, odd)
    lax.fori_loop(0, S // XR, first_q, None)
    wait(step0)
    repack_head(1, 0)

    def head_pair(i, carry):
        pl.when(i == 1)(lambda: wait(step1))
        pl.when(i == 4)(lambda: wait(step4))
        for odd in range(2):
            for n, r0 in enumerate(range(S - T, -1, -T)):
                s, top = scores(odd, r0)
                repack_head(jnp.minimum(i + 1 + odd, PAIRS - 1), 1 - odd, n, nblk)
                q = project_q(odd, r0, r0 + T)
                k, v = project_kv(odd, r0, r0 + T)
                attend(2 * i + odd, odd, r0, s, top, (q, k, v))
                _st(vc_s.at[H + odd], r0, r0 + T, v)
        return carry

    lax.fori_loop(0, PAIRS - 1, head_pair, None)

    def last_head(odd, carry):
        for n, r0 in enumerate(range(S - T, -1, -T)):
            s, top = scores(odd, r0)
            ctx = jnp.concatenate(
                [_ld(vc_s.at[odd * EARLY + h], r0, r0 + T) for h in range(EARLY)], axis=1)
            part = _dot(ctx, _ld(_band(wo_v, odd, EARLY * D), 0, EARLY * D))
            part_s[odd, r0:r0 + T, :] = part
            attend(H - 2 + odd, odd, r0, s, top, _tiles(part)[3::2])
        return carry

    wait(others)
    lax.fori_loop(0, 2, last_head, None)

    def shuffle_weights(i, carry):
        for n in range(nblk // 2):
            ctx = jnp.concatenate(
                [_ld(_band(vc_s.at[h], i, S // 2), n * T, (n + 1) * T)
                 for h in range(2 * EARLY, LATE)], axis=1)
            y = _dot(ctx, _ld(wo_v, 2 * EARLY * D, LATE * D))
            r = pl.ds(pl.multiple_of(i * (S // 2), S // 2) + n * T, T)
            part_s[0, r, :] += part_s[1, r, :] + y
            r = pl.ds(pl.multiple_of(i * (DB // 4), DB // 4) + n * RW, RW)
            for which, gate in enumerate(_tiles(y)[0:6:2]):
                gate = pltpu.bitcast(gate[0:RW], U32)
                w = [after(gate, t) for t in _tiles(wqkv_v[r, which * DB:(which + 1) * DB])]
                for j, t in enumerate(_permute_lanes(_exchange(w))):
                    wsh_s[r, which * DB + j * T:which * DB + (j + 1) * T] = t
        return carry

    lax.fori_loop(0, 2, shuffle_weights, None)

    for j in range(NB):
        bk_s[j, 0:HALO, :] = jnp.zeros((HALO, T), F32)
        bv_s[j, 0:HALO, :] = jnp.zeros((HALO, T), F32)

    def piece(src, col, row):
        return src[row:row + G, col * T:(col + 1) * T]

    def b_proj(xs, which):
        return _dot(xs, pltpu.bitcast(wsh_s[:, which * DB:(which + 1) * DB], BF16))

    def b_weights(pos, p, q, src):
        attn = []
        for g in range(T // G):
            r = HALO + p + g * G
            logits = [None] * WIN
            for j in range(NB):
                qj = after(piece(src, g, j * G), piece(q, j, g * G)) * (DH ** -0.5 * LOG2E)
                for w in range(WIN):
                    t = qj * bk_s[j, pl.ds(r - DIL * w, G), :]
                    logits[w] = t if logits[w] is None else logits[w] + t
            for w in range(WIN):
                t = logits[w] + pltpu.roll(logits[w], 64, 1)
                t = t + pltpu.roll(t, 32, 1)
                if p == 0 and g == 0 and w:
                    t = jnp.where(pos + lax.broadcasted_iota(I32, (G, T), 0) >= DIL * w, t, NEG)
                logits[w] = t
            top = functools.reduce(jnp.maximum, logits)
            e = [jnp.exp2(t - top) for t in logits]
            inv = 1.0 / functools.reduce(jnp.add, e)
            attn.append([t * inv for t in e])
        return attn

    def b_mix(p, attn, src):
        out = []
        for g in range(T // G):
            r = HALO + p + g * G
            acc = [None] * NB
            for w in range(WIN):
                a = after(piece(src, g, w * G), attn[g][w])
                for j in range(NB):
                    t = a * bv_s[j, pl.ds(r - DIL * w, G), :]
                    acc[j] = t if acc[j] is None else acc[j] + t
            out.append(_unshuffle(acc))
        return jnp.concatenate(out, axis=0)

    def out_copy(r0, branch):
        at = (pl.ds(r0, T), pl.ds(branch * M, M))
        return pltpu.make_async_copy(out_s.at[at], out_hbm.at[at], out_sem)

    def chunk(i, carry):
        r0 = pl.multiple_of(i * RC, RC)
        w0 = pl.multiple_of(i * (RC // 2), RC // 2)
        for p in range(0, RC, T):
            r = pl.ds(r0 + p, T)
            words = pl.ds(w0 + p // 2, T // 2)
            xs = pltpu.bitcast(bx_v[words, :], BF16)
            for j, t in enumerate(_tiles(b_proj(xs, 1))):
                bk_s[j, HALO + p:HALO + p + T, :] = t
            q = b_proj(xs, 0)
            v = b_proj(xs, 2)
            for j, t in enumerate(_tiles(v)):
                bv_s[j, HALO + p:HALO + p + T, :] = t
            attn = b_weights(r0, p, q, v)
            a = part_s[0, r, :]
            o = None
            for h0, h1 in ((LATE, (LATE + H) // 2), ((LATE + H) // 2, H)):
                ctx = jnp.concatenate(
                    [pltpu.bitcast(vc_s[h, words, :], BF16) for h in range(h0, h1)], axis=1)
                y = _dot(ctx, _ld(wo_v, h0 * D, h1 * D))
                a = a + y
                if o is None:
                    o = b_mix(p, attn, y)
            out_s[r, 0:M] = a.astype(BF16)
            out_copy(r0 + p, 0).start()
            out_s[r, M:] = _dot(o.astype(BF16), _ld(bwo_v, 0, DB)).astype(BF16)
            out_copy(r0 + p, 1).start()
        for j in range(NB):
            bk_s[j, 0:HALO, :] = bk_s[j, RC:RC + HALO, :]
            bv_s[j, 0:HALO, :] = bv_s[j, RC:RC + HALO, :]
        return carry

    lax.fori_loop(0, S // RC, chunk, None)
    pltpu.make_async_copy(out_s, out_hbm, out_sem).wait()


@jax.jit
def pallas_concat_heads__compressed_kv_cla__sliding_local_dilated__prompt_kernel(
    A_x: jax.Array,
    A_c_kv: jax.Array,
    A_w_q: jax.Array,
    A_w_uk: jax.Array,
    A_w_uv: jax.Array,
    A_w_o: jax.Array,
    B_x: jax.Array,
    B_wqkv: jax.Array,
    B_wo: jax.Array,
):
    scratch = [
        pltpu.VMEM((S // 2, M), U32),
        pltpu.VMEM((S // 2, DC), U32),
        pltpu.VMEM((PAIRS, M, D), U32),
        pltpu.VMEM((PAIRS, DC, D), U32),
        pltpu.VMEM((PAIRS, DC, D), U32),
        pltpu.VMEM((H * D // 2, M), U32),
        pltpu.VMEM((S // 2, DB), U32),
        pltpu.VMEM((DB // 2, 3 * DB), U32),
        pltpu.VMEM((DB // 2, DB), U32),
        pltpu.VMEM((2, M // 2, D), U32),
        pltpu.VMEM((2, DC // 2, D), U32),
        pltpu.VMEM((2, DC // 2, D), U32),
        pltpu.VMEM((2, S // 2, D), U32),
        pltpu.VMEM((2, S // 2, D), U32),
        pltpu.VMEM((H + 2, S // 2, D), U32),
        pltpu.VMEM((2, S, M), F32),
        pltpu.VMEM((DB // 2, 3 * DB), U32),
        pltpu.VMEM((NB, RC + HALO, T), F32),
        pltpu.VMEM((NB, RC + HALO, T), F32),
        pltpu.VMEM((S, M + DB), BF16),
        pltpu.SemaphoreType.DMA((S // CR,)),
        pltpu.SemaphoreType.DMA((S // XR,)),
        pltpu.SemaphoreType.DMA((6,)),
        pltpu.SemaphoreType.DMA,
    ]
    out = pl.pallas_call(
        _kernel,
        out_shape=jax.ShapeDtypeStruct((S, M + DB), BF16),
        in_specs=[pl.BlockSpec(memory_space=pl.ANY)] * 9,
        out_specs=pl.BlockSpec(memory_space=pl.ANY),
        scratch_shapes=scratch,
        compiler_params=pltpu.CompilerParams(vmem_limit_bytes=120 * 1024 * 1024),
        name="mla_local_concat",
    )(
        A_x.reshape(S, M),
        A_c_kv.reshape(S, DC),
        A_w_q.reshape(M, PAIRS, 2, D),
        A_w_uk.reshape(DC, PAIRS, 2, D),
        A_w_uv.reshape(DC, PAIRS, 2, D),
        A_w_o.reshape(H * D, M),
        B_x.reshape(S, DB),
        B_wqkv,
        B_wo,
    )
    return out.reshape(1, S, M + DB)
```

```python
import functools
import math

import jax
import jax.numpy as jnp
from jax import lax
import jax.experimental.pallas as pl
import jax.experimental.pallas.tpu as pltpu

BF16 = jnp.bfloat16
F32 = jnp.float32
U32 = jnp.uint32
I32 = jnp.int32

T = 128
G = 16
LOG2E = math.log2(math.e)
NEG = -1e9 * LOG2E

S = 2048
M = 1024
H = 32
D = 128
DC = 512
PAIRS = H // 2
Q_SCALE = D ** -0.5 * LOG2E
CR = 512
XR = 512
EXP_TILES = 4
EARLY = 2
LATE = 8
DB = 1024
DH = 32
NB = DB // T
WIN = 8
DIL = 2
HALO = 16
RW = 32
RC = 256


def _dot(a, b):
    return lax.dot_general(a, b, (((1,), (0,)), ((), ())), preferred_element_type=F32)


def _dot_nt(a, b):
    return lax.dot_general(a, b, (((1,), (1,)), ((), ())), preferred_element_type=F32)


def _ld(ref, r0, r1):
    return pltpu.bitcast(ref[r0 // 2:r1 // 2, :], BF16)


def _band(ref, n, size):
    return ref.at[pl.ds(pl.multiple_of(n * (size // 2), size // 2), size // 2)]


def _st(ref, r0, r1, val):
    ref[r0 // 2:r1 // 2, :] = pltpu.bitcast(val.astype(BF16), U32)


def _exchange(tiles):
    lane = lax.broadcasted_iota(I32, tiles[0].shape, 1)
    for bit in (1, 2, 4):
        pick = (lane & bit) != 0
        tiles = [jnp.where(pick, tiles[k ^ bit], tiles[k]) for k in range(NB)]
    return tiles


def _permute_lanes(tiles):
    lane = lax.broadcasted_iota(I32, (8, T), 1)
    base = ((lane >> 2) & 0x18) | ((lane << 2) & 0x60) | (lane & 7)
    return [
        jnp.concatenate(
            [jnp.take_along_axis(t[r:r + 8], base ^ k, axis=1) for r in range(0, t.shape[0], 8)],
            axis=0)
        for k, t in enumerate(tiles)
    ]


def _tiles(a):
    return [a[:, j * T:(j + 1) * T] for j in range(NB)]


def _unshuffle(tiles):
    return jnp.concatenate(_exchange(_permute_lanes(tiles)), axis=1)


def _kernel(x_hbm, c_hbm, wq_hbm, wuk_hbm, wuv_hbm, wo_hbm, bx_hbm, wqkv_hbm, bwo_hbm,
            out_hbm,
            x_v, c_v, wq_v, wuk_v, wuv_v, wo_v, bx_v, wqkv_v, bwo_v,
            wq_h, wuk_h, wuv_h, q_s, k_s, vc_s, part_s, wsh_s, bk_s, bv_s, out_s,
            c_sem, x_sem, in_sem, out_sem):

    def rows(src, dst, r0, n, sem):
        return pltpu.make_async_copy(
            src.bitcast(U32).at[pl.ds(r0, n)], dst.at[pl.ds(r0, n)], sem)

    def pair(src, dst, hp, sem):
        return pltpu.make_async_copy(src.bitcast(U32).at[:, hp, 0], dst.at[hp], sem)

    def head_pairs(p0, p1, sem):
        return [pair(src, dst, hp, sem) for hp in range(p0, p1)
                for src, dst in ((wq_hbm, wq_v), (wuk_hbm, wuk_v), (wuv_hbm, wuv_v))]

    def start(copies):
        for cp in copies:
            cp.start()

    def wait(copies):
        for cp in copies:
            cp.wait()

    def c_copies(n):
        return [rows(c_hbm, c_v, pl.multiple_of(n * (CR // 2), CR // 2), CR // 2, c_sem.at[n])]

    def x_copies(n):
        return [rows(x_hbm, x_v, pl.multiple_of(n * (XR // 2), XR // 2), XR // 2, x_sem.at[n])]

    wkv_first = [pair(wuk_hbm, wuk_v, 0, in_sem.at[0]), pair(wuv_hbm, wuv_v, 0, in_sem.at[0])]
    wq_first = [pair(wq_hbm, wq_v, 0, in_sem.at[1])]
    step0 = head_pairs(1, 3, in_sem.at[2])
    step1 = head_pairs(3, 6, in_sem.at[3])
    step4 = head_pairs(6, PAIRS, in_sem.at[4])
    others = [rows(src, dst, 0, dst.shape[0], in_sem.at[5])
              for src, dst in ((wo_hbm, wo_v), (bx_hbm, bx_v), (wqkv_hbm, wqkv_v),
                               (bwo_hbm, bwo_v))]
    start(wkv_first)
    for n in range(S // CR):
        start(c_copies(n))
    start(wq_first)
    for n in range(S // XR):
        start(x_copies(n))
    start(step0 + step1 + step4 + others)

    def after(src, val):
        nonneg = pltpu.bitcast(c_v[0:8, 0:T] >> 1, I32)
        return jnp.where(jnp.tile(nonneg, (val.shape[0] // 8, 1)) < 0, src, val)

    nblk = S // T

    def repack(src, dst, hp, odd, part=0, parts=1):
        n = dst.shape[1] // parts
        lo = src[hp, pl.ds(2 * n * part, n, stride=2), :]
        hi = src[hp, pl.ds(2 * n * part + 1, n, stride=2), :]
        if odd:
            w = (lo >> 16) | (hi & U32(0xFFFF0000))
        else:
            w = (lo & U32(0xFFFF)) | (hi << 16)
        dst[odd, n * part:n * (part + 1), :] = w

    def repack_head(*args):
        for src, dst in ((wq_v, wq_h), (wuk_v, wuk_h), (wuv_v, wuv_h)):
            repack(src, dst, *args)

    def project_q(odd, r0, r1):
        q = _dot(_ld(x_v, r0, r1), _ld(wq_h.at[odd], 0, M))
        _st(q_s.at[odd], r0, r1, q * Q_SCALE)
        return q

    def project_k(odd, r0, r1):
        k = _dot(_ld(c_v, r0, r1), _ld(wuk_h.at[odd], 0, DC))
        _st(k_s.at[odd], r0, r1, k)
        return k

    def project_v(odd, r0, r1):
        return _dot(_ld(c_v, r0, r1), _ld(wuv_h.at[odd], 0, DC))

    def scores(odd, r0):
        s = _dot_nt(_ld(q_s.at[odd], r0, r0 + T), _ld(k_s.at[odd], 0, r0 + T))
        s = [s[:, j:j + T] for j in range(0, r0 + T, T)]
        causal = (lax.broadcasted_iota(I32, (T, T), 1) <= lax.broadcasted_iota(I32, (T, T), 0))
        s[-1] = jnp.where(causal, s[-1], NEG)
        top = jnp.max(functools.reduce(jnp.maximum, s), axis=1, keepdims=True)
        return s, jnp.broadcast_to(top, (T, T))

    def attend(h, odd, r0, s, top, gates):
        groups = min(-(-len(s) // EXP_TILES), len(gates) + 1)
        per = -(-len(s) // groups)
        tops = [top] + [after(g, top) for g in gates[:groups - 1]]
        p = [jnp.exp2(t - tops[j // per]) for j, t in enumerate(s)]
        total = jnp.sum(functools.reduce(jnp.add, p), axis=1, keepdims=True)
        ctx = _dot(jnp.concatenate(p, axis=1).astype(BF16), _ld(vc_s.at[H + odd], 0, r0 + T))
        _st(vc_s.at[h], r0, r0 + T, ctx * (1.0 / total))

    def first_kv(n, carry):
        wait(c_copies(n))
        for odd in range(2):
            for w, dst in ((wuk_h, k_s.at[odd]), (wuv_h, vc_s.at[H + odd])):
                y = _dot(_ld(_band(c_v, n, CR), 0, CR), _ld(w.at[odd], 0, DC))
                _st(_band(dst, n, CR), 0, CR, y)
        return carry

    def first_q(n, carry):
        wait(x_copies(n))
        for odd in range(2):
            y = _dot(_ld(_band(x_v, n, XR), 0, XR), _ld(wq_h.at[odd], 0, M))
            _st(_band(q_s.at[odd], n, XR), 0, XR, y * Q_SCALE)
        return carry

    wait(wkv_first)
    for odd in range(2):
        repack(wuk_v, wuk_h, 0, odd)
        repack(wuv_v, wuv_h, 0, odd)
    lax.fori_loop(0, S // CR, first_kv, None)
    wait(wq_first)
    for odd in range(2):
        repack(wq_v, wq_h, 0, odd)
    lax.fori_loop(0, S // XR, first_q, None)
    wait(step0)
    repack_head(1, 0)

    def head_pair(i, carry):
        pl.when(i == 1)(lambda: wait(step1))
        pl.when(i == 4)(lambda: wait(step4))
        for odd in range(2):
            for n, r0 in enumerate(range(S - T, -1, -T)):
                v = project_v(odd, r0, r0 + T) if (odd, n) == (0, 0) else None
                s, top = scores(odd, r0)
                repack_head(jnp.minimum(i + 1 + odd, PAIRS - 1), 1 - odd, n, nblk)
                gates = [project_q(odd, r0, r0 + T), project_k(odd, r0, r0 + T)]
                if v is None and (odd, r0) != (1, 0):
                    v = project_v(odd, r0, r0 + T)
                    gates.append(v)
                attend(2 * i + odd, odd, r0, s, top, gates)
                if v is None:
                    v = project_v(odd, r0, r0 + T)
                _st(vc_s.at[H + odd], r0, r0 + T, v)
        return carry

    lax.fori_loop(0, PAIRS - 1, head_pair, None)

    def last_head(odd, carry):
        def early(r0):
            return jnp.concatenate(
                [_ld(vc_s.at[odd * EARLY + h], r0, r0 + T) for h in range(EARLY)], axis=1)

        ctx = early(S - T)
        for r0 in range(S - T, -1, -T):
            s, top = scores(odd, r0)
            part = _dot(ctx, _ld(_band(wo_v, odd, EARLY * D), 0, EARLY * D))
            part_s[odd, r0:r0 + T, :] = part
            if r0:
                ctx = early(r0 - T)
            attend(H - 2 + odd, odd, r0, s, top, _tiles(part)[3::2])
        return carry

    wait(others)
    lax.fori_loop(0, 2, last_head, None)

    def shuffle_weights(i, carry):
        for n in range(nblk // 2):
            ctx = jnp.concatenate(
                [_ld(_band(vc_s.at[h], i, S // 2), n * T, (n + 1) * T)
                 for h in range(2 * EARLY, LATE)], axis=1)
            y = _dot(ctx, _ld(wo_v, 2 * EARLY * D, LATE * D))
            r = pl.ds(pl.multiple_of(i * (S // 2), S // 2) + n * T, T)
            part_s[0, r, :] += part_s[1, r, :] + y
            r = pl.ds(pl.multiple_of(i * (DB // 4), DB // 4) + n * RW, RW)
            for which, gate in enumerate(_tiles(y)[0:6:2]):
                gate = pltpu.bitcast(gate[0:RW], U32)
                w = [after(gate, t) for t in _tiles(wqkv_v[r, which * DB:(which + 1) * DB])]
                for j, t in enumerate(_permute_lanes(_exchange(w))):
                    wsh_s[r, which * DB + j * T:which * DB + (j + 1) * T] = t
        return carry

    lax.fori_loop(0, 2, shuffle_weights, None)

    for j in range(NB):
        bk_s[j, 0:HALO, :] = jnp.zeros((HALO, T), F32)
        bv_s[j, 0:HALO, :] = jnp.zeros((HALO, T), F32)

    def piece(src, col, row):
        return src[row:row + G, col * T:(col + 1) * T]

    def b_proj(xs, which):
        return _dot(xs, pltpu.bitcast(wsh_s[:, which * DB:(which + 1) * DB], BF16))

    def b_weights(pos, p, q, src):
        attn = []
        for g in range(T // G):
            r = HALO + p + g * G
            logits = [None] * WIN
            for j in range(NB):
                qj = after(piece(src, g, j * G), piece(q, j, g * G)) * (DH ** -0.5 * LOG2E)
                for w in range(WIN):
                    t = qj * bk_s[j, pl.ds(r - DIL * w, G), :]
                    logits[w] = t if logits[w] is None else logits[w] + t
            for w in range(WIN):
                t = logits[w] + pltpu.roll(logits[w], 64, 1)
                t = t + pltpu.roll(t, 32, 1)
                if p == 0 and g == 0 and w:
                    t = jnp.where(pos + lax.broadcasted_iota(I32, (G, T), 0) >= DIL * w, t, NEG)
                logits[w] = t
            top = functools.reduce(jnp.maximum, logits)
            e = [jnp.exp2(t - top) for t in logits]
            inv = 1.0 / functools.reduce(jnp.add, e)
            attn.append([t * inv for t in e])
        return attn

    def b_mix(p, attn, src):
        out = []
        for g in range(T // G):
            r = HALO + p + g * G
            acc = [None] * NB
            for w in range(WIN):
                a = after(piece(src, g, w * G), attn[g][w])
                for j in range(NB):
                    t = a * bv_s[j, pl.ds(r - DIL * w, G), :]
                    acc[j] = t if acc[j] is None else acc[j] + t
            out.append(_unshuffle(acc))
        return jnp.concatenate(out, axis=0)

    def out_copy(r0, branch):
        at = (pl.ds(r0, T), pl.ds(branch * M, M))
        return pltpu.make_async_copy(out_s.at[at], out_hbm.at[at], out_sem)

    def chunk(i, carry):
        r0 = pl.multiple_of(i * RC, RC)
        w0 = pl.multiple_of(i * (RC // 2), RC // 2)
        for p in range(0, RC, T):
            r = pl.ds(r0 + p, T)
            words = pl.ds(w0 + p // 2, T // 2)
            xs = pltpu.bitcast(bx_v[words, :], BF16)
            for j, t in enumerate(_tiles(b_proj(xs, 1))):
                bk_s[j, HALO + p:HALO + p + T, :] = t
            q = b_proj(xs, 0)
            v = b_proj(xs, 2)
            for j, t in enumerate(_tiles(v)):
                bv_s[j, HALO + p:HALO + p + T, :] = t
            attn = b_weights(r0, p, q, v)
            a = part_s[0, r, :]
            o = None
            for h0, h1 in ((LATE, (LATE + H) // 2), ((LATE + H) // 2, H)):
                ctx = jnp.concatenate(
                    [pltpu.bitcast(vc_s[h, words, :], BF16) for h in range(h0, h1)], axis=1)
                y = _dot(ctx, _ld(wo_v, h0 * D, h1 * D))
                a = a + y
                if o is None:
                    o = b_mix(p, attn, y)
            out_s[r, 0:M] = a.astype(BF16)
            out_copy(r0 + p, 0).start()
            out_s[r, M:] = _dot(o.astype(BF16), _ld(bwo_v, 0, DB)).astype(BF16)
            out_copy(r0 + p, 1).start()
        for j in range(NB):
            bk_s[j, 0:HALO, :] = bk_s[j, RC:RC + HALO, :]
            bv_s[j, 0:HALO, :] = bv_s[j, RC:RC + HALO, :]
        return carry

    lax.fori_loop(0, S // RC, chunk, None)
    pltpu.make_async_copy(out_s, out_hbm, out_sem).wait()


@jax.jit
def pallas_concat_heads__compressed_kv_cla__sliding_local_dilated__prompt_kernel(
    A_x: jax.Array,
    A_c_kv: jax.Array,
    A_w_q: jax.Array,
    A_w_uk: jax.Array,
    A_w_uv: jax.Array,
    A_w_o: jax.Array,
    B_x: jax.Array,
    B_wqkv: jax.Array,
    B_wo: jax.Array,
):
    scratch = [
        pltpu.VMEM((S // 2, M), U32),
        pltpu.VMEM((S // 2, DC), U32),
        pltpu.VMEM((PAIRS, M, D), U32),
        pltpu.VMEM((PAIRS, DC, D), U32),
        pltpu.VMEM((PAIRS, DC, D), U32),
        pltpu.VMEM((H * D // 2, M), U32),
        pltpu.VMEM((S // 2, DB), U32),
        pltpu.VMEM((DB // 2, 3 * DB), U32),
        pltpu.VMEM((DB // 2, DB), U32),
        pltpu.VMEM((2, M // 2, D), U32),
        pltpu.VMEM((2, DC // 2, D), U32),
        pltpu.VMEM((2, DC // 2, D), U32),
        pltpu.VMEM((2, S // 2, D), U32),
        pltpu.VMEM((2, S // 2, D), U32),
        pltpu.VMEM((H + 2, S // 2, D), U32),
        pltpu.VMEM((2, S, M), F32),
        pltpu.VMEM((DB // 2, 3 * DB), U32),
        pltpu.VMEM((NB, RC + HALO, T), F32),
        pltpu.VMEM((NB, RC + HALO, T), F32),
        pltpu.VMEM((S, M + DB), BF16),
        pltpu.SemaphoreType.DMA((S // CR,)),
        pltpu.SemaphoreType.DMA((S // XR,)),
        pltpu.SemaphoreType.DMA((6,)),
        pltpu.SemaphoreType.DMA,
    ]
    out = pl.pallas_call(
        _kernel,
        out_shape=jax.ShapeDtypeStruct((S, M + DB), BF16),
        in_specs=[pl.BlockSpec(memory_space=pl.ANY)] * 9,
        out_specs=pl.BlockSpec(memory_space=pl.ANY),
        scratch_shapes=scratch,
        compiler_params=pltpu.CompilerParams(vmem_limit_bytes=120 * 1024 * 1024),
        name="mla_local_concat",
    )(
        A_x.reshape(S, M),
        A_c_kv.reshape(S, DC),
        A_w_q.reshape(M, PAIRS, 2, D),
        A_w_uk.reshape(DC, PAIRS, 2, D),
        A_w_uv.reshape(DC, PAIRS, 2, D),
        A_w_o.reshape(H * D, M),
        B_x.reshape(S, DB),
        B_wqkv,
        B_wo,
    )
    return out.reshape(1, S, M + DB)
```

```python
import functools
import math

import jax
import jax.numpy as jnp
from jax import lax
import jax.experimental.pallas as pl
import jax.experimental.pallas.tpu as pltpu

BF16 = jnp.bfloat16
F32 = jnp.float32
U32 = jnp.uint32
I32 = jnp.int32

T = 128
W = T // 2
G = 16
LOG2E = math.log2(math.e)
NEG = -1e9 * LOG2E

S = 2048
GROUPS = S // (2 * T)
M = 1024
H = 32
D = 128
DC = 512
PAIRS = H // 2
Q_SCALE = D ** -0.5 * LOG2E
STEP = 2
EXP_TILES = 4
EARLY = 2
LATE = 6
DB = 1024
DH = 32
NB = DB // T
WIN = 8
DIL = 2
HALO = 16


def _bf16(words):
    return pltpu.bitcast(words, BF16)


def _words(val):
    return pltpu.bitcast(val.astype(BF16), U32)


def _riffle(val):
    halves = [jnp.concatenate([val[r + b:r + b + 8] for r in range(0, val.shape[0], G)], axis=0)
              for b in (0, 8)]
    return pltpu.pack_elementwise(halves, packed_dtype=BF16)


def _riffled_iota(axis):
    i = lax.broadcasted_iota(I32, (T, T), axis)
    return (i & ~15) | ((i & 1) << 3) | ((i & 15) >> 1)


def _reciprocal(x):
    r = pl.reciprocal(x, approx=True)
    return r * (2.0 - x * r)


def _dot(a, b):
    return lax.dot_general(a, b, (((1,), (0,)), ((), ())), preferred_element_type=F32)


def _dot_nt(a, b):
    return lax.dot_general(a, b, (((1,), (1,)), ((), ())), preferred_element_type=F32)


def _at(n, size, offset=0, count=None):
    start = n * size if isinstance(n, int) else pl.multiple_of(n * size, size)
    return pl.ds(start + offset, size if count is None else count)


def _left(a11, a12, a21, a22):
    return [a11, a22, a11 + a22, a21 + a22, a11 + a12, a21 - a11, a12 - a22]


def _right(b11, b12, b21, b22):
    return [b12 - b22, b21 - b11, b11 + b22, b11, b22, b11 + b12, b21 + b22]


def _combine(m):
    return m[1] + m[2] - m[4] + m[6], m[0] + m[4], m[1] + m[3], m[0] + m[2] - m[3] + m[5]


def _half(words, index):
    return pltpu.unpack_elementwise(words, index=index, packed_dtype=BF16, unpacked_dtype=F32)


def _pack(lows, highs):
    return [pltpu.pack_elementwise([lo, hi], packed_dtype=BF16) for lo, hi in zip(lows, highs)]


def _on_words(sums, blocks):
    return _pack(*[sums(*[_half(b, index) for b in blocks]) for index in (0, 1)])


def _quarters(upper, lower):
    n = upper.shape[1] // 2
    return upper[:, :n], upper[:, n:], lower[:, :n], lower[:, n:]


def _exchange(tiles):
    lane = lax.broadcasted_iota(I32, tiles[0].shape, 1)
    for bit in (1, 2, 4):
        pick = (lane & bit) != 0
        tiles = [jnp.where(pick, tiles[k ^ bit], tiles[k]) for k in range(NB)]
    return tiles


def _permute_lanes(tiles):
    lane = lax.broadcasted_iota(I32, (8, T), 1)
    base = ((lane >> 2) & 0x18) | ((lane << 2) & 0x60) | (lane & 7)
    return [
        jnp.concatenate(
            [jnp.take_along_axis(t[r:r + 8], base ^ k, axis=1) for r in range(0, t.shape[0], 8)],
            axis=0)
        for k, t in enumerate(tiles)
    ]


def _tiles(a):
    return [a[:, c:c + T] for c in range(0, a.shape[1], T)]


def _shuffle(tiles):
    return jnp.concatenate(_permute_lanes(_exchange(tiles)), axis=1)


def _unshuffle(tiles):
    return jnp.concatenate(_exchange(_permute_lanes(tiles)), axis=1)


def _start(copies):
    for cp in copies:
        cp.start()


def _wait(copies):
    for cp in copies:
        cp.wait()


def _rows(src, dst, rows, sem):
    return pltpu.make_async_copy(src.bitcast(U32).at[rows], dst.at[rows], sem)


def _after(words, src, val):
    nonneg = pltpu.bitcast(words[0:8, 0:T] >> 1, I32)
    return jnp.where(jnp.tile(nonneg, (val.shape[0] // 8, 1)) < 0, src, val)


V_BASE = PAIRS * 7 * GROUPS * W


def _ctx_rows(hp, t, g):
    return _at((hp * 7 + t) * GROUPS + g, W)


def _project_out(ctx_s, wo_r, g, t, p0, p1, cols=slice(None)):
    ctx = jnp.concatenate([ctx_s[_ctx_rows(hp, t, g), :] for hp in range(p0, p1)], axis=1)
    return _dot(_bf16(ctx), _bf16(wo_r[t, (p0 + 1) * W:(p1 + 1) * W, cols]))


def _attention(x_hbm, c_hbm, wq_hbm, wuk_hbm, wuv_hbm, wo_hbm, later, ctx_s, wo_r, part_s,
               x_v, c_v, wq_v, wuk_v, wuv_v, wo_v, x_l, c_l, wq_r, wkv_r, q_s, k_s,
               c_sem, x_sem, in_sem):
    def pair(src, dst, hp, sem):
        return pltpu.make_async_copy(src.bitcast(U32).at[:, hp, 0], dst.at[hp], sem)

    def head_pairs(p0, p1, sem):
        return [pair(src, dst, hp, sem) for hp in range(p0, p1)
                for src, dst in ((wq_hbm, wq_v), (wuk_hbm, wuk_v), (wuv_hbm, wuv_v))]

    def out_weights(p0, p1, sem):
        return [_rows(wo_hbm, wo_v.at[pl.ds(T, PAIRS * T)], pl.ds(p0 * T, (p1 - p0) * T), sem)]

    def c_copies(n):
        return [_rows(c_hbm, c_v, _at(n, STEP * T), c_sem.at[n])]

    def x_copies(n):
        return [_rows(x_hbm, x_v, _at(n, STEP * T), x_sem.at[n])]

    wkv_first = [pair(wuk_hbm, wuk_v, 0, in_sem.at[0]), pair(wuv_hbm, wuv_v, 0, in_sem.at[0])]
    wq_first = [pair(wq_hbm, wq_v, 0, in_sem.at[1])]
    step0 = head_pairs(1, 3, in_sem.at[2])
    step1 = head_pairs(3, 6, in_sem.at[3]) + out_weights(0, 3, in_sem.at[3])
    step4 = head_pairs(6, PAIRS, in_sem.at[4]) + out_weights(3, PAIRS, in_sem.at[4])
    _start(wkv_first)
    for n in range(GROUPS // STEP):
        _start(c_copies(n))
    _start(wq_first)
    for n in range(GROUPS // STEP):
        _start(x_copies(n))
    _start(step0 + step1 + step4 + later)
    wo_v[0:T, :] = jnp.zeros((T, M), U32)

    def stage(src, hp, r, n):
        k = src.shape[1] // 2
        sums = []
        for odd_row in (0, 1):
            top, low = (src[hp, pl.ds(k0 + 2 * r + odd_row, n, stride=2), :] for k0 in (0, k))
            sums.append(_right(_half(top, 0), _half(top, 1), _half(low, 0), _half(low, 1)))
        return _pack(*sums)

    def stage_q(hp, slot, r, n):
        for t, w in enumerate(stage(wq_v, hp, r, n)):
            wq_r[slot, t, r:r + n, :] = w

    def stage_kv(hp, slot, which, r, n):
        for t, w in enumerate(stage((wuk_v, wuv_v)[which], hp, r, n)):
            wkv_r[slot, t, r:r + n, which * D:(which + 1) * D] = w

    def stage_out(slab, unit):
        r, c = unit // 4 * 8, unit % 4 * T
        blocks = [wo_v[_at(slab, T, head * W + r, 8), c0 + c:c0 + c + T]
                  for head in (0, 1) for c0 in (0, M // 2)]
        for t, w in enumerate(_on_words(_right, blocks)):
            wo_r[t, _at(slab, W, r, 8), c:c + T] = w

    def store_q(g, lower, odd, q):
        q_s[odd, _at(g, T, lower * W, W), :] = _riffle(q * Q_SCALE)

    def store_k(g, lower, odd, kv):
        k_s[odd, _at(g, T, lower * W, W), :] = _riffle(kv[:, :D])

    def store_v(g, lower, odd, kv):
        ctx_s[_at(g, T, V_BASE + odd * (S // 2) + lower * W, W), :] = _riffle(kv[:, D:])

    def first_projections(copies, src, left_s, right_s, stores):
        def step(n, carry):
            _wait(copies(n))
            for u in range(STEP):
                g = n * STEP + u
                left = _on_words(_left, _quarters(src[_at(g, T, 0, W), :], src[_at(g, T, W, W), :]))
                for t, w in enumerate(left):
                    left_s[t, _at(g, W), :] = w
                out = _combine([_dot(_bf16(left[t]), _bf16(right_s[0, t])) for t in range(7)])
                for b, y in enumerate(out):
                    for store in stores:
                        store(g, b // 2, b % 2, y)
            return carry

        lax.fori_loop(0, GROUPS // STEP, step, None)

    _wait(wkv_first)
    for which in (0, 1):
        stage_kv(0, 0, which, 0, DC // 4)
    first_projections(c_copies, c_v, c_l, wkv_r, (store_k, store_v))
    _wait(wq_first)
    stage_q(0, 0, 0, M // 4)
    first_projections(x_copies, x_v, x_l, wq_r, (store_q,))
    _wait(step0)
    stage_q(1, 1, 0, M // 4)
    for which in (0, 1):
        stage_kv(1, 1, which, 0, DC // 4)

    def attend(g, lower, odd, fill, v_base):
        tile = 2 * g + lower
        keys = (tile + 1) * W
        s = _tiles(_dot_nt(_bf16(q_s[odd, _at(tile, W), :]), _bf16(k_s[odd, 0:keys, :])))
        s[-1] = jnp.where(_riffled_iota(1) <= _riffled_iota(0), s[-1], NEG)
        top = jnp.max(functools.reduce(jnp.maximum, s), axis=1, keepdims=True)
        top = jnp.broadcast_to(top, (T, T))
        gates = fill()[-3:]
        v = ctx_s[pl.ds(v_base + odd * (S // 2), keys), :]
        total = ctx = None
        for j in range(0, len(s), EXP_TILES):
            at = _after(c_v, gates.pop(0)[:, -T:], top)
            p = [jnp.exp2(a - at) for a in s[j:j + EXP_TILES]]
            total = functools.reduce(jnp.add, p if total is None else [total] + p)
            y = _dot(jnp.concatenate(p, axis=1).astype(BF16),
                     _bf16(v[j * W:(j + len(p)) * W]))
            ctx = y if ctx is None else ctx + y
            gates.append(y)
        return ctx * _reciprocal(jnp.sum(total, axis=1, keepdims=True))

    def head_pair(hp, products, between, done, v_base=V_BASE):
        cuts = (0, 4, 7, 11, 14)
        for g in reversed(range(GROUPS)):
            todo, m, ctx = products(g), [], {}
            for b, (lower, odd) in enumerate(((1, 0), (1, 1), (0, 0), (0, 1))):
                def fill():
                    between(4 * g + b)
                    m.extend(f() for f in todo[cuts[b]:cuts[b + 1]])
                    done(g, b, m, False)
                    return m[cuts[b]:]

                ctx[lower, odd] = attend(g, lower, odd, fill, v_base)
                done(g, b, m, True)
                left = _left(*[ctx.get(k, ctx[1, 0]) for k in ((0, 0), (0, 1), (1, 0), (1, 1))])
                for t in ((), (1, 3), (0, 2, 5), (4, 6))[b]:
                    ctx_s[_ctx_rows(hp, t, g), :] = _riffle(left[t])

    def pair_step(hp, carry):
        pl.when(hp == 1)(lambda: _wait(step1))
        pl.when(hp == 4)(lambda: _wait(step4))
        slot = (hp + 1) % 2
        held = {}

        def products(g):
            return [lambda left=left, right=right, t=t:
                    _dot(_bf16(left[t, _at(g, W), :]), _bf16(right[slot, t]))
                    for left, right in ((x_l, wq_r), (c_l, wkv_r)) for t in range(7)]

        def between(unit):
            ahead = jnp.minimum(hp + 2, PAIRS - 1)
            stage_q(ahead, 1 - slot, unit * 8, 8)
            stage_kv(ahead, 1 - slot, unit % 2, unit // 2 * 8, 8)
            stage_out(hp, unit)

        def done(g, b, m, attended):
            if (b, attended) == (1, False):
                held["q"] = _combine(m[:7])
                for odd in (0, 1):
                    store_q(g, 1, odd, held["q"][2 + odd])
            if b >= 2 and not attended:
                store_q(g, 0, b - 2, held["q"][b - 2])
            if (b, attended) == (3, False):
                held["kv"] = _combine(m[7:])
                for n, y in enumerate(held["kv"]):
                    store_k(g, n // 2, n % 2, y)
                    if n != 1:
                        store_v(g, n // 2, n % 2, y)
            if (b, attended) == (3, True):
                store_v(g, 0, 1, held["kv"][1])

        head_pair(hp, products, between, done)
        return carry + V_BASE // (PAIRS - 1)

    v_base = lax.fori_loop(0, PAIRS - 1, pair_step, V_BASE % (PAIRS - 1))

    def early(g):
        return [functools.partial(_project_out, ctx_s, wo_r, g, t, 0, EARLY, pl.ds(c, M // 4))
                for t in range(7) for c in (0, M // 4)]

    def early_done(g, b, m, attended):
        if (b, attended) == (3, False):
            halves = [_combine(m[c::2]) for c in (0, 1)]
            for n in range(4):
                for c in (0, 1):
                    c0 = n % 2 * (M // 2) + c * (M // 4)
                    part_s[_at(2 * g + n // 2, T), c0:c0 + M // 4] = halves[c][n]

    def last_weights(unit):
        for slab in (PAIRS - 1, PAIRS):
            stage_out(slab, unit)

    head_pair(PAIRS - 1, early, last_weights, early_done, pl.multiple_of(v_base, W))


def _outputs(out_hbm, later, ctx_s, wo_r, part_s, bx_v, wqkv_v, bwo_v,
             wqkv_r, bwo_r, bk_s, bv_s, out_s, out_sem):
    after = functools.partial(_after, bx_v)
    _wait(later)

    def out_blocks(g):
        return [(_at(2 * g + n // 2, T), pl.ds(n % 2 * (M // 2), M // 2)) for n in range(4)]

    def prepare(i, carry):
        for u in range(2):
            g = 2 * i + u
            m = [_project_out(ctx_s, wo_r, g, t, EARLY, LATE) for t in range(7)]
            for at, y in zip(out_blocks(g), _combine(m)):
                part_s[at] += y
            size = DB // 4 // GROUPS
            for n in range(6):
                which, r = n // 2, n % 2 * (size // 2)
                w = jnp.concatenate(
                    [wqkv_v[_at(g, size, k0 + r, size // 2), which * DB:(which + 1) * DB]
                     for k0 in (0, DB // 4)], axis=0)
                gate = pltpu.bitcast(m[n][:size, T:2 * T], U32)
                w = _shuffle([after(gate, a) for a in _tiles(w)])
                for t, a in enumerate(_on_words(_right, _quarters(w[:size // 2], w[size // 2:]))):
                    wqkv_r[which, t, _at(g, size, r, size // 2), :] = a
            for n, r in enumerate(range(0, size, 8)):
                gate = pltpu.bitcast(m[n][:8, :T], U32)
                w = [jnp.concatenate(
                    [after(gate, a) for a in _tiles(bwo_v[_at(g, size, k0 + r, 8), :])], axis=1)
                    for k0 in (0, DB // 4)]
                for t, a in enumerate(_on_words(_right, _quarters(*w))):
                    bwo_r[t, _at(g, size, r, 8), :] = a
        return carry

    lax.fori_loop(0, GROUPS // 2, prepare, None)
    for j in range(NB):
        bk_s[j, 0:HALO, :] = jnp.zeros((HALO, T), F32)
        bv_s[j, 0:HALO, :] = jnp.zeros((HALO, T), F32)

    def b_proj(left, right):
        m = [_dot(left[t], _bf16(right[t])) for t in range(7)]
        c11, c12, c21, c22 = _combine(m)
        return m, jnp.concatenate(
            [jnp.concatenate([c11, c12], axis=1), jnp.concatenate([c21, c22], axis=1)], axis=0)

    def b_weights(pos, r, q, gate):
        logits = [None] * WIN
        for j, qj in enumerate(_tiles(q[r:r + G])):
            qj = after(gate[j * G:(j + 1) * G], qj) * (DH ** -0.5 * LOG2E)
            for w in range(WIN):
                t = qj * bk_s[j, pl.ds(HALO + r - DIL * w, G), :]
                logits[w] = t if logits[w] is None else logits[w] + t
        for w in range(WIN):
            t = logits[w] + pltpu.roll(logits[w], 64, 1)
            t = t + pltpu.roll(t, 32, 1)
            if r < DIL * w:
                t = jnp.where(pos + r + lax.broadcasted_iota(I32, (G, T), 0) >= DIL * w, t, NEG)
            logits[w] = t
        top = functools.reduce(jnp.maximum, logits)
        e = [jnp.exp2(t - top) for t in logits]
        inv = _reciprocal(functools.reduce(jnp.add, e))
        return [t * inv for t in e]

    def b_mix(r, attn, gate):
        acc = [None] * NB
        for w in range(WIN):
            a = after(gate[w * G:(w + 1) * G], attn[w])
            for j in range(NB):
                t = a * bv_s[j, pl.ds(HALO + r - DIL * w, G), :]
                acc[j] = t if acc[j] is None else acc[j] + t
        return _unshuffle(acc)

    def out_copy(g, branch):
        cols = pl.ds(branch * M, M)
        return pltpu.make_async_copy(
            out_s.at[g % 2, :, cols], out_hbm.bitcast(U32).at[_at(g, T), cols],
            out_sem.at[g % 2, branch])

    def group(g, carry):
        pl.when(g >= 2)(lambda: _wait([out_copy(g - 2, 0), out_copy(g - 2, 1)]))
        xs = _on_words(_left, _quarters(bx_v[_at(g, T, 0, W), :], bx_v[_at(g, T, W, W), :]))
        xs = [_bf16(a) for a in xs]
        _, k = b_proj(xs, wqkv_r.at[1])
        for j, t in enumerate(_tiles(k)):
            bk_s[j, HALO:, :] = t
        _, q = b_proj(xs, wqkv_r.at[0])
        m, v = b_proj(xs, wqkv_r.at[2])
        for j, t in enumerate(_tiles(v)):
            bv_s[j, HALO:, :] = t
        gates = [t for y in m for t in _tiles(y)[1::2]]
        m = [_project_out(ctx_s, wo_r, g, t, LATE, PAIRS) for t in range(7)]
        gates += [t for y in m for t in _tiles(y)]
        rows = range(0, 2 * T, G)
        attn = [b_weights(g * (2 * T), r, q, gates[n]) for n, r in enumerate(rows)]
        o = jnp.concatenate(
            [b_mix(r, attn[n], gates[len(rows) + 1 + n]) for n, r in enumerate(rows)], axis=0)
        for n, (at, y) in enumerate(zip(out_blocks(g), _combine(m))):
            y = _bf16(_riffle(part_s[at] + y)).astype(F32)
            out_s[g % 2, _at(n // 2, W), at[1]] = _riffle(y)
        out_copy(g, 0).start()
        _, y = b_proj([a.astype(BF16) for a in _left(*_quarters(o[:T], o[T:]))], bwo_r)
        out_s[g % 2, :, M:] = _words(y)
        for j in range(NB):
            bk_s[j, 0:HALO, :] = bk_s[j, 2 * T:, :]
            bv_s[j, 0:HALO, :] = bv_s[j, 2 * T:, :]
        out_copy(g, 1).start()
        return carry

    lax.fori_loop(0, GROUPS, group, None)
    for g in range(GROUPS - 2, GROUPS):
        _wait([out_copy(g, 0), out_copy(g, 1)])


def _kernel(x_hbm, c_hbm, wq_hbm, wuk_hbm, wuv_hbm, wo_hbm, bx_hbm, wqkv_hbm, bwo_hbm,
            out_hbm, ctx_s, wo_r, part_s, bx_v, wqkv_v, bwo_v, later_sem):
    later = [_rows(src, dst, slice(None), later_sem)
             for src, dst in ((bx_hbm, bx_v), (wqkv_hbm, wqkv_v), (bwo_hbm, bwo_v))]
    pl.run_scoped(
        functools.partial(_attention, x_hbm, c_hbm, wq_hbm, wuk_hbm, wuv_hbm, wo_hbm, later,
                          ctx_s, wo_r, part_s),
        pltpu.VMEM((S // 2, M), U32),
        pltpu.VMEM((S // 2, DC), U32),
        pltpu.VMEM((PAIRS, M, D), U32),
        pltpu.VMEM((PAIRS, DC, D), U32),
        pltpu.VMEM((PAIRS, DC, D), U32),
        pltpu.VMEM(((PAIRS + 1) * T, M), U32),
        pltpu.VMEM((7, S // 4, M // 2), U32),
        pltpu.VMEM((7, S // 4, DC // 2), U32),
        pltpu.VMEM((2, 7, M // 4, D), U32),
        pltpu.VMEM((2, 7, DC // 4, 2 * D), U32),
        pltpu.VMEM((2, S // 2, D), U32),
        pltpu.VMEM((2, S // 2, D), U32),
        pltpu.SemaphoreType.DMA((GROUPS // STEP,)),
        pltpu.SemaphoreType.DMA((GROUPS // STEP,)),
        pltpu.SemaphoreType.DMA((5,)),
    )
    pl.run_scoped(
        functools.partial(_outputs, out_hbm, later, ctx_s, wo_r, part_s, bx_v, wqkv_v, bwo_v),
        pltpu.VMEM((3, 7, DB // 4, DB // 2), U32),
        pltpu.VMEM((7, DB // 4, DB // 2), U32),
        pltpu.VMEM((NB, HALO + 2 * T, T), F32),
        pltpu.VMEM((NB, HALO + 2 * T, T), F32),
        pltpu.VMEM((2, T, M + DB), U32),
        pltpu.SemaphoreType.DMA((2, 2)),
    )


@jax.jit
def pallas_concat_heads__compressed_kv_cla__sliding_local_dilated__prompt_kernel(
    A_x: jax.Array,
    A_c_kv: jax.Array,
    A_w_q: jax.Array,
    A_w_uk: jax.Array,
    A_w_uv: jax.Array,
    A_w_o: jax.Array,
    B_x: jax.Array,
    B_wqkv: jax.Array,
    B_wo: jax.Array,
):
    out = pl.pallas_call(
        _kernel,
        out_shape=jax.ShapeDtypeStruct((S, M + DB), BF16),
        in_specs=[pl.BlockSpec(memory_space=pl.ANY)] * 9,
        out_specs=pl.BlockSpec(memory_space=pl.ANY),
        scratch_shapes=[
            pltpu.VMEM((V_BASE + S, D), U32),
            pltpu.VMEM((7, (PAIRS + 1) * W, M // 2), U32),
            pltpu.VMEM((S, M), F32),
            pltpu.VMEM((S // 2, DB), U32),
            pltpu.VMEM((DB // 2, 3 * DB), U32),
            pltpu.VMEM((DB // 2, DB), U32),
            pltpu.SemaphoreType.DMA,
        ],
        compiler_params=pltpu.CompilerParams(vmem_limit_bytes=124 * 1024 * 1024),
        name="mla_local_concat",
    )(
        A_x.reshape(S, M),
        A_c_kv.reshape(S, DC),
        A_w_q.reshape(M, PAIRS, 2, D),
        A_w_uk.reshape(DC, PAIRS, 2, D),
        A_w_uv.reshape(DC, PAIRS, 2, D),
        A_w_o.reshape(H * D, M),
        B_x.reshape(S, DB),
        B_wqkv,
        B_wo,
    )
    return out.reshape(1, S, M + DB)
```

```python
import functools
import math

import jax
import jax.numpy as jnp
from jax import lax
import jax.experimental.pallas as pl
import jax.experimental.pallas.tpu as pltpu

BF16 = jnp.bfloat16
F32 = jnp.float32
U32 = jnp.uint32
I32 = jnp.int32

T = 128
W = T // 2
G = 16
LOG2E = math.log2(math.e)
NEG = -1e9 * LOG2E

S = 2048
GROUPS = S // (2 * T)
M = 1024
H = 32
D = 128
DC = 512
PAIRS = H // 2
Q_SCALE = D ** -0.5 * LOG2E
STEP = 2
EXP_TILES = 4
EARLY = 2
LATE = 6
DB = 1024
DH = 32
NB = DB // T
WIN = 8
DIL = 2
HALO = 16


def _bf16(words):
    return pltpu.bitcast(words, BF16)


def _riffle(val):
    halves = [jnp.concatenate([val[r + b:r + b + 8] for r in range(0, val.shape[0], G)], axis=0)
              for b in (0, 8)]
    return pltpu.pack_elementwise(halves, packed_dtype=BF16)


def _riffled_iota(axis):
    i = lax.broadcasted_iota(I32, (T, T), axis)
    return (i & ~15) | ((i & 1) << 3) | ((i & 15) >> 1)


def _reciprocal(x):
    r = pl.reciprocal(x, approx=True)
    return r * (2.0 - x * r)


def _dot(a, b):
    return lax.dot_general(a, b, (((1,), (0,)), ((), ())), preferred_element_type=F32)


def _dot_nt(a, b):
    return lax.dot_general(a, b, (((1,), (1,)), ((), ())), preferred_element_type=F32)


def _at(n, size, offset=0, count=None):
    start = n * size if isinstance(n, int) else pl.multiple_of(n * size, size)
    return pl.ds(start + offset, size if count is None else count)


def _left(a11, a12, a21, a22):
    return [a11, a22, a11 + a22, a21 + a22, a11 + a12, a21 - a11, a12 - a22]


def _right(b11, b12, b21, b22):
    return [b12 - b22, b21 - b11, b11 + b22, b11, b22, b11 + b12, b21 + b22]


def _combine(m):
    return m[1] + m[2] - m[4] + m[6], m[0] + m[4], m[1] + m[3], m[0] + m[2] - m[3] + m[5]


def _half(words, index):
    return pltpu.unpack_elementwise(words, index=index, packed_dtype=BF16, unpacked_dtype=F32)


def _pack(lows, highs):
    return [pltpu.pack_elementwise([lo, hi], packed_dtype=BF16) for lo, hi in zip(lows, highs)]


def _on_words(sums, blocks):
    return _pack(*[sums(*[_half(b, index) for b in blocks]) for index in (0, 1)])


def _quarters(upper, lower):
    n = upper.shape[1] // 2
    return upper[:, :n], upper[:, n:], lower[:, :n], lower[:, n:]


def _exchange(tiles):
    lane = lax.broadcasted_iota(I32, tiles[0].shape, 1)
    for bit in (1, 2, 4):
        pick = (lane & bit) != 0
        tiles = [jnp.where(pick, tiles[k ^ bit], tiles[k]) for k in range(NB)]
    return tiles


def _permute_lanes(tiles):
    lane = lax.broadcasted_iota(I32, (8, T), 1)
    base = ((lane >> 2) & 0x18) | ((lane << 2) & 0x60) | (lane & 7)
    return [
        jnp.concatenate(
            [jnp.take_along_axis(t[r:r + 8], base ^ k, axis=1) for r in range(0, t.shape[0], 8)],
            axis=0)
        for k, t in enumerate(tiles)
    ]


def _tiles(a):
    return [a[:, c:c + T] for c in range(0, a.shape[1], T)]


def _shuffle(tiles):
    return jnp.concatenate(_permute_lanes(_exchange(tiles)), axis=1)


def _unshuffle(tiles):
    return jnp.concatenate(_exchange(_permute_lanes(tiles)), axis=1)


def _start(copies):
    for cp in copies:
        cp.start()


def _wait(copies):
    for cp in copies:
        cp.wait()


def _rows(src, dst, rows, sem):
    return pltpu.make_async_copy(src.bitcast(U32).at[rows], dst.at[rows], sem)


def _after(words, src, val):
    nonneg = pltpu.bitcast(words[0:8, 0:T] >> 1, I32)
    return jnp.where(jnp.tile(nonneg, (val.shape[0] // 8, 1)) < 0, src, val)


V_BASE = PAIRS * 7 * GROUPS * W


def _ctx_rows(hp, t, g):
    return _at((hp * 7 + t) * GROUPS + g, W)


def _project_out(ctx_s, wo_r, g, t, p0, p1, cols=slice(None)):
    ctx = jnp.concatenate([ctx_s[_ctx_rows(hp, t, g), :] for hp in range(p0, p1)], axis=1)
    return _dot(_bf16(ctx), _bf16(wo_r[t, (p0 + 1) * W:(p1 + 1) * W, cols]))


def _attention(x_hbm, c_hbm, wq_hbm, wuk_hbm, wuv_hbm, wo_hbm, later, ctx_s, wo_r, part_s,
               x_v, c_v, wq_v, wuk_v, wuv_v, wo_v, x_l, c_l, wq_r, wkv_r, q_s, k_s,
               c_sem, x_sem, in_sem):
    def pair(src, dst, hp, sem):
        return pltpu.make_async_copy(src.bitcast(U32).at[:, hp, 0], dst.at[hp], sem)

    def head_pairs(p0, p1, sem):
        return [pair(src, dst, hp, sem) for hp in range(p0, p1)
                for src, dst in ((wq_hbm, wq_v), (wuk_hbm, wuk_v), (wuv_hbm, wuv_v))]

    def out_weights(p0, p1, sem):
        return [_rows(wo_hbm, wo_v.at[pl.ds(T, PAIRS * T)], pl.ds(p0 * T, (p1 - p0) * T), sem)]

    def c_copies(n):
        return [_rows(c_hbm, c_v, _at(n, STEP * T), c_sem.at[n])]

    def x_copies(n):
        return [_rows(x_hbm, x_v, _at(n, STEP * T), x_sem.at[n])]

    wkv_first = [pair(wuk_hbm, wuk_v, 0, in_sem.at[0]), pair(wuv_hbm, wuv_v, 0, in_sem.at[0])]
    wq_first = [pair(wq_hbm, wq_v, 0, in_sem.at[1])]
    second = head_pairs(1, 2, in_sem.at[5])
    step0 = head_pairs(2, 3, in_sem.at[2])
    step1 = head_pairs(3, 6, in_sem.at[3]) + out_weights(0, 3, in_sem.at[3])
    step4 = head_pairs(6, PAIRS, in_sem.at[4]) + out_weights(3, PAIRS, in_sem.at[4])
    _start(wkv_first)
    for n in range(GROUPS // STEP):
        _start(c_copies(n))
    _start(wq_first)
    for n in range(GROUPS // STEP):
        _start(x_copies(n) + ([] if n else second))
    _start(step0 + step1 + step4 + later)
    wo_v[0:T, :] = jnp.zeros((T, M), U32)

    def stage(src, hp, r, n):
        k = src.shape[1] // 2
        sums = []
        for odd_row in (0, 1):
            top, low = (src[hp, pl.ds(2 * r + (k0 + odd_row), n, stride=2), :] for k0 in (0, k))
            sums.append(_right(_half(top, 0), _half(top, 1), _half(low, 0), _half(low, 1)))
        return _pack(*sums)

    def stage_q(hp, slot, r, n):
        for t, w in enumerate(stage(wq_v, hp, r, n)):
            wq_r[slot, t, pl.ds(r, n), :] = w

    def stage_kv(hp, slot, which, r, n):
        for t, w in enumerate(stage((wuk_v, wuv_v)[which], hp, r, n)):
            wkv_r[slot, t, pl.ds(r, n), which * D:(which + 1) * D] = w

    def stage_out(slab, unit):
        r, c = unit // 4 * 8, unit % 4 * T
        blocks = [wo_v[_at(slab, T, head * W + r, 8), c0 + c:c0 + c + T]
                  for head in (0, 1) for c0 in (0, M // 2)]
        for t, w in enumerate(_on_words(_right, blocks)):
            wo_r[t, _at(slab, W, r, 8), c:c + T] = w

    def store_q(g, lower, odd, q):
        q_s[odd, _at(g, T, lower * W, W), :] = _riffle(q * Q_SCALE)

    def store_k(g, lower, odd, kv):
        k_s[odd, _at(g, T, lower * W, W), :] = _riffle(kv[:, :D])

    def store_v(g, lower, odd, kv):
        ctx_s[_at(g, T, V_BASE + odd * (S // 2) + lower * W, W), :] = _riffle(kv[:, D:])

    def first_projections(copies, src, left_s, right_s, stores, also):
        def step(n, carry):
            _wait(copies(n))
            for u in range(STEP):
                g = n * STEP + u
                left = _on_words(_left, _quarters(src[_at(g, T, 0, W), :], src[_at(g, T, W, W), :]))
                for t, w in enumerate(left):
                    left_s[t, _at(g, W), :] = w
                out = _combine([_dot(_bf16(left[t]), _bf16(right_s[0, t])) for t in range(7)])
                for b, y in enumerate(out):
                    for store in stores:
                        store(g, b // 2, b % 2, y)
                also(g)
            return carry

        lax.fori_loop(0, GROUPS // STEP, step, None)

    def stage_part(hp, g, q=True, kv=True):
        size = DC // 4 // GROUPS
        r = pl.multiple_of(g * size, size)
        if q:
            stage_q(hp, hp, 2 * r, 2 * size)
        for which in (0, 1) if kv else ():
            stage_kv(hp, hp, which, r, size)

    _wait(wkv_first)
    pl.loop(0, GROUPS)(functools.partial(stage_part, 0, q=False))
    first_projections(c_copies, c_v, c_l, wkv_r, (store_k, store_v), lambda g: None)
    _wait(wq_first)
    pl.loop(0, GROUPS)(functools.partial(stage_part, 0, kv=False))
    _wait(second)
    first_projections(x_copies, x_v, x_l, wq_r, (store_q,), functools.partial(stage_part, 1))
    _wait(step0)

    def attend(g, lower, odd, fill, v_base):
        tile = 2 * g + lower
        keys = (tile + 1) * W
        s = _tiles(_dot_nt(_bf16(q_s[odd, _at(tile, W), :]), _bf16(k_s[odd, 0:keys, :])))
        s[-1] = jnp.where(_riffled_iota(1) <= _riffled_iota(0), s[-1], NEG)
        top = jnp.max(functools.reduce(jnp.maximum, s), axis=1, keepdims=True)
        top = jnp.broadcast_to(top, (T, T))
        gates = fill()[-3:]
        v = ctx_s[pl.ds(v_base + odd * (S // 2), keys), :]
        total = ctx = None
        for j in range(0, len(s), EXP_TILES):
            at = _after(c_v, gates.pop(0)[:, -T:], top)
            p = [jnp.exp2(a - at) for a in s[j:j + EXP_TILES]]
            total = functools.reduce(jnp.add, p if total is None else [total] + p)
            y = _dot(jnp.concatenate(p, axis=1).astype(BF16),
                     _bf16(v[j * W:(j + len(p)) * W]))
            ctx = y if ctx is None else ctx + y
            gates.append(y)
        return ctx * _reciprocal(jnp.sum(total, axis=1, keepdims=True))

    def head_pair(hp, products, between, done, v_base=V_BASE):
        cuts = (0, 3, 7, 10, 14)
        for g in reversed(range(GROUPS)):
            todo, m, ctx = products(g), [], {}
            for b, (lower, odd) in enumerate(((1, 0), (1, 1), (0, 0), (0, 1))):
                def fill():
                    between(4 * g + b)
                    m.extend(f() for f in todo[cuts[b]:cuts[b + 1]])
                    done(g, b, m, False)
                    return m[cuts[b]:]

                ctx[lower, odd] = attend(g, lower, odd, fill, v_base)
                done(g, b, m, True)
                left = _left(*[ctx.get(k, ctx[1, 0]) for k in ((0, 0), (0, 1), (1, 0), (1, 1))])
                for t in ((), (1, 3), (0, 2, 5), (4, 6))[b]:
                    ctx_s[_ctx_rows(hp, t, g), :] = _riffle(left[t])

    def pair_step(hp, carry):
        pl.when(hp == 1)(lambda: _wait(step1))
        pl.when(hp == 4)(lambda: _wait(step4))
        slot = (hp + 1) % 2
        held = {}

        def products(g):
            return [lambda left=left, right=right, t=t:
                    _dot(_bf16(left[t, _at(g, W), :]), _bf16(right[slot, t]))
                    for left, right in ((x_l, wq_r), (c_l, wkv_r)) for t in range(7)]

        def between(unit):
            ahead = jnp.minimum(hp + 2, PAIRS - 1)
            stage_q(ahead, 1 - slot, unit * 8, 8)
            stage_kv(ahead, 1 - slot, unit % 2, unit // 2 * 8, 8)
            stage_out(hp, unit)

        def done(g, b, m, attended):
            if (b, attended) == (1, False):
                held["q"] = _combine(m[:7])
                for odd in (0, 1):
                    store_q(g, 1, odd, held["q"][2 + odd])
            if b >= 2 and not attended:
                store_q(g, 0, b - 2, held["q"][b - 2])
            if (b, attended) == (3, False):
                held["kv"] = _combine(m[7:])
                for n, y in enumerate(held["kv"]):
                    store_k(g, n // 2, n % 2, y)
                    if n != 1:
                        store_v(g, n // 2, n % 2, y)
            if (b, attended) == (3, True):
                store_v(g, 0, 1, held["kv"][1])

        head_pair(hp, products, between, done)
        return carry + V_BASE // (PAIRS - 1)

    v_base = lax.fori_loop(0, PAIRS - 1, pair_step, V_BASE % (PAIRS - 1))

    def early(g):
        return [functools.partial(_project_out, ctx_s, wo_r, g, t, 0, EARLY, pl.ds(c, M // 4))
                for t in range(7) for c in (0, M // 4)]

    def early_done(g, b, m, attended):
        if (b, attended) == (3, False):
            halves = [_combine(m[c::2]) for c in (0, 1)]
            for n in range(4):
                for c in (0, 1):
                    c0 = n % 2 * (M // 2) + c * (M // 4)
                    part_s[_at(2 * g + n // 2, T), c0:c0 + M // 4] = halves[c][n]

    def last_weights(unit):
        for slab in (PAIRS - 1, PAIRS):
            stage_out(slab, unit)

    head_pair(PAIRS - 1, early, last_weights, early_done, pl.multiple_of(v_base, W))


def _outputs(out_hbm, later, ctx_s, wo_r, part_s, bx_v, wqkv_v, bwo_v,
             wqkv_r, bwo_r, bk_s, bv_s, out_s, out_sem):
    after = functools.partial(_after, bx_v)
    _wait(later)

    def out_blocks(g):
        return [(_at(2 * g + n // 2, T), pl.ds(n % 2 * (M // 2), M // 2)) for n in range(4)]

    def prepare(i, carry):
        for u in range(2):
            g = 2 * i + u
            m = [_project_out(ctx_s, wo_r, g, t, EARLY, LATE) for t in range(7)]
            for at, y in zip(out_blocks(g), _combine(m)):
                part_s[at] += y
            size = DB // 4 // GROUPS
            for n in range(6):
                which, r = n // 2, n % 2 * (size // 2)
                w = jnp.concatenate(
                    [wqkv_v[_at(g, size, k0 + r, size // 2), which * DB:(which + 1) * DB]
                     for k0 in (0, DB // 4)], axis=0)
                gate = pltpu.bitcast(m[n][:size, T:2 * T], U32)
                w = _shuffle([after(gate, a) for a in _tiles(w)])
                for t, a in enumerate(_on_words(_right, _quarters(w[:size // 2], w[size // 2:]))):
                    wqkv_r[which, t, _at(g, size, r, size // 2), :] = a
            for n, r in enumerate(range(0, size, 8)):
                gate = pltpu.bitcast(m[n][:8, :T], U32)
                w = [jnp.concatenate(
                    [after(gate, a) for a in _tiles(bwo_v[_at(g, size, k0 + r, 8), :])], axis=1)
                    for k0 in (0, DB // 4)]
                for t, a in enumerate(_on_words(_right, _quarters(*w))):
                    bwo_r[t, _at(g, size, r, 8), :] = a
        return carry

    lax.fori_loop(0, GROUPS // 2, prepare, None)
    for j in range(NB):
        bk_s[j, 0:HALO, :] = jnp.zeros((HALO, T), F32)
        bv_s[j, 0:HALO, :] = jnp.zeros((HALO, T), F32)

    def b_proj(left, right):
        m = [_dot(left[t], _bf16(right[t])) for t in range(7)]
        c11, c12, c21, c22 = _combine(m)
        return m, jnp.concatenate(
            [jnp.concatenate([c11, c12], axis=1), jnp.concatenate([c21, c22], axis=1)], axis=0)

    def b_weights(pos, r, q, gate):
        logits = [None] * WIN
        for j, qj in enumerate(_tiles(q[r:r + G])):
            qj = after(gate[j * G:(j + 1) * G], qj) * (DH ** -0.5 * LOG2E)
            for w in range(WIN):
                t = qj * bk_s[j, pl.ds(HALO + r - DIL * w, G), :]
                logits[w] = t if logits[w] is None else logits[w] + t
        for w in range(WIN):
            t = logits[w] + pltpu.roll(logits[w], 64, 1)
            t = t + pltpu.roll(t, 32, 1)
            if r < DIL * w:
                t = jnp.where(pos + r + lax.broadcasted_iota(I32, (G, T), 0) >= DIL * w, t, NEG)
            logits[w] = t
        top = functools.reduce(jnp.maximum, logits)
        e = [jnp.exp2(t - top) for t in logits]
        inv = _reciprocal(functools.reduce(jnp.add, e))
        return [t * inv for t in e]

    def b_mix(r, attn, gate):
        acc = [None] * NB
        for w in range(WIN):
            a = after(gate[w * G:(w + 1) * G], attn[w])
            for j in range(NB):
                t = a * bv_s[j, pl.ds(HALO + r - DIL * w, G), :]
                acc[j] = t if acc[j] is None else acc[j] + t
        return _unshuffle(acc)

    def out_copy(g, branch):
        cols = pl.ds(branch * M, M)
        return pltpu.make_async_copy(
            out_s.at[g % 2, :, cols], out_hbm.at[_at(g, 2 * T), cols], out_sem.at[g % 2, branch])

    def group(g, carry):
        pl.when(g >= 2)(lambda: _wait([out_copy(g - 2, 0), out_copy(g - 2, 1)]))
        xs = _on_words(_left, _quarters(bx_v[_at(g, T, 0, W), :], bx_v[_at(g, T, W, W), :]))
        xs = [_bf16(a) for a in xs]
        _, k = b_proj(xs, wqkv_r.at[1])
        for j, t in enumerate(_tiles(k)):
            bk_s[j, HALO:, :] = t
        _, q = b_proj(xs, wqkv_r.at[0])
        m, v = b_proj(xs, wqkv_r.at[2])
        for j, t in enumerate(_tiles(v)):
            bv_s[j, HALO:, :] = t
        gates = [t for y in m for t in _tiles(y)[1::2]]
        m = [_project_out(ctx_s, wo_r, g, t, LATE, PAIRS) for t in range(7)]
        gates += [t for y in m for t in _tiles(y)]
        rows = range(0, 2 * T, G)
        attn = [b_weights(g * (2 * T), r, q, gates[n]) for n, r in enumerate(rows)]
        o = jnp.concatenate(
            [b_mix(r, attn[n], gates[len(rows) + 1 + n]) for n, r in enumerate(rows)], axis=0)
        for n, (at, y) in enumerate(zip(out_blocks(g), _combine(m))):
            y = _bf16(_riffle(part_s[at] + y)).astype(F32)
            out_s[g % 2, _at(n // 2, T), at[1]] = _bf16(_riffle(y))
        out_copy(g, 0).start()
        _, y = b_proj([a.astype(BF16) for a in _left(*_quarters(o[:T], o[T:]))], bwo_r)
        out_s[g % 2, :, M:] = y.astype(BF16)
        for j in range(NB):
            bk_s[j, 0:HALO, :] = bk_s[j, 2 * T:, :]
            bv_s[j, 0:HALO, :] = bv_s[j, 2 * T:, :]
        out_copy(g, 1).start()
        return carry

    lax.fori_loop(0, GROUPS, group, None)
    for g in range(GROUPS - 2, GROUPS):
        _wait([out_copy(g, 0), out_copy(g, 1)])


def _kernel(x_hbm, c_hbm, wq_hbm, wuk_hbm, wuv_hbm, wo_hbm, bx_hbm, wqkv_hbm, bwo_hbm,
            out_hbm, ctx_s, wo_r, part_s, bx_v, wqkv_v, bwo_v, later_sem):
    later = [_rows(src, dst, slice(None), later_sem)
             for src, dst in ((bx_hbm, bx_v), (wqkv_hbm, wqkv_v), (bwo_hbm, bwo_v))]
    pl.run_scoped(
        functools.partial(_attention, x_hbm, c_hbm, wq_hbm, wuk_hbm, wuv_hbm, wo_hbm, later,
                          ctx_s, wo_r, part_s),
        pltpu.VMEM((S // 2, M), U32),
        pltpu.VMEM((S // 2, DC), U32),
        pltpu.VMEM((PAIRS, M, D), U32),
        pltpu.VMEM((PAIRS, DC, D), U32),
        pltpu.VMEM((PAIRS, DC, D), U32),
        pltpu.VMEM(((PAIRS + 1) * T, M), U32),
        pltpu.VMEM((7, S // 4, M // 2), U32),
        pltpu.VMEM((7, S // 4, DC // 2), U32),
        pltpu.VMEM((2, 7, M // 4, D), U32),
        pltpu.VMEM((2, 7, DC // 4, 2 * D), U32),
        pltpu.VMEM((2, S // 2, D), U32),
        pltpu.VMEM((2, S // 2, D), U32),
        pltpu.SemaphoreType.DMA((GROUPS // STEP,)),
        pltpu.SemaphoreType.DMA((GROUPS // STEP,)),
        pltpu.SemaphoreType.DMA((6,)),
    )
    pl.run_scoped(
        functools.partial(_outputs, out_hbm, later, ctx_s, wo_r, part_s, bx_v, wqkv_v, bwo_v),
        pltpu.VMEM((3, 7, DB // 4, DB // 2), U32),
        pltpu.VMEM((7, DB // 4, DB // 2), U32),
        pltpu.VMEM((NB, HALO + 2 * T, T), F32),
        pltpu.VMEM((NB, HALO + 2 * T, T), F32),
        pltpu.VMEM((2, 2 * T, M + DB), BF16),
        pltpu.SemaphoreType.DMA((2, 2)),
    )


@jax.jit
def pallas_concat_heads__compressed_kv_cla__sliding_local_dilated__prompt_kernel(
    A_x: jax.Array,
    A_c_kv: jax.Array,
    A_w_q: jax.Array,
    A_w_uk: jax.Array,
    A_w_uv: jax.Array,
    A_w_o: jax.Array,
    B_x: jax.Array,
    B_wqkv: jax.Array,
    B_wo: jax.Array,
):
    out = pl.pallas_call(
        _kernel,
        out_shape=jax.ShapeDtypeStruct((S, M + DB), BF16),
        in_specs=[pl.BlockSpec(memory_space=pl.ANY)] * 9,
        out_specs=pl.BlockSpec(memory_space=pl.ANY),
        scratch_shapes=[
            pltpu.VMEM((V_BASE + S, D), U32),
            pltpu.VMEM((7, (PAIRS + 1) * W, M // 2), U32),
            pltpu.VMEM((S, M), F32),
            pltpu.VMEM((S // 2, DB), U32),
            pltpu.VMEM((DB // 2, 3 * DB), U32),
            pltpu.VMEM((DB // 2, DB), U32),
            pltpu.SemaphoreType.DMA,
        ],
        compiler_params=pltpu.CompilerParams(vmem_limit_bytes=124 * 1024 * 1024),
        name="mla_local_concat",
    )(
        A_x.reshape(S, M),
        A_c_kv.reshape(S, DC),
        A_w_q.reshape(M, PAIRS, 2, D),
        A_w_uk.reshape(DC, PAIRS, 2, D),
        A_w_uv.reshape(DC, PAIRS, 2, D),
        A_w_o.reshape(H * D, M),
        B_x.reshape(S, DB),
        B_wqkv,
        B_wo,
    )
    return out.reshape(1, S, M + DB)
```

```python
import functools
import math

import jax
import jax.numpy as jnp
from jax import lax
import jax.experimental.pallas as pl
import jax.experimental.pallas.tpu as pltpu

BF16 = jnp.bfloat16
F32 = jnp.float32
U32 = jnp.uint32
I32 = jnp.int32

T = 128
W = T // 2
G = 16
LOG2E = math.log2(math.e)
NEG = -1e9 * LOG2E

S = 2048
GROUPS = S // (2 * T)
M = 1024
H = 32
D = 128
DC = 512
PAIRS = H // 2
Q_SCALE = D ** -0.5 * LOG2E
STEP = 2
EXP_TILES = 4
EARLY = 2
LATE = 6
DB = 1024
DH = 32
NB = DB // T
WIN = 8
DIL = 2
HALO = 16


def _bf16(words):
    return pltpu.bitcast(words, BF16)


def _riffle(val):
    halves = [jnp.concatenate([val[r + b:r + b + 8] for r in range(0, val.shape[0], G)], axis=0)
              for b in (0, 8)]
    return pltpu.pack_elementwise(halves, packed_dtype=BF16)


def _riffled_iota(axis):
    i = lax.broadcasted_iota(I32, (T, T), axis)
    return (i & ~15) | ((i & 1) << 3) | ((i & 15) >> 1)


def _reciprocal(x):
    r = pl.reciprocal(x, approx=True)
    return r * (2.0 - x * r)


def _dot(a, b):
    return lax.dot_general(a, b, (((1,), (0,)), ((), ())), preferred_element_type=F32)


def _dot_nt(a, b):
    return lax.dot_general(a, b, (((1,), (1,)), ((), ())), preferred_element_type=F32)


def _at(n, size, offset=0, count=None):
    start = n * size if isinstance(n, int) else pl.multiple_of(n * size, size)
    return pl.ds(start + offset, size if count is None else count)


def _left(a11, a12, a21, a22):
    return [a11, a22, a11 + a22, a21 + a22, a11 + a12, a21 - a11, a12 - a22]


def _right(b11, b12, b21, b22):
    return [b12 - b22, b21 - b11, b11 + b22, b11, b22, b11 + b12, b21 + b22]


def _combine(m):
    return m[1] + m[2] - m[4] + m[6], m[0] + m[4], m[1] + m[3], m[0] + m[2] - m[3] + m[5]


def _half(words, index):
    return pltpu.unpack_elementwise(words, index=index, packed_dtype=BF16, unpacked_dtype=F32)


def _pack(lows, highs):
    return [pltpu.pack_elementwise([lo, hi], packed_dtype=BF16) for lo, hi in zip(lows, highs)]


def _on_words(sums, blocks):
    return _pack(*[sums(*[_half(b, index) for b in blocks]) for index in (0, 1)])


def _quarters(upper, lower):
    n = upper.shape[1] // 2
    return upper[:, :n], upper[:, n:], lower[:, :n], lower[:, n:]


def _exchange(tiles):
    lane = lax.broadcasted_iota(I32, tiles[0].shape, 1)
    for bit in (1, 2, 4):
        pick = (lane & bit) != 0
        tiles = [jnp.where(pick, tiles[k ^ bit], tiles[k]) for k in range(NB)]
    return tiles


def _permute_lanes(tiles):
    lane = lax.broadcasted_iota(I32, (8, T), 1)
    base = ((lane >> 2) & 0x18) | ((lane << 2) & 0x60) | (lane & 7)
    return [
        jnp.concatenate(
            [jnp.take_along_axis(t[r:r + 8], base ^ k, axis=1) for r in range(0, t.shape[0], 8)],
            axis=0)
        for k, t in enumerate(tiles)
    ]


def _tiles(a):
    return [a[:, c:c + T] for c in range(0, a.shape[1], T)]


def _shuffle(tiles):
    return jnp.concatenate(_permute_lanes(_exchange(tiles)), axis=1)


def _unshuffle(tiles):
    return jnp.concatenate(_exchange(_permute_lanes(tiles)), axis=1)


def _start(copies):
    for cp in copies:
        cp.start()


def _wait(copies):
    for cp in copies:
        cp.wait()


def _rows(src, dst, rows, sem):
    return pltpu.make_async_copy(src.bitcast(U32).at[rows], dst.at[rows], sem)


def _after(words, src, val):
    nonneg = pltpu.bitcast(words[0:8, 0:T] >> 1, I32)
    return jnp.where(jnp.tile(nonneg, (val.shape[0] // 8, 1)) < 0, src, val)


V_BASE = PAIRS * 7 * GROUPS * W


def _ctx_rows(hp, t, g):
    return _at((hp * 7 + t) * GROUPS + g, W)


def _project_out(ctx_s, wo_r, g, t, p0, p1, cols=slice(None)):
    ctx = jnp.concatenate([ctx_s[_ctx_rows(hp, t, g), :] for hp in range(p0, p1)], axis=1)
    return _dot(_bf16(ctx), _bf16(wo_r[t, (p0 + 1) * W:(p1 + 1) * W, cols]))


def _out_blocks(g):
    return [(_at(2 * g + n // 2, T), pl.ds(n % 2 * (M // 2), M // 2)) for n in range(4)]


def _prepare(later, ctx_s, wo_r, part_s, wqkv_v, bwo_v, wqkv_r, bwo_r):
    after = functools.partial(_after, bwo_v)
    _wait(later)

    def prepare(i, carry):
        for u in range(2):
            g = 2 * i + u
            m = [_project_out(ctx_s, wo_r, g, t, EARLY, LATE) for t in range(7)]
            for at, y in zip(_out_blocks(g), _combine(m)):
                part_s[at] = y
            size = DB // 4 // GROUPS
            for n in range(6):
                which, r = n // 2, n % 2 * (size // 2)
                w = jnp.concatenate(
                    [wqkv_v[_at(g, size, k0 + r, size // 2), which * DB:(which + 1) * DB]
                     for k0 in (0, DB // 4)], axis=0)
                gate = pltpu.bitcast(m[n][:size, T:2 * T], U32)
                w = _shuffle([after(gate, a) for a in _tiles(w)])
                for t, a in enumerate(_on_words(_right, _quarters(w[:size // 2], w[size // 2:]))):
                    wqkv_r[which, t, _at(g, size, r, size // 2), :] = a
            for n, r in enumerate(range(0, size, 8)):
                gate = pltpu.bitcast(m[n][:8, :T], U32)
                w = [jnp.concatenate(
                    [after(gate, a) for a in _tiles(bwo_v[_at(g, size, k0 + r, 8), :])], axis=1)
                    for k0 in (0, DB // 4)]
                for t, a in enumerate(_on_words(_right, _quarters(*w))):
                    bwo_r[t, _at(g, size, r, 8), :] = a
        return carry

    lax.fori_loop(0, GROUPS // 2, prepare, None)

def _attention(x_hbm, c_hbm, wq_hbm, wuk_hbm, wuv_hbm, wo_hbm, later, prepare,
               ctx_s, wo_r, part_s, x_v, c_v, wq_v, wuk_v, wuv_v, wo_v, x_l, c_l, wq_r, wkv_r, q_s, k_s,
               c_sem, x_sem, in_sem):
    def pair(src, dst, hp, sem):
        return pltpu.make_async_copy(src.bitcast(U32).at[:, hp, 0], dst.at[hp], sem)

    def head_pairs(p0, p1, sem):
        return [pair(src, dst, hp, sem) for hp in range(p0, p1)
                for src, dst in ((wq_hbm, wq_v), (wuk_hbm, wuk_v), (wuv_hbm, wuv_v))]

    def out_weights(p0, p1, sem):
        return [_rows(wo_hbm, wo_v.at[pl.ds(T, PAIRS * T)], pl.ds(p0 * T, (p1 - p0) * T), sem)]

    def c_copies(n):
        return [_rows(c_hbm, c_v, _at(n, STEP * T), c_sem.at[n])]

    def x_copies(n):
        return [_rows(x_hbm, x_v, _at(n, STEP * T), x_sem.at[n])]

    wkv_first = [pair(wuk_hbm, wuk_v, 0, in_sem.at[0]), pair(wuv_hbm, wuv_v, 0, in_sem.at[0])]
    wq_first = [pair(wq_hbm, wq_v, 0, in_sem.at[1])]
    second = head_pairs(1, 2, in_sem.at[5])
    step0 = head_pairs(2, 3, in_sem.at[2])
    step1 = head_pairs(3, 6, in_sem.at[3]) + out_weights(0, 3, in_sem.at[3])
    step4 = head_pairs(6, PAIRS, in_sem.at[4]) + out_weights(3, PAIRS, in_sem.at[4])
    _start(wkv_first)
    for n in range(GROUPS // STEP):
        _start(c_copies(n))
    _start(wq_first)
    for n in range(GROUPS // STEP):
        _start(x_copies(n) + ([] if n else second))
    _start(step0 + step1 + step4 + later)
    wo_v[0:T, :] = jnp.zeros((T, M), U32)

    def stage(src, hp, r, n):
        k = src.shape[1] // 2
        sums = []
        for odd_row in (0, 1):
            top, low = (src[hp, pl.ds(2 * r + (k0 + odd_row), n, stride=2), :] for k0 in (0, k))
            sums.append(_right(_half(top, 0), _half(top, 1), _half(low, 0), _half(low, 1)))
        return _pack(*sums)

    def stage_q(hp, slot, r, n):
        for t, w in enumerate(stage(wq_v, hp, r, n)):
            wq_r[slot, t, pl.ds(r, n), :] = w

    def stage_kv(hp, slot, which, r, n):
        for t, w in enumerate(stage((wuk_v, wuv_v)[which], hp, r, n)):
            wkv_r[slot, t, pl.ds(r, n), which * D:(which + 1) * D] = w

    def stage_out(slab, unit):
        r, c = unit // 4 * 8, unit % 4 * T
        blocks = [wo_v[_at(slab, T, head * W + r, 8), c0 + c:c0 + c + T]
                  for head in (0, 1) for c0 in (0, M // 2)]
        for t, w in enumerate(_on_words(_right, blocks)):
            wo_r[t, _at(slab, W, r, 8), c:c + T] = w

    def store_q(g, lower, odd, q):
        q_s[odd, _at(g, T, lower * W, W), :] = _riffle(q * Q_SCALE)

    def store_k(g, lower, odd, kv):
        k_s[odd, _at(g, T, lower * W, W), :] = _riffle(kv[:, :D])

    def store_v(g, lower, odd, kv):
        ctx_s[_at(g, T, V_BASE + odd * (S // 2) + lower * W, W), :] = _riffle(kv[:, D:])

    def first_projections(copies, src, left_s, right_s, stores, also):
        def step(n, carry):
            _wait(copies(n))
            for u in range(STEP):
                g = n * STEP + u
                left = _on_words(_left, _quarters(src[_at(g, T, 0, W), :], src[_at(g, T, W, W), :]))
                for t, w in enumerate(left[2:]):
                    left_s[t, _at(g, W), :] = w
                out = _combine([_dot(_bf16(left[t]), _bf16(right_s[0, t])) for t in range(7)])
                for b, y in enumerate(out):
                    for store in stores:
                        store(g, b // 2, b % 2, y)
                also(g)
            return carry

        lax.fori_loop(0, GROUPS // STEP, step, None)

    def stage_part(hp, g, q=True, kv=True):
        size = DC // 4 // GROUPS
        r = pl.multiple_of(g * size, size)
        if q:
            stage_q(hp, hp, 2 * r, 2 * size)
        for which in (0, 1) if kv else ():
            stage_kv(hp, hp, which, r, size)

    _wait(wkv_first)
    pl.loop(0, GROUPS)(functools.partial(stage_part, 0, q=False))
    first_projections(c_copies, c_v, c_l, wkv_r, (store_k, store_v), lambda g: None)
    _wait(wq_first)
    pl.loop(0, GROUPS)(functools.partial(stage_part, 0, kv=False))
    _wait(second)
    first_projections(x_copies, x_v, x_l, wq_r, (store_q,), functools.partial(stage_part, 1))
    _wait(step0)

    def attend(g, lower, odd, fill, v_base):
        tile = 2 * g + lower
        keys = (tile + 1) * W
        s = _tiles(_dot_nt(_bf16(q_s[odd, _at(tile, W), :]), _bf16(k_s[odd, 0:keys, :])))
        s[-1] = jnp.where(_riffled_iota(1) <= _riffled_iota(0), s[-1], NEG)
        top = jnp.max(functools.reduce(jnp.maximum, s), axis=1, keepdims=True)
        top = jnp.broadcast_to(top, (T, T))
        gates = fill()[-3:]
        v = ctx_s[pl.ds(v_base + odd * (S // 2), keys), :]
        total = ctx = None
        for j in range(0, len(s), EXP_TILES):
            at = _after(c_v, gates.pop(0)[:, -T:], top)
            p = [jnp.exp2(a - at) for a in s[j:j + EXP_TILES]]
            total = functools.reduce(jnp.add, p if total is None else [total] + p)
            y = _dot(jnp.concatenate(p, axis=1).astype(BF16),
                     _bf16(v[j * W:(j + len(p)) * W]))
            ctx = y if ctx is None else ctx + y
            gates.append(y)
        return ctx * _reciprocal(jnp.sum(total, axis=1, keepdims=True))

    def head_pair(hp, products, between, done, v_base=V_BASE):
        cuts = (0, 3, 7, 10, 14)
        for g in reversed(range(GROUPS)):
            todo, m, ctx = products(g), [], {}
            for b, (lower, odd) in enumerate(((1, 0), (1, 1), (0, 0), (0, 1))):
                def fill():
                    between(4 * g + b)
                    m.extend(f() for f in todo[cuts[b]:cuts[b + 1]])
                    done(g, b, m, False)
                    return m[cuts[b]:]

                ctx[lower, odd] = attend(g, lower, odd, fill, v_base)
                done(g, b, m, True)
                left = _left(*[ctx.get(k, ctx[1, 0]) for k in ((0, 0), (0, 1), (1, 0), (1, 1))])
                for t in ((), (1, 3), (0, 2, 5), (4, 6))[b]:
                    ctx_s[_ctx_rows(hp, t, g), :] = _riffle(left[t])

    def pair_step(hp, carry):
        pl.when(hp == 1)(lambda: _wait(step1))
        pl.when(hp == 4)(lambda: _wait(step4))
        slot = (hp + 1) % 2
        held = {}

        def products(g):
            def product(src, sums, right, t):
                k = sums.shape[2]
                left = sums[t - 2, _at(g, W), :] if t >= 2 else src[_at(2 * g + t, W), pl.ds(t * k, k)]
                return _dot(_bf16(left), _bf16(right[slot, t]))

            return [functools.partial(product, *refs, t)
                    for refs in ((x_v, x_l, wq_r), (c_v, c_l, wkv_r)) for t in range(7)]

        def between(unit):
            ahead = jnp.minimum(hp + 2, PAIRS - 1)
            stage_q(ahead, 1 - slot, unit * 8, 8)
            stage_kv(ahead, 1 - slot, unit % 2, unit // 2 * 8, 8)
            stage_out(hp, unit)

        def done(g, b, m, attended):
            if (b, attended) == (1, False):
                held["q"] = _combine(m[:7])
                for odd in (0, 1):
                    store_q(g, 1, odd, held["q"][2 + odd])
            if b >= 2 and not attended:
                store_q(g, 0, b - 2, held["q"][b - 2])
            if (b, attended) == (3, False):
                held["kv"] = _combine(m[7:])
                for n, y in enumerate(held["kv"]):
                    store_k(g, n // 2, n % 2, y)
                    if n != 1:
                        store_v(g, n // 2, n % 2, y)
            if (b, attended) == (3, True):
                store_v(g, 0, 1, held["kv"][1])

        head_pair(hp, products, between, done)
        return carry + V_BASE // (PAIRS - 1)

    v_base = lax.fori_loop(0, PAIRS - 1, pair_step, V_BASE % (PAIRS - 1))

    prepare()

    def early(g):
        return [functools.partial(_project_out, ctx_s, wo_r, g, t, 0, EARLY, pl.ds(c, M // 4))
                for t in range(7) for c in (0, M // 4)]

    def early_done(g, b, m, attended):
        if (b, attended) == (3, False):
            halves = [_combine(m[c::2]) for c in (0, 1)]
            for n in range(4):
                for c in (0, 1):
                    c0 = n % 2 * (M // 2) + c * (M // 4)
                    part_s[_at(2 * g + n // 2, T), c0:c0 + M // 4] += halves[c][n]

    def last_weights(unit):
        for slab in (PAIRS - 1, PAIRS):
            stage_out(slab, unit)

    @pl.loop(V_BASE, v_base + 1)
    def _(base):
        head_pair(PAIRS - 1, early, last_weights, early_done, pl.multiple_of(base, W))


def _outputs(out_hbm, ctx_s, wo_r, part_s, bx_v, wqkv_r, bwo_r, bk_s, bv_s, out_s, out_sem):
    after = functools.partial(_after, bx_v)
    for j in range(NB):
        bk_s[j, 0:HALO, :] = jnp.zeros((HALO, T), F32)
        bv_s[j, 0:HALO, :] = jnp.zeros((HALO, T), F32)

    def b_proj(left, right):
        m = [_dot(left[t], _bf16(right[t])) for t in range(7)]
        c11, c12, c21, c22 = _combine(m)
        return m, jnp.concatenate(
            [jnp.concatenate([c11, c12], axis=1), jnp.concatenate([c21, c22], axis=1)], axis=0)

    def b_weights(pos, r, q, gate):
        logits = [None] * WIN
        for j, qj in enumerate(_tiles(q[r:r + G])):
            qj = after(gate[j * G:(j + 1) * G], qj) * (DH ** -0.5 * LOG2E)
            for w in range(WIN):
                t = qj * bk_s[j, pl.ds(HALO + r - DIL * w, G), :]
                logits[w] = t if logits[w] is None else logits[w] + t
        for w in range(WIN):
            t = logits[w] + pltpu.roll(logits[w], 64, 1)
            t = t + pltpu.roll(t, 32, 1)
            if r < DIL * w:
                t = jnp.where(pos + r + lax.broadcasted_iota(I32, (G, T), 0) >= DIL * w, t, NEG)
            logits[w] = t
        top = functools.reduce(jnp.maximum, logits)
        e = [jnp.exp2(t - top) for t in logits]
        inv = _reciprocal(functools.reduce(jnp.add, e))
        return [t * inv for t in e]

    def b_mix(r, attn, gate):
        acc = [None] * NB
        for w in range(WIN):
            a = after(gate[w * G:(w + 1) * G], attn[w])
            for j in range(NB):
                t = a * bv_s[j, pl.ds(HALO + r - DIL * w, G), :]
                acc[j] = t if acc[j] is None else acc[j] + t
        return _unshuffle(acc)

    def out_copy(g, branch):
        cols = pl.ds(branch * M, M)
        return pltpu.make_async_copy(
            out_s.at[g % 2, :, cols], out_hbm.at[_at(g, 2 * T), cols], out_sem.at[g % 2, branch])

    def group(g, carry):
        pl.when(g >= 2)(lambda: _wait([out_copy(g - 2, 0), out_copy(g - 2, 1)]))
        xs = _on_words(_left, _quarters(bx_v[_at(g, T, 0, W), :], bx_v[_at(g, T, W, W), :]))
        xs = [_bf16(a) for a in xs]
        _, k = b_proj(xs, wqkv_r.at[1])
        for j, t in enumerate(_tiles(k)):
            bk_s[j, HALO:, :] = t
        _, q = b_proj(xs, wqkv_r.at[0])
        m, v = b_proj(xs, wqkv_r.at[2])
        for j, t in enumerate(_tiles(v)):
            bv_s[j, HALO:, :] = t
        gates = [t for y in m for t in _tiles(y)[1::2]]
        m = [_project_out(ctx_s, wo_r, g, t, LATE, PAIRS) for t in range(7)]
        gates += [t for y in m for t in _tiles(y)]
        rows = range(0, 2 * T, G)
        attn = [b_weights(g * (2 * T), r, q, gates[n]) for n, r in enumerate(rows)]
        o = jnp.concatenate(
            [b_mix(r, attn[n], gates[len(rows) + 1 + n]) for n, r in enumerate(rows)], axis=0)
        for n, (at, y) in enumerate(zip(_out_blocks(g), _combine(m))):
            y = _bf16(_riffle(part_s[at] + y)).astype(F32)
            out_s[g % 2, _at(n // 2, T), at[1]] = _bf16(_riffle(y))
        out_copy(g, 0).start()
        _, y = b_proj([a.astype(BF16) for a in _left(*_quarters(o[:T], o[T:]))], bwo_r)
        out_s[g % 2, :, M:] = y.astype(BF16)
        for j in range(NB):
            bk_s[j, 0:HALO, :] = bk_s[j, 2 * T:, :]
            bv_s[j, 0:HALO, :] = bv_s[j, 2 * T:, :]
        out_copy(g, 1).start()
        return carry

    lax.fori_loop(0, GROUPS, group, None)
    for g in range(GROUPS - 2, GROUPS):
        _wait([out_copy(g, 0), out_copy(g, 1)])


def _kernel(x_hbm, c_hbm, wq_hbm, wuk_hbm, wuv_hbm, wo_hbm, bx_hbm, wqkv_hbm, bwo_hbm,
            out_hbm, ctx_s, wo_r, part_s, bx_v, wqkv_v, bwo_v, wqkv_r, bwo_r, later_sem):
    later = [_rows(src, dst, slice(None), later_sem)
             for src, dst in ((bx_hbm, bx_v), (wqkv_hbm, wqkv_v), (bwo_hbm, bwo_v))]
    prepare = functools.partial(_prepare, later, ctx_s, wo_r, part_s, wqkv_v, bwo_v, wqkv_r, bwo_r)
    pl.run_scoped(
        functools.partial(_attention, x_hbm, c_hbm, wq_hbm, wuk_hbm, wuv_hbm, wo_hbm, later,
                          prepare, ctx_s, wo_r, part_s),
        pltpu.VMEM((S // 2, M), U32),
        pltpu.VMEM((S // 2, DC), U32),
        pltpu.VMEM((PAIRS, M, D), U32),
        pltpu.VMEM((PAIRS, DC, D), U32),
        pltpu.VMEM((PAIRS, DC, D), U32),
        pltpu.VMEM(((PAIRS + 1) * T, M), U32),
        pltpu.VMEM((5, S // 4, M // 2), U32),
        pltpu.VMEM((5, S // 4, DC // 2), U32),
        pltpu.VMEM((2, 7, M // 4, D), U32),
        pltpu.VMEM((2, 7, DC // 4, 2 * D), U32),
        pltpu.VMEM((2, S // 2, D), U32),
        pltpu.VMEM((2, S // 2, D), U32),
        pltpu.SemaphoreType.DMA((GROUPS // STEP,)),
        pltpu.SemaphoreType.DMA((GROUPS // STEP,)),
        pltpu.SemaphoreType.DMA((6,)),
    )
    pl.run_scoped(
        functools.partial(_outputs, out_hbm, ctx_s, wo_r, part_s, bx_v, wqkv_r, bwo_r),
        pltpu.VMEM((NB, HALO + 2 * T, T), F32),
        pltpu.VMEM((NB, HALO + 2 * T, T), F32),
        pltpu.VMEM((2, 2 * T, M + DB), BF16),
        pltpu.SemaphoreType.DMA((2, 2)),
    )


@jax.jit
def pallas_concat_heads__compressed_kv_cla__sliding_local_dilated__prompt_kernel(
    A_x: jax.Array,
    A_c_kv: jax.Array,
    A_w_q: jax.Array,
    A_w_uk: jax.Array,
    A_w_uv: jax.Array,
    A_w_o: jax.Array,
    B_x: jax.Array,
    B_wqkv: jax.Array,
    B_wo: jax.Array,
):
    out = pl.pallas_call(
        _kernel,
        out_shape=jax.ShapeDtypeStruct((S, M + DB), BF16),
        in_specs=[pl.BlockSpec(memory_space=pl.ANY)] * 9,
        out_specs=pl.BlockSpec(memory_space=pl.ANY),
        scratch_shapes=[
            pltpu.VMEM((V_BASE + S, D), U32),
            pltpu.VMEM((7, (PAIRS + 1) * W, M // 2), U32),
            pltpu.VMEM((S, M), F32),
            pltpu.VMEM((S // 2, DB), U32),
            pltpu.VMEM((DB // 2, 3 * DB), U32),
            pltpu.VMEM((DB // 2, DB), U32),
            pltpu.VMEM((3, 7, DB // 4, DB // 2), U32),
            pltpu.VMEM((7, DB // 4, DB // 2), U32),
            pltpu.SemaphoreType.DMA,
        ],
        compiler_params=pltpu.CompilerParams(vmem_limit_bytes=126 * 1024 * 1024),
        name="mla_local_concat",
    )(
        A_x.reshape(S, M),
        A_c_kv.reshape(S, DC),
        A_w_q.reshape(M, PAIRS, 2, D),
        A_w_uk.reshape(DC, PAIRS, 2, D),
        A_w_uv.reshape(DC, PAIRS, 2, D),
        A_w_o.reshape(H * D, M),
        B_x.reshape(S, DB),
        B_wqkv,
        B_wo,
    )
    return out.reshape(1, S, M + DB)
```

```python
import functools
import math

import jax
import jax.numpy as jnp
from jax import lax
import jax.experimental.pallas as pl
import jax.experimental.pallas.tpu as pltpu

BF16 = jnp.bfloat16
F32 = jnp.float32
U32 = jnp.uint32
I32 = jnp.int32

T = 128
W = T // 2
G = 16
LOG2E = math.log2(math.e)
NEG = -1e9 * LOG2E

S = 2048
GROUPS = S // (2 * T)
M = 1024
H = 32
D = 128
DC = 512
PAIRS = H // 2
Q_SCALE = D ** -0.5 * LOG2E
STEP = 2
EXP_TILES = 4
EARLY = (4, 8)
MQ = M // 4
DB = 1024
DH = 32
NB = DB // T
WIN = 8
DIL = 2
HALO = 16


def _bf16(words):
    return pltpu.bitcast(words, BF16)


def _riffle(val):
    halves = [jnp.concatenate([val[r + b:r + b + 8] for r in range(0, val.shape[0], G)], axis=0)
              for b in (0, 8)]
    return pltpu.pack_elementwise(halves, packed_dtype=BF16)


def _riffled_iota(axis):
    i = lax.broadcasted_iota(I32, (T, T), axis)
    return (i & ~15) | ((i & 1) << 3) | ((i & 15) >> 1)


def _reciprocal(x):
    r = pl.reciprocal(x, approx=True)
    return r * (2.0 - x * r)


def _dot(a, b):
    return lax.dot_general(a, b, (((1,), (0,)), ((), ())), preferred_element_type=F32)


def _dot_nt(a, b):
    return lax.dot_general(a, b, (((1,), (1,)), ((), ())), preferred_element_type=F32)


def _at(n, size, offset=0, count=None):
    start = n * size if isinstance(n, int) else pl.multiple_of(n * size, size)
    return pl.ds(start + offset, size if count is None else count)


def _left(a11, a12, a21, a22):
    return [a11, a22, a11 + a22, a21 + a22, a11 + a12, a21 - a11, a12 - a22]


def _right(b11, b12, b21, b22):
    return [b12 - b22, b21 - b11, b11 + b22, b11, b22, b11 + b12, b21 + b22]


def _combine(m):
    return m[1] + m[2] - m[4] + m[6], m[0] + m[4], m[1] + m[3], m[0] + m[2] - m[3] + m[5]


def _half(words, index):
    return pltpu.unpack_elementwise(words, index=index, packed_dtype=BF16, unpacked_dtype=F32)


def _pack(lows, highs):
    return [pltpu.pack_elementwise([lo, hi], packed_dtype=BF16) for lo, hi in zip(lows, highs)]


def _on_words(sums, blocks):
    return _pack(*[sums(*[_half(b, index) for b in blocks]) for index in (0, 1)])


def _quarters(upper, lower):
    n = upper.shape[1] // 2
    return upper[:, :n], upper[:, n:], lower[:, :n], lower[:, n:]


def _exchange(tiles):
    lane = lax.broadcasted_iota(I32, tiles[0].shape, 1)
    for bit in (1, 2, 4):
        pick = (lane & bit) != 0
        tiles = [jnp.where(pick, tiles[k ^ bit], tiles[k]) for k in range(NB)]
    return tiles


def _permute_lanes(tiles):
    lane = lax.broadcasted_iota(I32, (8, T), 1)
    base = ((lane >> 2) & 0x18) | ((lane << 2) & 0x60) | (lane & 7)
    return [
        jnp.concatenate(
            [jnp.take_along_axis(t[r:r + 8], base ^ k, axis=1) for r in range(0, t.shape[0], 8)],
            axis=0)
        for k, t in enumerate(tiles)
    ]


def _tiles(a):
    return [a[:, c:c + T] for c in range(0, a.shape[1], T)]


def _shuffle(tiles):
    return jnp.concatenate(_permute_lanes(_exchange(tiles)), axis=1)


def _unshuffle(tiles):
    return jnp.concatenate(_exchange(_permute_lanes(tiles)), axis=1)


def _start(copies):
    for cp in copies:
        cp.start()


def _wait(copies):
    for cp in copies:
        cp.wait()


def _rows(src, dst, rows, sem):
    return pltpu.make_async_copy(src.bitcast(U32).at[rows], dst.at[rows], sem)


def _after(words, src, val):
    nonneg = pltpu.bitcast(words[0:8, 0:T] >> 1, I32)
    return jnp.where(jnp.tile(nonneg, (val.shape[0] // 8, 1)) < 0, src, val)


V_BASE = PAIRS * 7 * GROUPS * W


def _ctx_rows(hp, t, g):
    return _at((hp * 7 + t) * GROUPS + g, W)


def _project_out(ctx_s, wo_r, g, t, p0, p1, cols):
    ctx = jnp.concatenate([ctx_s[_ctx_rows(hp, t, g), :] for hp in range(p0, p1)], axis=1)
    return _dot(_bf16(ctx), _bf16(wo_r[t, (p0 + 1) * W:(p1 + 1) * W, cols]))


def _out_blocks(g, c0, width):
    return [(_at(2 * g + n // 2, T), pl.ds(n % 2 * (M // 2) + c0, width)) for n in range(4)]


def _prepare(later, ctx_s, wo_r, part_s, wqkv_v, bwo_v, wqkv_r, bwo_r):
    after = functools.partial(_after, bwo_v)
    _wait(later)

    def prepare(i, carry):
        for u in range(2):
            g = 2 * i + u
            m = [_project_out(ctx_s, wo_r, g, t, 0, EARLY[1], pl.ds(MQ, MQ)) for t in range(7)]
            for at, y in zip(_out_blocks(g, MQ, MQ), _combine(m)):
                part_s[at] = y
            size = DB // 4 // GROUPS
            for n in range(6):
                which, r = n // 2, n % 2 * (size // 2)
                w = jnp.concatenate(
                    [wqkv_v[_at(g, size, k0 + r, size // 2), which * DB:(which + 1) * DB]
                     for k0 in (0, DB // 4)], axis=0)
                gate = pltpu.bitcast(m[n][:size, :T], U32)
                w = _shuffle([after(gate, a) for a in _tiles(w)])
                for t, a in enumerate(_on_words(_right, _quarters(w[:size // 2], w[size // 2:]))):
                    wqkv_r[which, t, _at(g, size, r, size // 2), :] = a
            for n, r in enumerate(range(0, size, 8)):
                gate = pltpu.bitcast(m[n][:8, T:], U32)
                w = [jnp.concatenate(
                    [after(gate, a) for a in _tiles(bwo_v[_at(g, size, k0 + r, 8), :])], axis=1)
                    for k0 in (0, DB // 4)]
                for t, a in enumerate(_on_words(_right, _quarters(*w))):
                    bwo_r[t, _at(g, size, r, 8), :] = a
        return carry

    lax.fori_loop(0, GROUPS // 2, prepare, None)

def _attention(x_hbm, c_hbm, wq_hbm, wuk_hbm, wuv_hbm, wo_hbm, later, prepare,
               ctx_s, wo_r, part_s, x_v, c_v, wq_v, wuk_v, wuv_v, wo_v, x_l, c_l, wq_r, wkv_r, q_s, k_s,
               c_sem, x_sem, in_sem):
    def pair(src, dst, hp, sem):
        return pltpu.make_async_copy(src.bitcast(U32).at[:, hp, 0], dst.at[hp], sem)

    def head_pairs(p0, p1, sem):
        return [pair(src, dst, hp, sem) for hp in range(p0, p1)
                for src, dst in ((wq_hbm, wq_v), (wuk_hbm, wuk_v), (wuv_hbm, wuv_v))]

    def out_weights(p0, p1, sem):
        return [_rows(wo_hbm, wo_v.at[pl.ds(T, PAIRS * T)], pl.ds(p0 * T, (p1 - p0) * T), sem)]

    def c_copies(n):
        return [_rows(c_hbm, c_v, _at(n, STEP * T), c_sem.at[n])]

    def x_copies(n):
        return [_rows(x_hbm, x_v, _at(n, STEP * T), x_sem.at[n])]

    wkv_first = [pair(wuk_hbm, wuk_v, 0, in_sem.at[0]), pair(wuv_hbm, wuv_v, 0, in_sem.at[0])]
    wq_first = [pair(wq_hbm, wq_v, 0, in_sem.at[1])]
    second = head_pairs(1, 2, in_sem.at[5])
    step0 = head_pairs(2, 3, in_sem.at[2])
    step1 = head_pairs(3, 6, in_sem.at[3]) + out_weights(0, 3, in_sem.at[3])
    step4 = head_pairs(6, PAIRS, in_sem.at[4]) + out_weights(3, PAIRS, in_sem.at[4])
    _start(wkv_first)
    for n in range(GROUPS // STEP):
        _start(c_copies(n))
    _start(wq_first)
    for n in range(GROUPS // STEP):
        _start(x_copies(n) + ([] if n else second))
    _start(step0 + step1 + step4 + later)
    wo_v[0:T, :] = jnp.zeros((T, M), U32)

    def stage(src, hp, r, n):
        k = src.shape[1] // 2
        sums = []
        for odd_row in (0, 1):
            top, low = (src[hp, pl.ds(2 * r + (k0 + odd_row), n, stride=2), :] for k0 in (0, k))
            sums.append(_right(_half(top, 0), _half(top, 1), _half(low, 0), _half(low, 1)))
        return _pack(*sums)

    def stage_q(hp, slot, r, n):
        words = stage(wq_v, hp, r, n)
        for t, w in enumerate(words):
            wq_r[slot, t, pl.ds(r, n), :] = w
        return words

    def stage_kv(hp, slot, which, r, n):
        words = stage((wuk_v, wuv_v)[which], hp, r, n)
        for t, w in enumerate(words):
            wkv_r[slot, t, pl.ds(r, n), which * D:(which + 1) * D] = w
        return words

    def stage_out(slab, unit):
        r, c = unit // 4 * 8, unit % 4 * T
        blocks = [wo_v[_at(slab, T, head * W + r, 8), c0 + c:c0 + c + T]
                  for head in (0, 1) for c0 in (0, M // 2)]
        words = _on_words(_right, blocks)
        for t, w in enumerate(words):
            wo_r[t, _at(slab, W, r, 8), c:c + T] = w
        return words

    def store_q(g, lower, odd, q):
        q_s[odd, _at(g, T, lower * W, W), :] = _riffle(q * Q_SCALE)

    def store_k(g, lower, odd, kv):
        k_s[odd, _at(g, T, lower * W, W), :] = _riffle(kv[:, :D])

    def store_v(g, lower, odd, kv):
        ctx_s[_at(g, T, V_BASE + odd * (S // 2) + lower * W, W), :] = _riffle(kv[:, D:])

    def first_projections(copies, src, left_s, right_s, stores, also):
        def step(n, carry):
            _wait(copies(n))
            for u in range(STEP):
                g = n * STEP + u
                left = _on_words(_left, _quarters(src[_at(g, T, 0, W), :], src[_at(g, T, W, W), :]))
                for t, w in enumerate(left[2:]):
                    left_s[t, _at(g, W), :] = w
                out = _combine([_dot(_bf16(left[t]), _bf16(right_s[0, t])) for t in range(7)])
                for b, y in enumerate(out):
                    for store in stores:
                        store(g, b // 2, b % 2, y)
                also(g)
            return carry

        lax.fori_loop(0, GROUPS // STEP, step, None)

    def stage_part(hp, g, q=True, kv=True):
        size = DC // 4 // GROUPS
        r = pl.multiple_of(g * size, size)
        if q:
            stage_q(hp, hp, 2 * r, 2 * size)
        for which in (0, 1) if kv else ():
            stage_kv(hp, hp, which, r, size)

    _wait(wkv_first)
    pl.loop(0, GROUPS)(functools.partial(stage_part, 0, q=False))
    first_projections(c_copies, c_v, c_l, wkv_r, (store_k, store_v), lambda g: None)
    _wait(wq_first)
    pl.loop(0, GROUPS)(functools.partial(stage_part, 0, kv=False))
    _wait(second)
    first_projections(x_copies, x_v, x_l, wq_r, (store_q,), functools.partial(stage_part, 1))
    _wait(step0)

    def attend(g, lower, odd, chores, fill, v_base):
        tile = 2 * g + lower
        keys = (tile + 1) * W
        s = _tiles(_dot_nt(_bf16(q_s[odd, _at(tile, W), :]), _bf16(k_s[odd, 0:keys, :])))
        s[-1] = jnp.where(_riffled_iota(1) <= _riffled_iota(0), s[-1], NEG)
        top = functools.reduce(jnp.maximum, s)
        top = [top[r:r + 8] for r in range(0, T, 8)]
        for n, w in enumerate(chores):
            top[n % len(top)] = _after(c_v, pltpu.bitcast(w, F32), top[n % len(top)])
        top = jnp.max(jnp.concatenate(top, axis=0), axis=1, keepdims=True)
        top = jnp.broadcast_to(top, (T, T))
        gates = fill()[-3:]
        v = ctx_s[pl.ds(v_base + odd * (S // 2), keys), :]
        total = ctx = None
        for j in range(0, len(s), EXP_TILES):
            at = _after(c_v, gates.pop(0)[:, -T:], top)
            p = [jnp.exp2(a - at) for a in s[j:j + EXP_TILES]]
            total = functools.reduce(jnp.add, p if total is None else [total] + p)
            y = _dot(jnp.concatenate(p, axis=1).astype(BF16),
                     _bf16(v[j * W:(j + len(p)) * W]))
            ctx = y if ctx is None else ctx + y
            gates.append(y)
        return ctx * _reciprocal(jnp.sum(total, axis=1, keepdims=True))

    def head_pair(hp, products, chores, done, v_base=V_BASE):
        cuts = (0, 3, 7, 10, 14)
        for g in reversed(range(GROUPS)):
            todo, m, ctx = products(g), [], {}
            for b, (lower, odd) in enumerate(((1, 0), (1, 1), (0, 0), (0, 1))):
                def fill():
                    m.extend(f() for f in todo[cuts[b]:cuts[b + 1]])
                    done(g, b, m, False)
                    return m[cuts[b]:]

                ctx[lower, odd] = attend(g, lower, odd, chores(4 * g + b), fill, v_base)
                done(g, b, m, True)
                left = _left(*[ctx.get(k, ctx[1, 0]) for k in ((0, 0), (0, 1), (1, 0), (1, 1))])
                for t in ((), (1, 3), (0, 2, 5), (4, 6))[b]:
                    ctx_s[_ctx_rows(hp, t, g), :] = _riffle(left[t])

    def pair_step(hp, carry):
        pl.when(hp == 1)(lambda: _wait(step1))
        pl.when(hp == 4)(lambda: _wait(step4))
        slot = (hp + 1) % 2
        held = {}

        def products(g):
            def product(src, sums, right, t):
                k = sums.shape[2]
                left = sums[t - 2, _at(g, W), :] if t >= 2 else src[_at(2 * g + t, W), pl.ds(t * k, k)]
                return _dot(_bf16(left), _bf16(right[slot, t]))

            return [functools.partial(product, *refs, t)
                    for refs in ((x_v, x_l, wq_r), (c_v, c_l, wkv_r)) for t in range(7)]

        def chores(unit):
            ahead = jnp.minimum(hp + 2, PAIRS - 1)
            stage_out(hp, unit)
            words = zip(stage_q(ahead, 1 - slot, unit * 8, 8),
                        stage_kv(ahead, 1 - slot, unit % 2, unit // 2 * 8, 8))
            return [w for group in words for w in group]

        def done(g, b, m, attended):
            if (b, attended) == (1, False):
                held["q"] = _combine(m[:7])
                for odd in (0, 1):
                    store_q(g, 1, odd, held["q"][2 + odd])
            if b >= 2 and not attended:
                store_q(g, 0, b - 2, held["q"][b - 2])
            if (b, attended) == (3, False):
                held["kv"] = _combine(m[7:])
                for n, y in enumerate(held["kv"]):
                    store_k(g, n // 2, n % 2, y)
                    if n != 1:
                        store_v(g, n // 2, n % 2, y)
            if (b, attended) == (3, True):
                store_v(g, 0, 1, held["kv"][1])

        head_pair(hp, products, chores, done)
        return carry + V_BASE // (PAIRS - 1)

    v_base = lax.fori_loop(0, PAIRS - 1, pair_step, V_BASE % (PAIRS - 1))

    prepare()

    def early(g):
        return [functools.partial(_project_out, ctx_s, wo_r, g, t, 0, EARLY[0], pl.ds(c0, T))
                for c0 in (0, T) for t in range(7)]

    def early_done(g, b, m, attended):
        if b % 2 and not attended:
            for at, y in zip(_out_blocks(g, b // 2 * T, T), _combine(m[-7:])):
                part_s[at] = y

    def last_weights(unit):
        return stage_out(PAIRS - 1, unit) + stage_out(PAIRS, unit)

    @pl.loop(V_BASE, v_base + 1)
    def _(base):
        head_pair(PAIRS - 1, early, last_weights, early_done, pl.multiple_of(base, W))


def _outputs(out_hbm, ctx_s, wo_r, part_s, bx_v, wqkv_r, bwo_r, bk_s, bv_s, out_s, out_sem):
    after = functools.partial(_after, bx_v)
    for j in range(NB):
        bk_s[j, 0:HALO, :] = jnp.zeros((HALO, T), F32)
        bv_s[j, 0:HALO, :] = jnp.zeros((HALO, T), F32)

    def b_proj(left, right):
        m = [_dot(left[t], _bf16(right[t])) for t in range(7)]
        c11, c12, c21, c22 = _combine(m)
        return m, jnp.concatenate(
            [jnp.concatenate([c11, c12], axis=1), jnp.concatenate([c21, c22], axis=1)], axis=0)

    def b_weights(pos, r, q, gate):
        logits = [None] * WIN
        for j, qj in enumerate(_tiles(q[r:r + G])):
            qj = after(gate[j * G:(j + 1) * G], qj) * (DH ** -0.5 * LOG2E)
            for w in range(WIN):
                t = qj * bk_s[j, pl.ds(HALO + r - DIL * w, G), :]
                logits[w] = t if logits[w] is None else logits[w] + t
        for w in range(WIN):
            t = logits[w] + pltpu.roll(logits[w], 64, 1)
            t = t + pltpu.roll(t, 32, 1)
            if r < DIL * w:
                t = jnp.where(pos + r + lax.broadcasted_iota(I32, (G, T), 0) >= DIL * w, t, NEG)
            logits[w] = t
        top = functools.reduce(jnp.maximum, logits)
        e = [jnp.exp2(t - top) for t in logits]
        inv = _reciprocal(functools.reduce(jnp.add, e))
        return [t * inv for t in e]

    def b_mix(r, attn, gate):
        acc = [None] * NB
        for w in range(WIN):
            a = after(gate[w * G:(w + 1) * G], attn[w])
            for j in range(NB):
                t = a * bv_s[j, pl.ds(HALO + r - DIL * w, G), :]
                acc[j] = t if acc[j] is None else acc[j] + t
        return _unshuffle(acc)

    def out_copy(g, r0, rows, c0, cols):
        return pltpu.make_async_copy(
            out_s.at[g % 2, pl.ds(r0, rows), pl.ds(c0, cols)],
            out_hbm.at[_at(g, 2 * T, r0, rows), pl.ds(c0, cols)], out_sem.at[g % 2])

    def out_wait(g):
        out_copy(g, 0, 2 * T, 0, M + DB).wait()

    def group(g, carry):
        pl.when(g >= 2)(lambda: out_wait(g - 2))
        xs = _on_words(_left, _quarters(bx_v[_at(g, T, 0, W), :], bx_v[_at(g, T, W, W), :]))
        xs = [_bf16(a) for a in xs]
        _, k = b_proj(xs, wqkv_r.at[1])
        for j, t in enumerate(_tiles(k)):
            bk_s[j, HALO:, :] = t
        _, q = b_proj(xs, wqkv_r.at[0])
        m, v = b_proj(xs, wqkv_r.at[2])
        for j, t in enumerate(_tiles(v)):
            bv_s[j, HALO:, :] = t
        gates = [t for y in m for t in _tiles(y)[1::2]]
        late = [[_project_out(ctx_s, wo_r, g, t, EARLY[c], PAIRS, pl.ds(c * MQ, MQ))
                 for t in range(7)] for c in (0, 1)]
        gates += [t for m in late for y in m for t in _tiles(y)]
        rows = range(0, 2 * T, G)
        attn = [b_weights(g * (2 * T), r, q, gates[n]) for n, r in enumerate(rows)]
        o = jnp.concatenate(
            [b_mix(r, attn[n], gates[len(rows) + 1 + n]) for n, r in enumerate(rows)], axis=0)
        for c, m in enumerate(late):
            for n, (at, y) in enumerate(zip(_out_blocks(g, c * MQ, MQ), _combine(m))):
                y = _bf16(_riffle(part_s[at] + y)).astype(F32)
                out_s[g % 2, _at(n // 2, T), at[1]] = _bf16(_riffle(y))
        out_copy(g, 0, 2 * T, 0, M).start()
        for j in range(NB):
            bk_s[j, 0:HALO, :] = bk_s[j, 2 * T:, :]
            bv_s[j, 0:HALO, :] = bv_s[j, 2 * T:, :]
        m, _ = b_proj([a.astype(BF16) for a in _left(*_quarters(o[:T], o[T:]))], bwo_r)
        y = _combine(m)
        for n in (2, 1, 3, 0):
            r0, c0 = n // 2 * T, M + n % 2 * (DB // 2)
            out_s[g % 2, r0:r0 + T, c0:c0 + DB // 2] = y[n].astype(BF16)
            out_copy(g, r0, T, c0, DB // 2).start()
        return carry

    lax.fori_loop(0, GROUPS, group, None)
    for g in range(GROUPS - 2, GROUPS):
        out_wait(g)


def _kernel(x_hbm, c_hbm, wq_hbm, wuk_hbm, wuv_hbm, wo_hbm, bx_hbm, wqkv_hbm, bwo_hbm,
            out_hbm, ctx_s, wo_r, part_s, bx_v, wqkv_v, bwo_v, wqkv_r, bwo_r, later_sem):
    later = [_rows(src, dst, slice(None), later_sem)
             for src, dst in ((bx_hbm, bx_v), (wqkv_hbm, wqkv_v), (bwo_hbm, bwo_v))]
    prepare = functools.partial(_prepare, later, ctx_s, wo_r, part_s, wqkv_v, bwo_v, wqkv_r, bwo_r)
    pl.run_scoped(
        functools.partial(_attention, x_hbm, c_hbm, wq_hbm, wuk_hbm, wuv_hbm, wo_hbm, later,
                          prepare, ctx_s, wo_r, part_s),
        pltpu.VMEM((S // 2, M), U32),
        pltpu.VMEM((S // 2, DC), U32),
        pltpu.VMEM((PAIRS, M, D), U32),
        pltpu.VMEM((PAIRS, DC, D), U32),
        pltpu.VMEM((PAIRS, DC, D), U32),
        pltpu.VMEM(((PAIRS + 1) * T, M), U32),
        pltpu.VMEM((5, S // 4, M // 2), U32),
        pltpu.VMEM((5, S // 4, DC // 2), U32),
        pltpu.VMEM((2, 7, M // 4, D), U32),
        pltpu.VMEM((2, 7, DC // 4, 2 * D), U32),
        pltpu.VMEM((2, S // 2, D), U32),
        pltpu.VMEM((2, S // 2, D), U32),
        pltpu.SemaphoreType.DMA((GROUPS // STEP,)),
        pltpu.SemaphoreType.DMA((GROUPS // STEP,)),
        pltpu.SemaphoreType.DMA((6,)),
    )
    pl.run_scoped(
        functools.partial(_outputs, out_hbm, ctx_s, wo_r, part_s, bx_v, wqkv_r, bwo_r),
        pltpu.VMEM((NB, HALO + 2 * T, T), F32),
        pltpu.VMEM((NB, HALO + 2 * T, T), F32),
        pltpu.VMEM((2, 2 * T, M + DB), BF16),
        pltpu.SemaphoreType.DMA((2,)),
    )


@jax.jit
def pallas_concat_heads__compressed_kv_cla__sliding_local_dilated__prompt_kernel(
    A_x: jax.Array,
    A_c_kv: jax.Array,
    A_w_q: jax.Array,
    A_w_uk: jax.Array,
    A_w_uv: jax.Array,
    A_w_o: jax.Array,
    B_x: jax.Array,
    B_wqkv: jax.Array,
    B_wo: jax.Array,
):
    out = pl.pallas_call(
        _kernel,
        out_shape=jax.ShapeDtypeStruct((S, M + DB), BF16),
        in_specs=[pl.BlockSpec(memory_space=pl.ANY)] * 9,
        out_specs=pl.BlockSpec(memory_space=pl.ANY),
        scratch_shapes=[
            pltpu.VMEM((V_BASE + S, D), U32),
            pltpu.VMEM((7, (PAIRS + 1) * W, M // 2), U32),
            pltpu.VMEM((S, M), F32),
            pltpu.VMEM((S // 2, DB), U32),
            pltpu.VMEM((DB // 2, 3 * DB), U32),
            pltpu.VMEM((DB // 2, DB), U32),
            pltpu.VMEM((3, 7, DB // 4, DB // 2), U32),
            pltpu.VMEM((7, DB // 4, DB // 2), U32),
            pltpu.SemaphoreType.DMA,
        ],
        compiler_params=pltpu.CompilerParams(vmem_limit_bytes=126 * 1024 * 1024),
        name="mla_local_concat",
    )(
        A_x.reshape(S, M),
        A_c_kv.reshape(S, DC),
        A_w_q.reshape(M, PAIRS, 2, D),
        A_w_uk.reshape(DC, PAIRS, 2, D),
        A_w_uv.reshape(DC, PAIRS, 2, D),
        A_w_o.reshape(H * D, M),
        B_x.reshape(S, DB),
        B_wqkv,
        B_wo,
    )
    return out.reshape(1, S, M + DB)
```

```python
import functools
import math

import jax
import jax.numpy as jnp
from jax import lax
import jax.experimental.pallas as pl
import jax.experimental.pallas.tpu as pltpu

BF16 = jnp.bfloat16
F32 = jnp.float32
U32 = jnp.uint32
I32 = jnp.int32

T = 128
W = T // 2
G = 16
LOG2E = math.log2(math.e)
NEG = -1e9 * LOG2E

S = 2048
GROUPS = S // (2 * T)
M = 1024
H = 32
D = 128
DC = 512
PAIRS = H // 2
Q_SCALE = D ** -0.5 * LOG2E
STEP = 2
EXP_TILES = 4
EARLY = (4, 5)
MQ = M // 4
DB = 1024
DH = 32
NB = DB // T
WIN = 8
DIL = 2
HALO = 16


def _bf16(words):
    return pltpu.bitcast(words, BF16)


def _riffle(val):
    halves = [jnp.concatenate([val[r + b:r + b + 8] for r in range(0, val.shape[0], G)], axis=0)
              for b in (0, 8)]
    return pltpu.pack_elementwise(halves, packed_dtype=BF16)


def _riffled_iota(axis):
    i = lax.broadcasted_iota(I32, (T, T), axis)
    return (i & ~15) | ((i & 1) << 3) | ((i & 15) >> 1)


def _reciprocal(x):
    r = pl.reciprocal(x, approx=True)
    return r * (2.0 - x * r)


def _dot(a, b):
    return lax.dot_general(a, b, (((1,), (0,)), ((), ())), preferred_element_type=F32)


def _dot_nt(a, b):
    return lax.dot_general(a, b, (((1,), (1,)), ((), ())), preferred_element_type=F32)


def _at(n, size, offset=0, count=None):
    start = n * size if isinstance(n, int) else pl.multiple_of(n * size, size)
    return pl.ds(start + offset, size if count is None else count)


def _left(a11, a12, a21, a22):
    return [a11, a22, a11 + a22, a21 + a22, a11 + a12, a21 - a11, a12 - a22]


def _right(b11, b12, b21, b22):
    return [b12 - b22, b21 - b11, b11 + b22, b11, b22, b11 + b12, b21 + b22]


def _combine(m):
    return m[1] + m[2] - m[4] + m[6], m[0] + m[4], m[1] + m[3], m[0] + m[2] - m[3] + m[5]


def _half(words, index):
    return pltpu.unpack_elementwise(words, index=index, packed_dtype=BF16, unpacked_dtype=F32)


def _pack(lows, highs):
    return [pltpu.pack_elementwise([lo, hi], packed_dtype=BF16) for lo, hi in zip(lows, highs)]


def _on_words(sums, blocks):
    return _pack(*[sums(*[_half(b, index) for b in blocks]) for index in (0, 1)])


def _quarters(upper, lower):
    n = upper.shape[1] // 2
    return upper[:, :n], upper[:, n:], lower[:, :n], lower[:, n:]


def _exchange(tiles):
    lane = lax.broadcasted_iota(I32, tiles[0].shape, 1)
    for bit in (1, 2, 4):
        pick = (lane & bit) != 0
        tiles = [jnp.where(pick, tiles[k ^ bit], tiles[k]) for k in range(NB)]
    return tiles


def _permute_lanes(tiles):
    lane = lax.broadcasted_iota(I32, (8, T), 1)
    base = ((lane >> 2) & 0x18) | ((lane << 2) & 0x60) | (lane & 7)
    return [
        jnp.concatenate(
            [jnp.take_along_axis(t[r:r + 8], base ^ k, axis=1) for r in range(0, t.shape[0], 8)],
            axis=0)
        for k, t in enumerate(tiles)
    ]


def _tiles(a):
    return [a[:, c:c + T] for c in range(0, a.shape[1], T)]


def _shuffle(tiles):
    return jnp.concatenate(_permute_lanes(_exchange(tiles)), axis=1)


def _unshuffle(tiles):
    return jnp.concatenate(_exchange(_permute_lanes(tiles)), axis=1)


def _start(copies):
    for cp in copies:
        cp.start()


def _wait(copies):
    for cp in copies:
        cp.wait()


def _rows(src, dst, rows, sem):
    return pltpu.make_async_copy(src.bitcast(U32).at[rows], dst.at[rows], sem)


def _after(words, src, val):
    nonneg = pltpu.bitcast(words[0:8, 0:T] >> 1, I32)
    return jnp.where(jnp.tile(nonneg, (val.shape[0] // 8, 1)) < 0, src, val)


V_BASE = PAIRS * 7 * GROUPS * W


def _ctx_rows(hp, t, g):
    return _at((hp * 7 + t) * GROUPS + g, W)


def _project_out(ctx_s, wo_r, g, t, p0, p1, cols):
    ctx = jnp.concatenate([ctx_s[_ctx_rows(hp, t, g), :] for hp in range(p0, p1)], axis=1)
    return _dot(_bf16(ctx), _bf16(wo_r[t, (p0 + 1) * W:(p1 + 1) * W, cols]))


def _out_blocks(g, c0, width):
    return [(_at(2 * g + n // 2, T), pl.ds(n % 2 * (M // 2) + c0, width)) for n in range(4)]


def _prepare(later, ctx_s, wo_r, part_s, wqkv_v, bwo_v, wqkv_r, bwo_r):
    after = functools.partial(_after, bwo_v)
    _wait(later)

    def prepare(i, carry):
        for u in range(GROUPS // 2):
            g = GROUPS // 2 * i + u
            m = [_project_out(ctx_s, wo_r, g, t, 0, EARLY[1], pl.ds(MQ, MQ)) for t in range(7)]
            for at, y in zip(_out_blocks(g, MQ, MQ), _combine(m)):
                part_s[at] = y
            size = DB // 4 // GROUPS
            for n in range(6):
                which, r = n // 2, n % 2 * (size // 2)
                w = jnp.concatenate(
                    [wqkv_v[_at(g, size, k0 + r, size // 2), which * DB:(which + 1) * DB]
                     for k0 in (0, DB // 4)], axis=0)
                gate = pltpu.bitcast(m[n][:size, :T], U32)
                w = _shuffle([after(gate, a) for a in _tiles(w)])
                for t, a in enumerate(_on_words(_right, _quarters(w[:size // 2], w[size // 2:]))):
                    wqkv_r[which, t, _at(g, size, r, size // 2), :] = a
            for n, r in enumerate(range(0, size, 8)):
                gate = pltpu.bitcast(m[n][:8, T:], U32)
                w = [jnp.concatenate(
                    [after(gate, a) for a in _tiles(bwo_v[_at(g, size, k0 + r, 8), :])], axis=1)
                    for k0 in (0, DB // 4)]
                for t, a in enumerate(_on_words(_right, _quarters(*w))):
                    bwo_r[t, _at(g, size, r, 8), :] = a
        return carry

    lax.fori_loop(0, 2, prepare, None)


def _attention(x_hbm, c_hbm, wq_hbm, wuk_hbm, wuv_hbm, wo_hbm, later, prepare,
               ctx_s, wo_r, part_s,
               x_v, c_v, wq_v, wuk_v, wuv_v, wo_v, x_l, c_l, wq_r, wkv_r, q_s, k_s,
               c_sem, x_sem, in_sem):
    def pair(src, dst, hp, sem):
        return pltpu.make_async_copy(src.bitcast(U32).at[:, hp, 0], dst.at[hp], sem)

    def head_pairs(p0, p1, sem):
        return [pair(src, dst, hp, sem) for hp in range(p0, p1)
                for src, dst in ((wq_hbm, wq_v), (wuk_hbm, wuk_v), (wuv_hbm, wuv_v))]

    def out_weights(p0, p1, sem):
        return [_rows(wo_hbm, wo_v.at[pl.ds(T, PAIRS * T)], pl.ds(p0 * T, (p1 - p0) * T), sem)]

    def c_copies(n):
        return [_rows(c_hbm, c_v, _at(n, STEP * T), c_sem.at[n])]

    def x_copies(n):
        return [_rows(x_hbm, x_v, _at(n, STEP * T), x_sem.at[n])]

    wkv_first = [pair(wuk_hbm, wuk_v, 0, in_sem.at[0]), pair(wuv_hbm, wuv_v, 0, in_sem.at[0])]
    wq_first = [pair(wq_hbm, wq_v, 0, in_sem.at[1])]
    second = head_pairs(1, 2, in_sem.at[5])
    step0 = head_pairs(2, 3, in_sem.at[2])
    step1 = head_pairs(3, 6, in_sem.at[3]) + out_weights(0, 3, in_sem.at[3])
    step4 = head_pairs(6, PAIRS, in_sem.at[4]) + out_weights(3, PAIRS, in_sem.at[4])
    _start(wkv_first)
    for n in range(GROUPS // STEP):
        _start(c_copies(n))
    _start(wq_first)
    for n in range(GROUPS // STEP):
        _start(x_copies(n) + ([] if n else second))
    _start(step0 + step1 + step4 + later)
    wo_v[0:T, :] = jnp.zeros((T, M), U32)

    def stage(src, hp, r, n):
        k = src.shape[1] // 2
        sums = []
        for odd_row in (0, 1):
            top, low = (src[hp, pl.ds(2 * r + (k0 + odd_row), n, stride=2), :] for k0 in (0, k))
            sums.append(_right(_half(top, 0), _half(top, 1), _half(low, 0), _half(low, 1)))
        return _pack(*sums)

    def stage_q(hp, slot, r, n):
        words = stage(wq_v, hp, r, n)
        for t, w in enumerate(words):
            wq_r[slot, t, pl.ds(r, n), :] = w
        return words

    def stage_kv(hp, slot, which, r, n):
        words = stage((wuk_v, wuv_v)[which], hp, r, n)
        for t, w in enumerate(words):
            wkv_r[slot, t, pl.ds(r, n), which * D:(which + 1) * D] = w
        return words

    def stage_out(slab, unit):
        r, c = unit // 4 * 8, unit % 4 * T
        blocks = [wo_v[_at(slab, T, head * W + r, 8), c0 + c:c0 + c + T]
                  for head in (0, 1) for c0 in (0, M // 2)]
        words = _on_words(_right, blocks)
        for t, w in enumerate(words):
            wo_r[t, _at(slab, W, r, 8), c:c + T] = w
        return words

    def store_q(g, lower, odd, q):
        q_s[odd, _at(g, T, lower * W, W), :] = _riffle(q * Q_SCALE)

    def store_k(g, lower, odd, kv):
        k_s[odd, _at(g, T, lower * W, W), :] = _riffle(kv[:, :D])

    def store_v(g, lower, odd, kv):
        ctx_s[_at(g, T, V_BASE + odd * (S // 2) + lower * W, W), :] = _riffle(kv[:, D:])

    def first_projections(copies, src, left_s, right_s, stores, also):
        def step(n, carry):
            _wait(copies(n))
            for u in range(STEP):
                g = n * STEP + u
                left = _on_words(_left, _quarters(src[_at(g, T, 0, W), :], src[_at(g, T, W, W), :]))
                for t, w in enumerate(left[2:]):
                    left_s[t, _at(g, W), :] = w
                out = _combine([_dot(_bf16(left[t]), _bf16(right_s[0, t])) for t in range(7)])
                for b, y in enumerate(out):
                    for store in stores:
                        store(g, b // 2, b % 2, y)
                also(g)
            return carry

        lax.fori_loop(0, GROUPS // STEP, step, None)

    def stage_part(hp, g, q=True, kv=True):
        size = DC // 4 // GROUPS
        r = pl.multiple_of(g * size, size)
        if q:
            stage_q(hp, hp, 2 * r, 2 * size)
        for which in (0, 1) if kv else ():
            stage_kv(hp, hp, which, r, size)

    _wait(wkv_first)
    pl.loop(0, GROUPS)(functools.partial(stage_part, 0, q=False))
    first_projections(c_copies, c_v, c_l, wkv_r, (store_k, store_v), lambda g: None)
    _wait(wq_first)
    pl.loop(0, GROUPS)(functools.partial(stage_part, 0, kv=False))
    _wait(second)
    first_projections(x_copies, x_v, x_l, wq_r, (store_q,), functools.partial(stage_part, 1))
    _wait(step0)

    def attend(g, lower, odd, chores, fill, v_base):
        tile = 2 * g + lower
        keys = (tile + 1) * W
        s = _tiles(_dot_nt(_bf16(q_s[odd, _at(tile, W), :]), _bf16(k_s[odd, 0:keys, :])))
        s[-1] = jnp.where(_riffled_iota(1) <= _riffled_iota(0), s[-1], NEG)
        top = functools.reduce(jnp.maximum, s)
        top = [top[r:r + 8] for r in range(0, T, 8)]
        for n, w in enumerate(chores):
            top[n % len(top)] = _after(c_v, pltpu.bitcast(w, F32), top[n % len(top)])
        top = jnp.max(jnp.concatenate(top, axis=0), axis=1, keepdims=True)
        top = jnp.broadcast_to(top, (T, T))
        gates = fill()[-3:]
        v = ctx_s[pl.ds(v_base + odd * (S // 2), keys), :]
        total = ctx = None
        for j in range(0, len(s), EXP_TILES):
            at = _after(c_v, gates.pop(0)[:, -T:], top)
            p = [jnp.exp2(a - at) for a in s[j:j + EXP_TILES]]
            total = functools.reduce(jnp.add, p if total is None else [total] + p)
            y = _dot(jnp.concatenate(p, axis=1).astype(BF16),
                     _bf16(v[j * W:(j + len(p)) * W]))
            ctx = y if ctx is None else ctx + y
            gates.append(y)
        return ctx * _reciprocal(jnp.sum(total, axis=1, keepdims=True))

    def head_pair(hp, products, chores, done, v_base=V_BASE):
        cuts = (0, 3, 7, 10, 14)
        for g in reversed(range(GROUPS)):
            todo, m, ctx = products(g), [], {}
            for b, (lower, odd) in enumerate(((1, 0), (1, 1), (0, 0), (0, 1))):
                def fill():
                    m.extend(f() for f in todo[cuts[b]:cuts[b + 1]])
                    done(g, b, m, False)
                    return m[cuts[b]:]

                ctx[lower, odd] = attend(g, lower, odd, chores(4 * g + b), fill, v_base)
                done(g, b, m, True)
                left = _left(*[ctx.get(k, ctx[1, 0]) for k in ((0, 0), (0, 1), (1, 0), (1, 1))])
                for t in ((), (1, 3), (0, 2, 5), (4, 6))[b]:
                    ctx_s[_ctx_rows(hp, t, g), :] = _riffle(left[t])

    def pair_step(hp, carry):
        pl.when(hp == 1)(lambda: _wait(step1))
        pl.when(hp == 4)(lambda: _wait(step4))
        slot = (hp + 1) % 2
        held = {}

        def products(g):
            def product(src, sums, right, t):
                k = sums.shape[2]
                left = (sums[t - 2, _at(g, W), :] if t >= 2
                        else src[_at(2 * g + t, W), pl.ds(t * k, k)])
                return _dot(_bf16(left), _bf16(right[slot, t]))

            return [functools.partial(product, *refs, t)
                    for refs in ((x_v, x_l, wq_r), (c_v, c_l, wkv_r)) for t in range(7)]

        def chores(unit):
            ahead = jnp.minimum(hp + 2, PAIRS - 1)
            stage_out(hp, unit)
            words = zip(stage_q(ahead, 1 - slot, unit * 8, 8),
                        stage_kv(ahead, 1 - slot, unit % 2, unit // 2 * 8, 8))
            return [w for group in words for w in group]

        def done(g, b, m, attended):
            if (b, attended) == (1, False):
                held["q"] = _combine(m[:7])
                for odd in (0, 1):
                    store_q(g, 1, odd, held["q"][2 + odd])
            if b >= 2 and not attended:
                store_q(g, 0, b - 2, held["q"][b - 2])
            if (b, attended) == (3, False):
                held["kv"] = _combine(m[7:])
                for n, y in enumerate(held["kv"]):
                    store_k(g, n // 2, n % 2, y)
                    if n != 1:
                        store_v(g, n // 2, n % 2, y)
            if (b, attended) == (3, True):
                store_v(g, 0, 1, held["kv"][1])

        head_pair(hp, products, chores, done)
        return carry + V_BASE // (PAIRS - 1)

    v_base = lax.fori_loop(0, PAIRS - 1, pair_step, V_BASE % (PAIRS - 1))

    prepare()

    def early(g):
        return [functools.partial(_project_out, ctx_s, wo_r, g, t, 0, EARLY[0], pl.ds(c0, T))
                for c0 in (0, T) for t in range(7)]

    def early_done(g, b, m, attended):
        if b % 2 and not attended:
            for at, y in zip(_out_blocks(g, b // 2 * T, T), _combine(m[-7:])):
                part_s[at] = y

    def last_weights(unit):
        return stage_out(PAIRS - 1, unit) + stage_out(PAIRS, unit)

    @pl.loop(V_BASE, v_base + 1)
    def _(base):
        head_pair(PAIRS - 1, early, last_weights, early_done, pl.multiple_of(base, W))


def _outputs(out_hbm, ctx_s, wo_r, part_s, bx_v, wqkv_r, bwo_r, bk_s, bv_s, out_s, out_sem):
    after = functools.partial(_after, bx_v)
    for j in range(NB):
        bk_s[j, 0:HALO, :] = jnp.zeros((HALO, T), F32)
        bv_s[j, 0:HALO, :] = jnp.zeros((HALO, T), F32)

    def b_proj(left, right):
        m = [_dot(left[t], _bf16(right[t])) for t in range(7)]
        c11, c12, c21, c22 = _combine(m)
        return m, jnp.concatenate(
            [jnp.concatenate([c11, c12], axis=1), jnp.concatenate([c21, c22], axis=1)], axis=0)

    def b_weights(pos, r, q, gate):
        logits = [None] * WIN
        for j, qj in enumerate(_tiles(q[r:r + G])):
            qj = after(gate[j * G:(j + 1) * G], qj) * (DH ** -0.5 * LOG2E)
            for w in range(WIN):
                t = qj * bk_s[j, pl.ds(HALO + r - DIL * w, G), :]
                logits[w] = t if logits[w] is None else logits[w] + t
        for w in range(WIN):
            t = logits[w] + pltpu.roll(logits[w], 64, 1)
            t = t + pltpu.roll(t, 32, 1)
            if r < DIL * w:
                t = jnp.where(pos + r + lax.broadcasted_iota(I32, (G, T), 0) >= DIL * w, t, NEG)
            logits[w] = t
        top = functools.reduce(jnp.maximum, logits)
        e = [jnp.exp2(t - top) for t in logits]
        inv = _reciprocal(functools.reduce(jnp.add, e))
        return [t * inv for t in e]

    def b_mix(r, attn, gate):
        acc = [None] * NB
        for w in range(WIN):
            a = after(gate[w * G:(w + 1) * G], attn[w])
            for j in range(NB):
                t = a * bv_s[j, pl.ds(HALO + r - DIL * w, G), :]
                acc[j] = t if acc[j] is None else acc[j] + t
        return _unshuffle(acc)

    def out_copy(g, r0, rows, c0, cols):
        return pltpu.make_async_copy(
            out_s.at[g % 2, pl.ds(r0, rows), pl.ds(c0, cols)],
            out_hbm.at[_at(g, 2 * T, r0, rows), pl.ds(c0, cols)], out_sem.at[g % 2])

    def out_wait(g):
        out_copy(g, 0, 2 * T, 0, M + DB).wait()

    def group(g, carry):
        pl.when(g >= 2)(lambda: out_wait(g - 2))
        xs = _on_words(_left, _quarters(bx_v[_at(g, T, 0, W), :], bx_v[_at(g, T, W, W), :]))
        xs = [_bf16(a) for a in xs]
        _, k = b_proj(xs, wqkv_r.at[1])
        for j, t in enumerate(_tiles(k)):
            bk_s[j, HALO:, :] = t
        _, q = b_proj(xs, wqkv_r.at[0])
        m, v = b_proj(xs, wqkv_r.at[2])
        for j, t in enumerate(_tiles(v)):
            bv_s[j, HALO:, :] = t
        gates = [t for y in m for t in _tiles(y)[1::2]]
        late = [[_project_out(ctx_s, wo_r, g, t, EARLY[c], PAIRS, pl.ds(c * MQ, MQ))
                 for t in range(7)] for c in (0, 1)]
        gates += [t for m in late for y in m for t in _tiles(y)]
        rows = range(0, 2 * T, G)
        attn = [b_weights(g * (2 * T), r, q, gates[n]) for n, r in enumerate(rows)]
        o = jnp.concatenate(
            [b_mix(r, attn[n], gates[len(rows) + 1 + n]) for n, r in enumerate(rows)], axis=0)
        for c, m in enumerate(late):
            for n, (at, y) in enumerate(zip(_out_blocks(g, c * MQ, MQ), _combine(m))):
                y = _bf16(_riffle(part_s[at] + y)).astype(F32)
                out_s[g % 2, _at(n // 2, T), at[1]] = _bf16(_riffle(y))
        out_copy(g, 0, 2 * T, 0, M).start()
        for j in range(NB):
            bk_s[j, 0:HALO, :] = bk_s[j, 2 * T:, :]
            bv_s[j, 0:HALO, :] = bv_s[j, 2 * T:, :]
        m, _ = b_proj([a.astype(BF16) for a in _left(*_quarters(o[:T], o[T:]))], bwo_r)
        y = _combine(m)
        for n in (2, 1, 3, 0):
            r0, c0 = n // 2 * T, M + n % 2 * (DB // 2)
            out_s[g % 2, r0:r0 + T, c0:c0 + DB // 2] = y[n].astype(BF16)
            out_copy(g, r0, T, c0, DB // 2).start()
        return carry

    lax.fori_loop(0, GROUPS, group, None)
    for g in range(GROUPS - 2, GROUPS):
        out_wait(g)


def _kernel(x_hbm, c_hbm, wq_hbm, wuk_hbm, wuv_hbm, wo_hbm, bx_hbm, wqkv_hbm, bwo_hbm,
            out_hbm, ctx_s, wo_r, part_s, bx_v, wqkv_v, bwo_v, wqkv_r, bwo_r, later_sem):
    later = [_rows(src, dst, slice(None), later_sem)
             for src, dst in ((bx_hbm, bx_v), (wqkv_hbm, wqkv_v), (bwo_hbm, bwo_v))]
    prepare = functools.partial(_prepare, later, ctx_s, wo_r, part_s, wqkv_v, bwo_v, wqkv_r, bwo_r)
    pl.run_scoped(
        functools.partial(_attention, x_hbm, c_hbm, wq_hbm, wuk_hbm, wuv_hbm, wo_hbm, later,
                          prepare, ctx_s, wo_r, part_s),
        pltpu.VMEM((S // 2, M), U32),
        pltpu.VMEM((S // 2, DC), U32),
        pltpu.VMEM((PAIRS, M, D), U32),
        pltpu.VMEM((PAIRS, DC, D), U32),
        pltpu.VMEM((PAIRS, DC, D), U32),
        pltpu.VMEM(((PAIRS + 1) * T, M), U32),
        pltpu.VMEM((5, S // 4, M // 2), U32),
        pltpu.VMEM((5, S // 4, DC // 2), U32),
        pltpu.VMEM((2, 7, M // 4, D), U32),
        pltpu.VMEM((2, 7, DC // 4, 2 * D), U32),
        pltpu.VMEM((2, S // 2, D), U32),
        pltpu.VMEM((2, S // 2, D), U32),
        pltpu.SemaphoreType.DMA((GROUPS // STEP,)),
        pltpu.SemaphoreType.DMA((GROUPS // STEP,)),
        pltpu.SemaphoreType.DMA((6,)),
    )
    pl.run_scoped(
        functools.partial(_outputs, out_hbm, ctx_s, wo_r, part_s, bx_v, wqkv_r, bwo_r),
        pltpu.VMEM((NB, HALO + 2 * T, T), F32),
        pltpu.VMEM((NB, HALO + 2 * T, T), F32),
        pltpu.VMEM((2, 2 * T, M + DB), BF16),
        pltpu.SemaphoreType.DMA((2,)),
    )


@jax.jit
def pallas_concat_heads__compressed_kv_cla__sliding_local_dilated__prompt_kernel(
    A_x: jax.Array,
    A_c_kv: jax.Array,
    A_w_q: jax.Array,
    A_w_uk: jax.Array,
    A_w_uv: jax.Array,
    A_w_o: jax.Array,
    B_x: jax.Array,
    B_wqkv: jax.Array,
    B_wo: jax.Array,
):
    out = pl.pallas_call(
        _kernel,
        out_shape=jax.ShapeDtypeStruct((S, M + DB), BF16),
        in_specs=[pl.BlockSpec(memory_space=pl.ANY)] * 9,
        out_specs=pl.BlockSpec(memory_space=pl.ANY),
        scratch_shapes=[
            pltpu.VMEM((V_BASE + S, D), U32),
            pltpu.VMEM((7, (PAIRS + 1) * W, M // 2), U32),
            pltpu.VMEM((S, M), F32),
            pltpu.VMEM((S // 2, DB), U32),
            pltpu.VMEM((DB // 2, 3 * DB), U32),
            pltpu.VMEM((DB // 2, DB), U32),
            pltpu.VMEM((3, 7, DB // 4, DB // 2), U32),
            pltpu.VMEM((7, DB // 4, DB // 2), U32),
            pltpu.SemaphoreType.DMA,
        ],
        compiler_params=pltpu.CompilerParams(vmem_limit_bytes=126 * 1024 * 1024),
        name="mla_local_concat",
    )(
        A_x.reshape(S, M),
        A_c_kv.reshape(S, DC),
        A_w_q.reshape(M, PAIRS, 2, D),
        A_w_uk.reshape(DC, PAIRS, 2, D),
        A_w_uv.reshape(DC, PAIRS, 2, D),
        A_w_o.reshape(H * D, M),
        B_x.reshape(S, DB),
        B_wqkv,
        B_wo,
    )
    return out.reshape(1, S, M + DB)
```

```python
import functools
import math

import jax
import jax.numpy as jnp
from jax import lax
import jax.experimental.pallas as pl
import jax.experimental.pallas.tpu as pltpu

BF16 = jnp.bfloat16
F32 = jnp.float32
U32 = jnp.uint32
I32 = jnp.int32

T = 128
W = T // 2
G = 16
LOG2E = math.log2(math.e)
NEG = -1e9 * LOG2E

S = 2048
GROUPS = S // (2 * T)
M = 1024
H = 32
D = 128
DC = 512
PAIRS = H // 2
Q_SCALE = D ** -0.5 * LOG2E
STEP = 2
EXP_TILES = 4
EARLY = (4, 5)
MQ = M // 4
DB = 1024
DH = 32
NB = DB // T
WIN = 8
DIL = 2
HALO = 16


def _bf16(words):
    return pltpu.bitcast(words, BF16)


def _riffle(val):
    halves = [jnp.concatenate([val[r + b:r + b + 8] for r in range(0, val.shape[0], G)], axis=0)
              for b in (0, 8)]
    return pltpu.pack_elementwise(halves, packed_dtype=BF16)


def _riffled_iota(axis):
    i = lax.broadcasted_iota(I32, (T, T), axis)
    return (i & ~15) | ((i & 1) << 3) | ((i & 15) >> 1)


def _reciprocal(x):
    r = pl.reciprocal(x, approx=True)
    return r * (2.0 - x * r)


def _dot(a, b):
    return lax.dot_general(a, b, (((1,), (0,)), ((), ())), preferred_element_type=F32)


def _dot_nt(a, b):
    return lax.dot_general(a, b, (((1,), (1,)), ((), ())), preferred_element_type=F32)


def _at(n, size, offset=0, count=None):
    start = n * size if isinstance(n, int) else pl.multiple_of(n * size, size)
    return pl.ds(start + offset, size if count is None else count)


def _left(a11, a12, a21, a22):
    return [a11, a22, a11 + a22, a21 + a22, a11 + a12, a21 - a11, a12 - a22]


def _right(b11, b12, b21, b22):
    return [b12 - b22, b21 - b11, b11 + b22, b11, b22, b11 + b12, b21 + b22]


def _combine(m):
    return m[1] + m[2] - m[4] + m[6], m[0] + m[4], m[1] + m[3], m[0] + m[2] - m[3] + m[5]


def _half(words, index):
    return pltpu.unpack_elementwise(words, index=index, packed_dtype=BF16, unpacked_dtype=F32)


def _pack(lows, highs):
    return [pltpu.pack_elementwise([lo, hi], packed_dtype=BF16) for lo, hi in zip(lows, highs)]


def _on_words(sums, blocks):
    return _pack(*[sums(*[_half(b, index) for b in blocks]) for index in (0, 1)])


def _quarters(upper, lower):
    n = upper.shape[1] // 2
    return upper[:, :n], upper[:, n:], lower[:, :n], lower[:, n:]


def _exchange(tiles):
    lane = lax.broadcasted_iota(I32, tiles[0].shape, 1)
    for bit in (1, 2, 4):
        pick = (lane & bit) != 0
        tiles = [jnp.where(pick, tiles[k ^ bit], tiles[k]) for k in range(NB)]
    return tiles


def _permute_lanes(tiles):
    lane = lax.broadcasted_iota(I32, (8, T), 1)
    base = ((lane >> 2) & 0x18) | ((lane << 2) & 0x60) | (lane & 7)
    return [
        jnp.concatenate(
            [jnp.take_along_axis(t[r:r + 8], base ^ k, axis=1) for r in range(0, t.shape[0], 8)],
            axis=0)
        for k, t in enumerate(tiles)
    ]


def _tiles(a):
    return [a[:, c:c + T] for c in range(0, a.shape[1], T)]


def _shuffle(tiles):
    return jnp.concatenate(_permute_lanes(_exchange(tiles)), axis=1)


def _unshuffle(tiles):
    return jnp.concatenate(_exchange(_permute_lanes(tiles)), axis=1)


def _start(copies):
    for cp in copies:
        cp.start()


def _wait(copies):
    for cp in copies:
        cp.wait()


def _rows(src, dst, rows, sem):
    return pltpu.make_async_copy(src.bitcast(U32).at[rows], dst.at[rows], sem)


def _after(words, src, val):
    nonneg = pltpu.bitcast(words[0:8, 0:T] >> 1, I32)
    return jnp.where(jnp.tile(nonneg, (val.shape[0] // 8, 1)) < 0, src, val)


V_BASE = PAIRS * 7 * GROUPS * W


def _ctx_rows(hp, t, g):
    return _at((hp * 7 + t) * GROUPS + g, W)


def _project_out(ctx_s, wo_r, g, t, p0, p1, cols):
    ctx = jnp.concatenate([ctx_s[_ctx_rows(hp, t, g), :] for hp in range(p0, p1)], axis=1)
    return _dot(_bf16(ctx), _bf16(wo_r[t, (p0 + 1) * W:(p1 + 1) * W, cols]))


def _out_blocks(g, c0, width):
    return [(_at(2 * g + n // 2, T), pl.ds(n % 2 * (M // 2) + c0, width)) for n in range(4)]


def _prepare(later, ctx_s, wo_r, part_s, wqkv_v, bwo_v, wqkv_r, bwo_r):
    after = functools.partial(_after, bwo_v)
    _wait(later)

    def prepare(i, carry):
        for u in range(GROUPS // 2):
            g = GROUPS // 2 * i + u
            m = [_project_out(ctx_s, wo_r, g, t, 0, EARLY[1], pl.ds(MQ, MQ)) for t in range(7)]
            for at, y in zip(_out_blocks(g, MQ, MQ), _combine(m)):
                part_s[at] = y
            size = DB // 4 // GROUPS
            for n in range(6):
                which, r = n // 2, n % 2 * (size // 2)
                w = jnp.concatenate(
                    [wqkv_v[_at(g, size, k0 + r, size // 2), which * DB:(which + 1) * DB]
                     for k0 in (0, DB // 4)], axis=0)
                gate = pltpu.bitcast(m[n][:size, :T], U32)
                w = _shuffle([after(gate, a) for a in _tiles(w)])
                for t, a in enumerate(_on_words(_right, _quarters(w[:size // 2], w[size // 2:]))):
                    wqkv_r[which, t, _at(g, size, r, size // 2), :] = a
            for n, r in enumerate(range(0, size, 8)):
                gate = pltpu.bitcast(m[n][:8, T:], U32)
                w = [jnp.concatenate(
                    [after(gate, a) for a in _tiles(bwo_v[_at(g, size, k0 + r, 8), :])], axis=1)
                    for k0 in (0, DB // 4)]
                for t, a in enumerate(_on_words(_right, _quarters(*w))):
                    bwo_r[t, _at(g, size, r, 8), :] = a
        return carry

    lax.fori_loop(0, 2, prepare, None)


def _attention(x_hbm, c_hbm, wq_hbm, wuk_hbm, wuv_hbm, wo_hbm, later, prepare,
               ctx_s, wo_r, part_s,
               x_v, c_v, wq_v, wuk_v, wuv_v, wo_v, x_l, c_l, wq_r, wkv_r, q_s, k_s,
               c_sem, x_sem, in_sem):
    def pair(src, dst, hp, sem):
        return pltpu.make_async_copy(src.bitcast(U32).at[:, hp, 0], dst.at[hp], sem)

    def head_pairs(p0, p1, sem):
        return [pair(src, dst, hp, sem) for hp in range(p0, p1)
                for src, dst in ((wq_hbm, wq_v), (wuk_hbm, wuk_v), (wuv_hbm, wuv_v))]

    def out_weights(p0, p1, sem):
        return [_rows(wo_hbm, wo_v.at[pl.ds(T, PAIRS * T)], pl.ds(p0 * T, (p1 - p0) * T), sem)]

    def c_copies(n):
        return [_rows(c_hbm, c_v, _at(n, STEP * T), c_sem.at[n])]

    def x_copies(n):
        return [_rows(x_hbm, x_v, _at(n, STEP * T), x_sem.at[n])]

    wkv_first = [pair(wuk_hbm, wuk_v, 0, in_sem.at[0]), pair(wuv_hbm, wuv_v, 0, in_sem.at[0])]
    wq_first = [pair(wq_hbm, wq_v, 0, in_sem.at[1])]
    second = head_pairs(1, 2, in_sem.at[5])
    step0 = head_pairs(2, 3, in_sem.at[2])
    step1 = head_pairs(3, 6, in_sem.at[3]) + out_weights(0, 3, in_sem.at[3])
    step4 = head_pairs(6, PAIRS, in_sem.at[4]) + out_weights(3, PAIRS, in_sem.at[4])
    _start(wkv_first)
    for n in range(GROUPS // STEP):
        _start(c_copies(n))
    _start(wq_first)
    for n in range(GROUPS // STEP):
        _start(x_copies(n) + ([] if n else second))
    _start(step0 + step1 + step4 + later)
    wo_v[0:T, :] = jnp.zeros((T, M), U32)

    def stage(src, hp, r, n):
        k = src.shape[1] // 2
        sums = []
        for odd_row in (0, 1):
            top, low = (src[hp, pl.ds(2 * r + (k0 + odd_row), n, stride=2), :] for k0 in (0, k))
            sums.append(_right(_half(top, 0), _half(top, 1), _half(low, 0), _half(low, 1)))
        return _pack(*sums)

    def stage_q(hp, slot, r, n):
        words = stage(wq_v, hp, r, n)
        for t, w in enumerate(words):
            wq_r[slot, t, pl.ds(r, n), :] = w
        return words

    def stage_kv(hp, slot, which, r, n):
        words = stage((wuk_v, wuv_v)[which], hp, r, n)
        for t, w in enumerate(words):
            wkv_r[slot, t, pl.ds(r, n), which * D:(which + 1) * D] = w
        return words

    def stage_out(slab, unit):
        r, c = unit // 4 * 8, unit % 4 * T
        blocks = [wo_v[_at(slab, T, head * W + r, 8), c0 + c:c0 + c + T]
                  for head in (0, 1) for c0 in (0, M // 2)]
        words = _on_words(_right, blocks)
        for t, w in enumerate(words):
            wo_r[t, _at(slab, W, r, 8), c:c + T] = w
        return words

    def store_q(g, lower, odd, q):
        q_s[odd, _at(g, T, lower * W, W), :] = _riffle(q * Q_SCALE)

    def store_k(g, lower, odd, kv):
        k_s[odd, _at(g, T, lower * W, W), :] = _riffle(kv[:, :D])

    def store_v(g, lower, odd, kv):
        ctx_s[_at(g, T, V_BASE + odd * (S // 2) + lower * W, W), :] = _riffle(kv[:, D:])

    def first_projections(copies, src, left_s, right_s, stores, also):
        def step(n, carry):
            _wait(copies(n))
            for u in range(STEP):
                g = n * STEP + u
                left = _on_words(_left, _quarters(src[_at(g, T, 0, W), :], src[_at(g, T, W, W), :]))
                for t, w in enumerate(left[2:]):
                    left_s[t, _at(g, W), :] = w
                out = _combine([_dot(_bf16(left[t]), _bf16(right_s[0, t])) for t in range(7)])
                for b, y in enumerate(out):
                    for store in stores:
                        store(g, b // 2, b % 2, y)
                also(g)
            return carry

        lax.fori_loop(0, GROUPS // STEP, step, None)

    def stage_part(hp, g, q=True, kv=True):
        size = DC // 4 // GROUPS
        r = pl.multiple_of(g * size, size)
        if q:
            stage_q(hp, hp, 2 * r, 2 * size)
        for which in (0, 1) if kv else ():
            stage_kv(hp, hp, which, r, size)

    _wait(wkv_first)
    pl.loop(0, GROUPS)(functools.partial(stage_part, 0, q=False))
    first_projections(c_copies, c_v, c_l, wkv_r, (store_k, store_v), lambda g: None)
    _wait(wq_first)
    pl.loop(0, GROUPS)(functools.partial(stage_part, 0, kv=False))
    _wait(second)
    first_projections(x_copies, x_v, x_l, wq_r, (store_q,), functools.partial(stage_part, 1))
    _wait(step0)

    def attend(g, lower, odd, chores, fill, v_base):
        tile = 2 * g + lower
        keys = (tile + 1) * W
        s = _tiles(_dot_nt(_bf16(q_s[odd, _at(tile, W), :]), _bf16(k_s[odd, 0:keys, :])))
        s[-1] = jnp.where(_riffled_iota(1) <= _riffled_iota(0), s[-1], NEG)
        top = functools.reduce(jnp.maximum, s)
        top = [top[r:r + 8] for r in range(0, T, 8)]
        for n, w in enumerate(chores):
            top[n % len(top)] = _after(c_v, pltpu.bitcast(w, F32), top[n % len(top)])
        top = jnp.max(jnp.concatenate(top, axis=0), axis=1, keepdims=True)
        top = jnp.broadcast_to(top, (T, T))
        gates = fill()[-3:]
        v = ctx_s[pl.ds(v_base + odd * (S // 2), keys), :]
        total = ctx = None
        for j in range(0, len(s), EXP_TILES):
            at = _after(c_v, gates.pop(0)[:, -T:], top)
            p = [jnp.exp2(a - at) for a in s[j:j + EXP_TILES]]
            total = functools.reduce(jnp.add, p if total is None else [total] + p)
            words = _riffle(jnp.concatenate(p, axis=1))
            y = _dot(_bf16(words), _bf16(v[j * W:(j + len(p)) * W]))
            if len(s) > 6:
                rows = [total[r:r + 8] for r in range(0, T, 8)]
                for n, w in enumerate(_tiles(pltpu.bitcast(words, F32))):
                    for r in range(8):
                        rows[2 * r + n % 2] = _after(c_v, w[8 * r:8 * r + 8], rows[2 * r + n % 2])
                total = jnp.concatenate(rows, axis=0)
            ctx = y if ctx is None else ctx + y
            gates.append(y)
        inv = jnp.broadcast_to(_reciprocal(jnp.sum(total, axis=1, keepdims=True)), (T, T))
        head = _half(pltpu.bitcast(inv, U32), 1)
        return ctx * sum(_bf16(_riffle(a)).astype(F32) for a in (head, inv - head))

    def head_pair(hp, products, chores, done, v_base=V_BASE):
        cuts = (0, 3, 7, 10, 14)
        for g in reversed(range(GROUPS)):
            todo, m, ctx = products(g), [], {}
            for b, (lower, odd) in enumerate(((1, 0), (1, 1), (0, 0), (0, 1))):
                def fill():
                    m.extend(f() for f in todo[cuts[b]:cuts[b + 1]])
                    done(g, b, m, False)
                    return m[cuts[b]:]

                ctx[lower, odd] = attend(g, lower, odd, chores(4 * g + b), fill, v_base)
                done(g, b, m, True)
                left = _left(*[ctx.get(k, ctx[1, 0]) for k in ((0, 0), (0, 1), (1, 0), (1, 1))])
                for t in ((), (1, 3), (0, 2, 5), (4, 6))[b]:
                    ctx_s[_ctx_rows(hp, t, g), :] = _riffle(left[t])

    def pair_step(hp, carry):
        pl.when(hp == 1)(lambda: _wait(step1))
        pl.when(hp == 4)(lambda: _wait(step4))
        slot = (hp + 1) % 2
        held = {}

        def products(g):
            def product(src, sums, right, t):
                k = sums.shape[2]
                left = (sums[t - 2, _at(g, W), :] if t >= 2
                        else src[_at(2 * g + t, W), pl.ds(t * k, k)])
                return _dot(_bf16(left), _bf16(right[slot, t]))

            return [functools.partial(product, *refs, t)
                    for refs in ((x_v, x_l, wq_r), (c_v, c_l, wkv_r)) for t in range(7)]

        def chores(unit):
            ahead = jnp.minimum(hp + 2, PAIRS - 1)
            stage_out(hp, unit)
            words = zip(stage_q(ahead, 1 - slot, unit * 8, 8),
                        stage_kv(ahead, 1 - slot, unit % 2, unit // 2 * 8, 8))
            return [w for group in words for w in group]

        def done(g, b, m, attended):
            if (b, attended) == (1, False):
                held["q"] = _combine(m[:7])
                for odd in (0, 1):
                    store_q(g, 1, odd, held["q"][2 + odd])
            if b >= 2 and not attended:
                store_q(g, 0, b - 2, held["q"][b - 2])
            if (b, attended) == (3, False):
                held["kv"] = _combine(m[7:])
                for n, y in enumerate(held["kv"]):
                    store_k(g, n // 2, n % 2, y)
                    if n != 1:
                        store_v(g, n // 2, n % 2, y)
            if (b, attended) == (3, True):
                store_v(g, 0, 1, held["kv"][1])

        head_pair(hp, products, chores, done)
        return carry + V_BASE // (PAIRS - 1)

    v_base = lax.fori_loop(0, PAIRS - 1, pair_step, V_BASE % (PAIRS - 1))

    prepare()

    def early(g):
        return [functools.partial(_project_out, ctx_s, wo_r, g, t, 0, EARLY[0], pl.ds(c0, T))
                for c0 in (0, T) for t in range(7)]

    def early_done(g, b, m, attended):
        if b % 2 and not attended:
            for at, y in zip(_out_blocks(g, b // 2 * T, T), _combine(m[-7:])):
                part_s[at] = y

    def last_weights(unit):
        return stage_out(PAIRS - 1, unit) + stage_out(PAIRS, unit)

    @pl.loop(V_BASE, v_base + 1)
    def _(base):
        head_pair(PAIRS - 1, early, last_weights, early_done, pl.multiple_of(base, W))


def _outputs(out_hbm, ctx_s, wo_r, part_s, bx_v, wqkv_r, bwo_r, bk_s, bv_s, out_s, out_sem):
    after = functools.partial(_after, bx_v)
    for j in range(NB):
        bk_s[j, 0:HALO, :] = jnp.zeros((HALO, T), F32)
        bv_s[j, 0:HALO, :] = jnp.zeros((HALO, T), F32)

    def b_proj(left, right):
        m = [_dot(left[t], _bf16(right[t])) for t in range(7)]
        c11, c12, c21, c22 = _combine(m)
        return m, jnp.concatenate(
            [jnp.concatenate([c11, c12], axis=1), jnp.concatenate([c21, c22], axis=1)], axis=0)

    def b_weights(pos, r, q, gate):
        logits = [None] * WIN
        for j, qj in enumerate(_tiles(q[r:r + G])):
            qj = after(gate[j * G:(j + 1) * G], qj) * (DH ** -0.5 * LOG2E)
            for w in range(WIN):
                t = qj * bk_s[j, pl.ds(HALO + r - DIL * w, G), :]
                logits[w] = t if logits[w] is None else logits[w] + t
        for w in range(WIN):
            t = logits[w] + pltpu.roll(logits[w], 64, 1)
            t = t + pltpu.roll(t, 32, 1)
            if r < DIL * w:
                t = jnp.where(pos + r + lax.broadcasted_iota(I32, (G, T), 0) >= DIL * w, t, NEG)
            logits[w] = t
        top = functools.reduce(jnp.maximum, logits)
        e = [jnp.exp2(t - top) for t in logits]
        inv = _reciprocal(functools.reduce(jnp.add, e))
        return [t * inv for t in e]

    def b_mix(r, attn, gate):
        acc = [None] * NB
        for w in range(WIN):
            a = after(gate[w * G:(w + 1) * G], attn[w])
            for j in range(NB):
                t = a * bv_s[j, pl.ds(HALO + r - DIL * w, G), :]
                acc[j] = t if acc[j] is None else acc[j] + t
        return _unshuffle(acc)

    def out_copy(g, r0, rows, c0, cols):
        return pltpu.make_async_copy(
            out_s.at[g % 2, pl.ds(r0, rows), pl.ds(c0, cols)],
            out_hbm.at[_at(g, 2 * T, r0, rows), pl.ds(c0, cols)], out_sem.at[g % 2])

    def out_wait(g):
        out_copy(g, 0, 2 * T, 0, M + DB).wait()

    def group(g, carry):
        pl.when(g >= 2)(lambda: out_wait(g - 2))
        xs = _on_words(_left, _quarters(bx_v[_at(g, T, 0, W), :], bx_v[_at(g, T, W, W), :]))
        xs = [_bf16(a) for a in xs]
        _, k = b_proj(xs, wqkv_r.at[1])
        for j, t in enumerate(_tiles(k)):
            bk_s[j, HALO:, :] = t
        _, q = b_proj(xs, wqkv_r.at[0])
        m, v = b_proj(xs, wqkv_r.at[2])
        for j, t in enumerate(_tiles(v)):
            bv_s[j, HALO:, :] = t
        gates = [t for y in m for t in _tiles(y)[1::2]]
        late = [[_project_out(ctx_s, wo_r, g, t, EARLY[c], PAIRS, pl.ds(c * MQ, MQ))
                 for t in range(7)] for c in (0, 1)]
        gates += [t for m in late for y in m for t in _tiles(y)]
        rows = range(0, 2 * T, G)
        attn = [b_weights(g * (2 * T), r, q, gates[n]) for n, r in enumerate(rows)]
        o = jnp.concatenate(
            [b_mix(r, attn[n], gates[len(rows) + 1 + n]) for n, r in enumerate(rows)], axis=0)
        for c, m in enumerate(late):
            for n, (at, y) in enumerate(zip(_out_blocks(g, c * MQ, MQ), _combine(m))):
                out_s[g % 2, _at(n // 2, T), at[1]] = _bf16(_riffle(part_s[at] + y))
        out_copy(g, 0, 2 * T, 0, M).start()
        for j in range(NB):
            bk_s[j, 0:HALO, :] = bk_s[j, 2 * T:, :]
            bv_s[j, 0:HALO, :] = bv_s[j, 2 * T:, :]
        m, _ = b_proj([a.astype(BF16) for a in _left(*_quarters(o[:T], o[T:]))], bwo_r)
        y = _combine(m)
        for n in (2, 1, 3, 0):
            r0, c0 = n // 2 * T, M + n % 2 * (DB // 2)
            out_s[g % 2, r0:r0 + T, c0:c0 + DB // 2] = y[n].astype(BF16)
            out_copy(g, r0, T, c0, DB // 2).start()
        return carry

    lax.fori_loop(0, GROUPS, group, None)
    for g in range(GROUPS - 2, GROUPS):
        out_wait(g)


def _kernel(x_hbm, c_hbm, wq_hbm, wuk_hbm, wuv_hbm, wo_hbm, bx_hbm, wqkv_hbm, bwo_hbm,
            out_hbm, ctx_s, wo_r, part_s, bx_v, wqkv_v, bwo_v, wqkv_r, bwo_r, later_sem):
    later = [_rows(src, dst, slice(None), later_sem)
             for src, dst in ((bx_hbm, bx_v), (wqkv_hbm, wqkv_v), (bwo_hbm, bwo_v))]
    prepare = functools.partial(_prepare, later, ctx_s, wo_r, part_s, wqkv_v, bwo_v, wqkv_r, bwo_r)
    pl.run_scoped(
        functools.partial(_attention, x_hbm, c_hbm, wq_hbm, wuk_hbm, wuv_hbm, wo_hbm, later,
                          prepare, ctx_s, wo_r, part_s),
        pltpu.VMEM((S // 2, M), U32),
        pltpu.VMEM((S // 2, DC), U32),
        pltpu.VMEM((PAIRS, M, D), U32),
        pltpu.VMEM((PAIRS, DC, D), U32),
        pltpu.VMEM((PAIRS, DC, D), U32),
        pltpu.VMEM(((PAIRS + 1) * T, M), U32),
        pltpu.VMEM((5, S // 4, M // 2), U32),
        pltpu.VMEM((5, S // 4, DC // 2), U32),
        pltpu.VMEM((2, 7, M // 4, D), U32),
        pltpu.VMEM((2, 7, DC // 4, 2 * D), U32),
        pltpu.VMEM((2, S // 2, D), U32),
        pltpu.VMEM((2, S // 2, D), U32),
        pltpu.SemaphoreType.DMA((GROUPS // STEP,)),
        pltpu.SemaphoreType.DMA((GROUPS // STEP,)),
        pltpu.SemaphoreType.DMA((6,)),
    )
    pl.run_scoped(
        functools.partial(_outputs, out_hbm, ctx_s, wo_r, part_s, bx_v, wqkv_r, bwo_r),
        pltpu.VMEM((NB, HALO + 2 * T, T), F32),
        pltpu.VMEM((NB, HALO + 2 * T, T), F32),
        pltpu.VMEM((2, 2 * T, M + DB), BF16),
        pltpu.SemaphoreType.DMA((2,)),
    )


@jax.jit
def pallas_concat_heads__compressed_kv_cla__sliding_local_dilated__prompt_kernel(
    A_x: jax.Array,
    A_c_kv: jax.Array,
    A_w_q: jax.Array,
    A_w_uk: jax.Array,
    A_w_uv: jax.Array,
    A_w_o: jax.Array,
    B_x: jax.Array,
    B_wqkv: jax.Array,
    B_wo: jax.Array,
):
    out = pl.pallas_call(
        _kernel,
        out_shape=jax.ShapeDtypeStruct((S, M + DB), BF16),
        in_specs=[pl.BlockSpec(memory_space=pl.ANY)] * 9,
        out_specs=pl.BlockSpec(memory_space=pl.ANY),
        scratch_shapes=[
            pltpu.VMEM((V_BASE + S, D), U32),
            pltpu.VMEM((7, (PAIRS + 1) * W, M // 2), U32),
            pltpu.VMEM((S, M), F32),
            pltpu.VMEM((S // 2, DB), U32),
            pltpu.VMEM((DB // 2, 3 * DB), U32),
            pltpu.VMEM((DB // 2, DB), U32),
            pltpu.VMEM((3, 7, DB // 4, DB // 2), U32),
            pltpu.VMEM((7, DB // 4, DB // 2), U32),
            pltpu.SemaphoreType.DMA,
        ],
        compiler_params=pltpu.CompilerParams(vmem_limit_bytes=126 * 1024 * 1024),
        name="mla_local_concat",
    )(
        A_x.reshape(S, M),
        A_c_kv.reshape(S, DC),
        A_w_q.reshape(M, PAIRS, 2, D),
        A_w_uk.reshape(DC, PAIRS, 2, D),
        A_w_uv.reshape(DC, PAIRS, 2, D),
        A_w_o.reshape(H * D, M),
        B_x.reshape(S, DB),
        B_wqkv,
        B_wo,
    )
    return out.reshape(1, S, M + DB)
```
